```python
import jax
import jax.numpy as jnp

def _softmax(x, axis=-1):
    return jax.nn.softmax(x, axis=axis)

def _gelu(x):
    return jax.nn.gelu(x, approximate=True)

def _silu(x):
    return jax.nn.silu(x)

def _sigmoid(x):
    return jax.nn.sigmoid(x)

def _layernorm(x, axis=-1, eps=1e-05):
    m = jnp.mean(x, axis=axis, keepdims=True)
    v = jnp.var(x, axis=axis, keepdims=True)
    return (x - m) / jnp.sqrt(v + eps)

def _scatter_add(tgt, idx, src, axis=0):
    return tgt.at[idx].add(src)

def _segment_sum(src, seg, n):
    return jax.ops.segment_sum(src, seg, n)

class _Rng:

    def __init__(self, key):
        self._k = key

    def _next(self):
        self._k, sub = jax.random.split(self._k)
        return sub

    def normal(self, shape):
        return jax.random.normal(self._next(), shape, dtype=jnp.bfloat16)

    def randint(self, lo, hi, shape):
        return jax.random.randint(self._next(), shape, lo, hi, dtype=jnp.int32)

    def uniform(self, shape, lo=0.0, hi=1.0):
        return jax.random.uniform(self._next(), shape, jnp.bfloat16, lo, hi)

    def permutation(self, n):
        return jax.random.permutation(self._next(), n)
kernel_name = 'adaLN_cond__compressed_kv_cla__mixer_s_mlp__prompt'

def setup_inputs():
    _rng = _Rng(jax.random.key(int.from_bytes(__import__("os").urandom(4), "little")))
    _w = lambda a: (lambda t: t.astype(jnp.bfloat16) if jnp.issubdtype(t.dtype, jnp.floating) else t)(jnp.asarray(a))

    def _A_setup():
        B, H, Sq, Sk, D, M = (1, 32, 2048, 2048, 128, 640)
        Dc = 4 * D
        return {'x': _w((lambda *s: _rng.normal(s) * 0.05)(B, Sq, M)), 'c_kv': _w((lambda *s: _rng.normal(s) * 0.05)(B, Sk, Dc)), 'w_q': _w((lambda *s: _rng.normal(s) * 0.05)(M, H, D) * M ** (-0.5)), 'w_uk': _w((lambda *s: _rng.normal(s) * 0.05)(Dc, H, D) * Dc ** (-0.5)), 'w_uv': _w((lambda *s: _rng.normal(s) * 0.05)(Dc, H, D) * Dc ** (-0.5)), 'w_o': _w((lambda *s: _rng.normal(s) * 0.05)(H, D, M) * (H * D) ** (-0.5))}
    _A_in = _A_setup()

    def _B_setup():
        B, S, D, F = (1, 2048, 640, 1728)
        return {'x': _w((lambda *s: _rng.normal(s) * 0.05)(B, S, D)), 'w1': _w((lambda *s: _rng.normal(s) * 0.05)(D, D) * D ** (-0.5)), 'w2': _w((lambda *s: _rng.normal(s) * 0.05)(D, D) * D ** (-0.5)), 'w3': _w((lambda *s: _rng.normal(s) * 0.05)(D, F) * D ** (-0.5)), 'w4': _w((lambda *s: _rng.normal(s) * 0.05)(F, D) * F ** (-0.5))}
    _B_in = _B_setup()
    return {'A_x': _A_in['x'], 'A_c_kv': _A_in['c_kv'], 'A_w_q': _A_in['w_q'], 'A_w_uk': _A_in['w_uk'], 'A_w_uv': _A_in['w_uv'], 'A_w_o': _A_in['w_o'], 'B_x': _B_in['x'], 'B_w1': _B_in['w1'], 'B_w2': _B_in['w2'], 'B_w3': _B_in['w3'], 'B_w4': _B_in['w4'], 'c': _w((lambda *s: _rng.normal(s) * 0.05)(1, 640)), 'w_mod': _w((lambda *s: _rng.normal(s) * 0.05)(640, 6 * 640) * 640 ** (-0.5))}

def reference(A_x, A_c_kv, A_w_q, A_w_uk, A_w_uv, A_w_o, B_x, B_w1, B_w2, B_w3, B_w4, c, w_mod):

    def _A_ref(x, c_kv, w_q, w_uk, w_uv, w_o):
        B, Sq, M = (x.shape[0], x.shape[1], x.shape[2])
        Sk = c_kv.shape[1]
        H, D = (w_q.shape[1], w_q.shape[2])
        q = jnp.einsum('bqm,mhd->bhqd', x, w_q)
        k = jnp.einsum('bkc,chd->bhkd', c_kv, w_uk)
        v = jnp.einsum('bkc,chd->bhkd', c_kv, w_uv)
        scores = jnp.einsum('bhqd,bhkd->bhqk', q, k) * D ** (-0.5)
        off = Sk - Sq
        qi = jnp.arange(Sq)[:, None]
        kj = jnp.arange(Sk)[None, :]
        cmask = kj <= qi + off
        scores = jnp.where(cmask[None, None], scores, -1000000000.0)
        p = _softmax(scores, axis=-1)
        ctx = jnp.einsum('bhqk,bhkd->bhqd', p, v)
        return jnp.einsum('bhqd,hdm->bqm', ctx, w_o)

    def _B_ref(x, w1, w2, w3, w4):
        B, S, D = x.shape
        h = _gelu(_layernorm(x, axis=-1) @ w1)
        c = D // 4
        g0 = jnp.pad(h[:, :, 0 * c:1 * c], ((0, 0), (1, 0), (0, 0)))[:, :S, :]
        g1 = jnp.pad(h[:, :, 1 * c:2 * c], ((0, 0), (0, 1), (0, 0)))[:, 1:, :]
        g2 = jnp.pad(h[:, :, 2 * c:3 * c], ((0, 0), (2, 0), (0, 0)))[:, :S, :]
        g3 = jnp.pad(h[:, :, 3 * c:], ((0, 0), (0, 2), (0, 0)))[:, 2:, :]
        hs = jnp.concatenate([g0, g1, g2, g3], axis=-1) @ w2
        x1 = x + hs
        h2 = _gelu(_layernorm(x1, axis=-1) @ w3) @ w4
        return x1 + h2
    x = A_x
    mod = (_silu(c) @ w_mod).reshape(c.shape[0], 6, 1, -1)
    sa, ca, ga, sb, cb, gb = (mod[:, 0].copy(), mod[:, 1].copy(), mod[:, 2].copy(), mod[:, 3].copy(), mod[:, 4].copy(), mod[:, 5].copy())
    h = _layernorm(x, axis=-1) * (1 + ca) + sa
    x = x + ga * _A_ref(h, A_c_kv, A_w_q, A_w_uk, A_w_uv, A_w_o)
    h = _layernorm(x, axis=-1) * (1 + cb) + sb
    x = x + gb * _B_ref(h, B_w1, B_w2, B_w3, B_w4)
    return x
```

```python
import functools
import math

import jax
import jax.numpy as jnp
from jax import lax
import jax.experimental.pallas as pl
import jax.experimental.pallas.tpu as pltpu

F32 = jnp.float32
BF16 = jnp.bfloat16
EPS = 1e-5
NEG = -1e30
TQ = 256
TR = 256
PAD = 8


def _ln(x):
    m = jnp.mean(x, axis=-1, keepdims=True)
    xc = x - m
    v = jnp.mean(xc * xc, axis=-1, keepdims=True)
    return xc * lax.rsqrt(v + EPS)


def _gelu(x):
    c = math.sqrt(2.0 / math.pi)
    return 0.5 * x * (1.0 + jnp.tanh(c * (x + 0.044715 * (x * x * x))))


def _dot(a, b):
    return jnp.dot(a, b, preferred_element_type=F32)


def _dot_nt(a, b):
    return lax.dot_general(a, b, (((1,), (1,)), ((), ())), preferred_element_type=F32)


def _unpack_pair(u):
    lo = pltpu.bitcast(u << 16, F32).astype(BF16)
    hi = pltpu.bitcast(u & jnp.uint32(0xFFFF0000), F32).astype(BF16)
    return jnp.concatenate([lo, hi], axis=1)


def _kernel(x_ref, ckv_ref, wq_ref, wk_ref, wv_ref, wo_ref, w1_ref, w2_ref, w3_ref, w4_ref,
            c_ref, wmod_ref, o_ref,
            mod_ref, h_ref, q_ref, k_ref, v_ref, ctx_ref, x1_ref, h2_ref, hh_ref,
            wq_buf, wk_buf, wv_buf, wsem,
            *, S, M, Dc, H, D):
    g = pl.program_id(0)
    npairs = H // 2
    nchunks = S // TR

    slot = g % 2

    def w_copies(pair, sl):
        return [
            pltpu.make_async_copy(src.bitcast(jnp.uint32).at[:, pair, :], dst.at[sl], wsem.at[j, sl])
            for j, (src, dst) in enumerate(((wq_ref, wq_buf), (wk_ref, wk_buf), (wv_ref, wv_buf)))
        ]

    @pl.when(g == 0)
    def _prologue():
        for cp in w_copies(0, 0):
            cp.start()
        c = c_ref[...].astype(F32)
        sc = c * (1.0 / (1.0 + jnp.exp(-c)))
        sc8 = jnp.broadcast_to(sc, (8, M)).astype(BF16)
        mod_ref[...] = _dot(sc8, wmod_ref[...])
        sa = mod_ref[0:1, 0:M]
        ca = mod_ref[0:1, M:2 * M]

        def body(i, _):
            r = pl.multiple_of(i * TR, TR)
            x = x_ref[pl.ds(r, TR), :].astype(F32)
            h_ref[pl.ds(r, TR), :] = (_ln(x) * (1.0 + ca) + sa).astype(BF16)
            return 0
        lax.fori_loop(0, nchunks, body, 0)

    qscale = (D ** -0.5) * math.log2(math.e)
    for cp in w_copies(g, slot):
        cp.wait()

    @pl.when(g + 1 < npairs)
    def _():
        for cp in w_copies(g + 1, 1 - slot):
            cp.start()

    wq = _unpack_pair(wq_buf[slot])
    wk = _unpack_pair(wk_buf[slot])
    wv = _unpack_pair(wv_buf[slot])
    PR = 512
    for i in range(S // PR):
        rows = slice(i * PR, (i + 1) * PR)
        q_ref[rows, :] = (_dot(h_ref[rows, :], wq) * qscale).astype(BF16)
        k_ref[rows, :] = _dot(ckv_ref[rows, :], wk).astype(BF16)
        v_ref[rows, :] = _dot(ckv_ref[rows, :], wv).astype(BF16)

    row = lax.broadcasted_iota(jnp.int32, (TQ, TQ), 0)
    col = lax.broadcasted_iota(jnp.int32, (TQ, TQ), 1)
    tri = col <= row
    for hh in range(2):
        lanes = slice(hh * D, (hh + 1) * D)
        for i in range(S // TQ):
            r0 = i * TQ
            q = q_ref[r0:r0 + TQ, lanes]
            sd = jnp.where(tri, _dot_nt(q, k_ref[r0:r0 + TQ, lanes]), NEG)
            m = jnp.max(sd, axis=-1, keepdims=True)
            if i > 0:
                so = _dot_nt(q, k_ref[0:r0, lanes])
                m = jnp.maximum(m, jnp.max(so, axis=-1, keepdims=True))
            pd = jnp.exp2(sd - m)
            l = jnp.sum(pd, axis=-1, keepdims=True)
            acc = _dot(pd.astype(BF16), v_ref[r0:r0 + TQ, lanes])
            if i > 0:
                po = jnp.exp2(so - m)
                l = l + jnp.sum(po, axis=-1, keepdims=True)
                acc = acc + _dot(po.astype(BF16), v_ref[0:r0, lanes])
            ctx_ref[g, r0:r0 + TQ, lanes] = (acc * (1.0 / l)).astype(BF16)

    @pl.when(g == npairs - 1)
    def _epilogue():
        ga = mod_ref[0:1, 2 * M:3 * M]
        sb = mod_ref[0:1, 3 * M:4 * M]
        cb = mod_ref[0:1, 4 * M:5 * M]
        gb = mod_ref[0:1, 5 * M:6 * M]
        hh_ref[0:PAD, :] = jnp.zeros((PAD, M), F32)
        hh_ref[PAD + S:PAD + S + PAD, :] = jnp.zeros((PAD, M), F32)

        def phase1(i, _):
            r = pl.multiple_of(i * TR, TR)
            attn = _dot(ctx_ref[0, pl.ds(r, TR), :], wo_ref[0:2 * D, :])
            for p in range(1, npairs):
                attn = attn + _dot(ctx_ref[p, pl.ds(r, TR), :], wo_ref[p * 2 * D:(p + 1) * 2 * D, :])
            x1 = x_ref[pl.ds(r, TR), :].astype(F32) + ga * attn
            x1_ref[pl.ds(r, TR), :] = x1
            h2 = _ln(x1) * (1.0 + cb) + sb
            h2_ref[pl.ds(r, TR), :] = h2
            hh_ref[pl.ds(PAD + r, TR), :] = _gelu(_dot(_ln(h2).astype(BF16), w1_ref[...]))
            return 0
        lax.fori_loop(0, nchunks, phase1, 0)

        cgrp = M // 4
        lane = lax.broadcasted_iota(jnp.int32, (TR, M), 1)

        for i in range(nchunks):
            r = i * TR
            g0 = hh_ref[PAD + r - 1:PAD + r - 1 + TR, :]
            g1 = hh_ref[PAD + r + 1:PAD + r + 1 + TR, :]
            g2 = hh_ref[PAD + r - 2:PAD + r - 2 + TR, :]
            g3 = hh_ref[PAD + r + 2:PAD + r + 2 + TR, :]
            sh = jnp.where(lane < cgrp, g0,
                           jnp.where(lane < 2 * cgrp, g1,
                                     jnp.where(lane < 3 * cgrp, g2, g3)))
            y1 = h2_ref[r:r + TR, :] + _dot(sh.astype(BF16), w2_ref[...])
            t = _gelu(_dot_nt(_ln(y1).astype(BF16), w3_ref[...]))
            y2 = y1 + _dot(t.astype(BF16), w4_ref[...])
            o_ref[r:r + TR, :] = (x1_ref[r:r + TR, :] + gb * y2).astype(o_ref.dtype)


@jax.jit
def pallas_adaLN_cond__compressed_kv_cla__mixer_s_mlp__prompt_kernel(
    A_x, A_c_kv, A_w_q, A_w_uk, A_w_uv, A_w_o, B_x, B_w1, B_w2, B_w3, B_w4, c, w_mod,
):
    del B_x
    _, S, M = A_x.shape
    Dc = A_c_kv.shape[2]
    H, D = A_w_q.shape[1], A_w_q.shape[2]
    x = A_x.reshape(S, M)
    ckv = A_c_kv.reshape(S, Dc)
    wq, wk, wv = A_w_q, A_w_uk, A_w_uv
    w3t = B_w3.T
    wo = A_w_o.reshape(H * D, M)
    ins = (x, ckv, wq, wk, wv, wo, B_w1, B_w2, w3t, B_w4, c, w_mod)

    def full(a):
        return pl.BlockSpec(a.shape, lambda g: (0,) * a.ndim, pipeline_mode=pl.Buffered(1))

    out = pl.pallas_call(
        functools.partial(_kernel, S=S, M=M, Dc=Dc, H=H, D=D),
        grid=(H // 2,),
        in_specs=[pl.BlockSpec(memory_space=pl.ANY) if a.ndim == 3 else full(a) for a in ins],
        out_specs=pl.BlockSpec((S, M), lambda g: (0, 0)),
        out_shape=jax.ShapeDtypeStruct((S, M), A_x.dtype),
        scratch_shapes=[
            pltpu.VMEM((8, 6 * M), F32),
            pltpu.VMEM((S, M), BF16),
            pltpu.VMEM((S, 2 * D), BF16),
            pltpu.VMEM((S, 2 * D), BF16),
            pltpu.VMEM((S, 2 * D), BF16),
            pltpu.VMEM((H // 2, S, 2 * D), BF16),
            pltpu.VMEM((S, M), F32),
            pltpu.VMEM((S, M), F32),
            pltpu.VMEM((S + 2 * PAD, M), F32),
            pltpu.VMEM((2, M, D), jnp.uint32),
            pltpu.VMEM((2, Dc, D), jnp.uint32),
            pltpu.VMEM((2, Dc, D), jnp.uint32),
            pltpu.SemaphoreType.DMA((3, 2)),
        ],
        compiler_params=pltpu.CompilerParams(
            dimension_semantics=("arbitrary",),
            vmem_limit_bytes=110 * 1024 * 1024,
        ),
    )(*ins)
    return out.reshape(1, S, M)
```

```python
import functools
import math

import jax
import jax.numpy as jnp
from jax import lax
import jax.experimental.pallas as pl
import jax.experimental.pallas.tpu as pltpu

F32 = jnp.float32
BF16 = jnp.bfloat16
EPS = 1e-5
NEG = -1e30
TQ = 256
TR = 256
PAD = 8


def _ln(x):
    m = jnp.mean(x, axis=-1, keepdims=True)
    xc = x - m
    v = jnp.mean(xc * xc, axis=-1, keepdims=True)
    return xc * lax.rsqrt(v + EPS)


def _gelu(x):
    c = math.sqrt(2.0 / math.pi)
    return 0.5 * x * (1.0 + jnp.tanh(c * (x + 0.044715 * (x * x * x))))


def _dot(a, b):
    return jnp.dot(a, b, preferred_element_type=F32)


def _dot_nt(a, b):
    return lax.dot_general(a, b, (((1,), (1,)), ((), ())), preferred_element_type=F32)


def _unpack_pair(u):
    lo = pltpu.bitcast(u << 16, F32).astype(BF16)
    hi = pltpu.bitcast(u & jnp.uint32(0xFFFF0000), F32).astype(BF16)
    return jnp.concatenate([lo, hi], axis=1)


def _kernel(x_ref, ckv_ref, wq_ref, wk_ref, wv_ref, wo_ref, w1_ref, w2_ref, w3_ref, w4_ref,
            c_ref, wmod_ref, o_ref,
            mod_ref, h_ref, q_ref, k_ref, v_ref, ctx_ref, x1_ref, h2_ref, hh_ref,
            wq_buf, wk_buf, wv_buf, wsem,
            *, S, M, Dc, H, D):
    g = pl.program_id(0)
    npairs = H // 2
    nchunks = S // TR

    slot = g % 2

    def w_copies(pair, sl):
        return [
            pltpu.make_async_copy(src.bitcast(jnp.uint32).at[:, pair, :], dst.at[sl], wsem.at[j, sl])
            for j, (src, dst) in enumerate(((wq_ref, wq_buf), (wk_ref, wk_buf), (wv_ref, wv_buf)))
        ]

    @pl.when(g == 0)
    def _prologue():
        for cp in w_copies(0, 0):
            cp.start()
        c = c_ref[...].astype(F32)
        sc = c * (1.0 / (1.0 + jnp.exp(-c)))
        sc8 = jnp.broadcast_to(sc, (8, M)).astype(BF16)
        mod_ref[...] = _dot(sc8, wmod_ref[...])
        sa = mod_ref[0:1, 0:M]
        ca = mod_ref[0:1, M:2 * M]

        def body(i, _):
            r = pl.multiple_of(i * TR, TR)
            x = x_ref[pl.ds(r, TR), :].astype(F32)
            h_ref[pl.ds(r, TR), :] = (_ln(x) * (1.0 + ca) + sa).astype(BF16)
            return 0
        lax.fori_loop(0, nchunks, body, 0)

    qscale = (D ** -0.5) * math.log2(math.e)
    for cp in w_copies(g, slot):
        cp.wait()

    @pl.when(g + 1 < npairs)
    def _():
        for cp in w_copies(g + 1, 1 - slot):
            cp.start()

    wq = _unpack_pair(wq_buf[slot])
    wk = _unpack_pair(wk_buf[slot])
    wv = _unpack_pair(wv_buf[slot])
    PR = 512
    for i in range(S // PR):
        rows = slice(i * PR, (i + 1) * PR)
        q_ref[rows, :] = (_dot(h_ref[rows, :], wq) * qscale).astype(BF16)
        k_ref[rows, :] = _dot(ckv_ref[rows, :], wk).astype(BF16)
        v_ref[rows, :] = _dot(ckv_ref[rows, :], wv).astype(BF16)

    row = lax.broadcasted_iota(jnp.int32, (TQ, TQ), 0)
    col = lax.broadcasted_iota(jnp.int32, (TQ, TQ), 1)
    tri = col <= row
    for hh in range(2):
        lanes = slice(hh * D, (hh + 1) * D)
        for i in range(S // TQ):
            r0 = i * TQ
            q = q_ref[r0:r0 + TQ, lanes]
            sd = jnp.where(tri, _dot_nt(q, k_ref[r0:r0 + TQ, lanes]), NEG)
            m = jnp.max(sd, axis=-1, keepdims=True)
            if i > 0:
                so = _dot_nt(q, k_ref[0:r0, lanes])
                m = jnp.maximum(m, jnp.max(so, axis=-1, keepdims=True))
            pd = jnp.exp2(sd - m)
            l = jnp.sum(pd, axis=-1, keepdims=True)
            acc = _dot(pd.astype(BF16), v_ref[r0:r0 + TQ, lanes])
            if i > 0:
                po = jnp.exp2(so - m)
                l = l + jnp.sum(po, axis=-1, keepdims=True)
                acc = acc + _dot(po.astype(BF16), v_ref[0:r0, lanes])
            ctx_ref[g, r0:r0 + TQ, lanes] = (acc * (1.0 / l)).astype(BF16)

    @pl.when(g == npairs - 1)
    def _epilogue():
        ga = mod_ref[0:1, 2 * M:3 * M]
        sb = mod_ref[0:1, 3 * M:4 * M]
        cb = mod_ref[0:1, 4 * M:5 * M]
        gb = mod_ref[0:1, 5 * M:6 * M]
        hh_ref[0:PAD, :] = jnp.zeros((PAD, M), F32)
        hh_ref[PAD + S:PAD + S + PAD, :] = jnp.zeros((PAD, M), F32)

        def phase1(i, _):
            r = pl.multiple_of(i * TR, TR)
            attn = _dot(ctx_ref[0, pl.ds(r, TR), :], wo_ref[0:2 * D, :])
            for p in range(1, npairs):
                attn = attn + _dot(ctx_ref[p, pl.ds(r, TR), :], wo_ref[p * 2 * D:(p + 1) * 2 * D, :])
            x1 = x_ref[pl.ds(r, TR), :].astype(F32) + ga * attn
            x1_ref[pl.ds(r, TR), :] = x1
            h2 = _ln(x1) * (1.0 + cb) + sb
            h2_ref[pl.ds(r, TR), :] = h2
            hh_ref[pl.ds(PAD + r, TR), :] = _gelu(_dot(_ln(h2).astype(BF16), w1_ref[...]))
            return 0
        lax.fori_loop(0, nchunks, phase1, 0)

        cgrp = M // 4
        lane = lax.broadcasted_iota(jnp.int32, (TR, M), 1)

        def phase2(i, _):
            r = pl.multiple_of(i * TR, TR)
            win = hh_ref[pl.ds(r, TR + 2 * PAD), :]
            g0 = win[PAD - 1:PAD - 1 + TR, :]
            g1 = win[PAD + 1:PAD + 1 + TR, :]
            g2 = win[PAD - 2:PAD - 2 + TR, :]
            g3 = win[PAD + 2:PAD + 2 + TR, :]
            sh = jnp.where(lane < cgrp, g0,
                           jnp.where(lane < 2 * cgrp, g1,
                                     jnp.where(lane < 3 * cgrp, g2, g3)))
            y1 = h2_ref[pl.ds(r, TR), :] + _dot(sh.astype(BF16), w2_ref[...])
            t = _gelu(_dot_nt(_ln(y1).astype(BF16), w3_ref[...]))
            y2 = y1 + _dot(t.astype(BF16), w4_ref[...])
            o_ref[pl.ds(r, TR), :] = (x1_ref[pl.ds(r, TR), :] + gb * y2).astype(o_ref.dtype)
            return 0
        lax.fori_loop(0, nchunks, phase2, 0)


@jax.jit
def pallas_adaLN_cond__compressed_kv_cla__mixer_s_mlp__prompt_kernel(
    A_x, A_c_kv, A_w_q, A_w_uk, A_w_uv, A_w_o, B_x, B_w1, B_w2, B_w3, B_w4, c, w_mod,
):
    del B_x
    _, S, M = A_x.shape
    Dc = A_c_kv.shape[2]
    H, D = A_w_q.shape[1], A_w_q.shape[2]
    x = A_x.reshape(S, M)
    ckv = A_c_kv.reshape(S, Dc)
    wq, wk, wv = A_w_q, A_w_uk, A_w_uv
    w3t = B_w3.T
    wo = A_w_o.reshape(H * D, M)
    ins = (x, ckv, wq, wk, wv, wo, B_w1, B_w2, w3t, B_w4, c, w_mod)

    def full(a):
        return pl.BlockSpec(a.shape, lambda g: (0,) * a.ndim, pipeline_mode=pl.Buffered(1))

    out = pl.pallas_call(
        functools.partial(_kernel, S=S, M=M, Dc=Dc, H=H, D=D),
        grid=(H // 2,),
        in_specs=[pl.BlockSpec(memory_space=pl.ANY) if a.ndim == 3 else full(a) for a in ins],
        out_specs=pl.BlockSpec((S, M), lambda g: (0, 0)),
        out_shape=jax.ShapeDtypeStruct((S, M), A_x.dtype),
        scratch_shapes=[
            pltpu.VMEM((8, 6 * M), F32),
            pltpu.VMEM((S, M), BF16),
            pltpu.VMEM((S, 2 * D), BF16),
            pltpu.VMEM((S, 2 * D), BF16),
            pltpu.VMEM((S, 2 * D), BF16),
            pltpu.VMEM((H // 2, S, 2 * D), BF16),
            pltpu.VMEM((S, M), F32),
            pltpu.VMEM((S, M), F32),
            pltpu.VMEM((S + 2 * PAD, M), F32),
            pltpu.VMEM((2, M, D), jnp.uint32),
            pltpu.VMEM((2, Dc, D), jnp.uint32),
            pltpu.VMEM((2, Dc, D), jnp.uint32),
            pltpu.SemaphoreType.DMA((3, 2)),
        ],
        compiler_params=pltpu.CompilerParams(
            dimension_semantics=("arbitrary",),
            vmem_limit_bytes=110 * 1024 * 1024,
        ),
    )(*ins)
    return out.reshape(1, S, M)
```

```python
import functools
import math

import jax
import jax.numpy as jnp
from jax import lax
import jax.experimental.pallas as pl
import jax.experimental.pallas.tpu as pltpu

SKIP = ''
VAR = 'y23'
GR = 512
SC = 128
HALO = 16
F32 = jnp.float32
BF16 = jnp.bfloat16
U32 = jnp.uint32
EPS = 1e-5
NEG = -1e30
T = 128
TR = 256
PAD = 8


def _ln(x):
    m = jnp.mean(x, axis=-1, keepdims=True)
    xc = x - m
    v = jnp.mean(xc * xc, axis=-1, keepdims=True)
    return xc * lax.rsqrt(v + EPS)


def _gelu(x):
    c = math.sqrt(2.0 / math.pi)
    return 0.5 * x * (1.0 + jnp.tanh(c * (x + 0.044715 * (x * x * x))))


def _dot(a, b):
    return jnp.dot(a, b, preferred_element_type=F32)


def _dot_nt(a, b):
    return lax.dot_general(a, b, (((1,), (1,)), ((), ())), preferred_element_type=F32)


def _recip(l):
    r = pl.reciprocal(l, approx=True)
    return r * (2.0 - l * r)


def _unpack_pair(u):
    lo = pltpu.bitcast(u << 16, F32).astype(BF16)
    hi = pltpu.bitcast(u & jnp.uint32(0xFFFF0000), F32).astype(BF16)
    return jnp.concatenate([lo, hi], axis=1)


def _softmax_rows(s, tri):
    n = s.shape[1]
    sd = jnp.where(tri, s[:, n - T:], NEG)
    s = sd if n == T else jnp.concatenate([s[:, :n - T], sd], axis=1)
    m = jnp.max(s, axis=-1, keepdims=True)
    p = jnp.exp2(s - m)
    l = jnp.sum(p, axis=-1, keepdims=True)
    return p.astype(BF16), l


def _schedule(var, nblk):
    ops = []
    if var[0] == 'a':
        od = int(var[1])
        for i in range(4):
            ops.append(('K', i * 512, 512))
        for i in reversed(range(4)):
            ops.append(('Q', i * 512, 512))
        for i in range(4):
            ops.append(('V', i * 512, 512))
        jobs = [(hh, i) for i in reversed(range(nblk)) for hh in range(2)]
        oq = []
        for t in range(len(jobs) + 1):
            if t < len(jobs):
                ops.append(('S',) + jobs[t])
            if t >= 1:
                ops.append(('P',) + jobs[t - 1])
                if jobs[t - 1][0] == 1:
                    oq.append((t + od, jobs[t - 1][1]))
            while oq and oq[0][0] <= t:
                ops.append(('O', oq.pop(0)[1]))
        ops += [('O', i) for _, i in oq]
    elif var[0] == 'u':
        la = int(var[1])
        for i in range(la):
            ops += [('K', i * T, T), ('Q', i * T, T), ('V', i * T, T)]
        for i in range(nblk):
            j = i + la
            ops.append(('S', 0, i))
            if j < nblk:
                ops.append(('K', j * T, T))
            if i > 0:
                ops.append(('P', 1, i - 1))
            ops.append(('S', 1, i))
            if j < nblk:
                ops.append(('Q', j * T, T))
            if i > 1:
                ops.append(('O', i - 2))
            ops.append(('P', 0, i))
            if j < nblk:
                ops.append(('V', j * T, T))
        ops += [('O', nblk - 2), ('P', 1, nblk - 1), ('O', nblk - 1)]
    elif var[0] == 'w':
        od = int(var[1])
        ops += [('K', 0, T), ('Q', 0, T), ('V', 0, T)]
        for i in range(nblk):
            j = i + 1
            ops.append(('S', 0, i))
            if j < nblk:
                ops.append(('K', j * T, T))
            else:
                ops.append(('O', i - od))
            if i > 0:
                ops.append(('P', 1, i - 1))
            ops.append(('S', 1, i))
            if j < nblk:
                ops.append(('Q', j * T, T))
                if i >= od:
                    ops.append(('O', i - od))
            else:
                ops.append(('O', i - od + 1))
            ops.append(('P', 0, i))
            if j < nblk:
                ops.append(('V', j * T, T))
        rest = list(range(nblk - od + 1, nblk))
        k = max(0, len(rest) - 2)
        ops += [('O', i) for i in rest[:k]]
        ops.append(('P', 1, nblk - 1))
        ops += [('O', i) for i in rest[k:]]
    elif var[0] == 'x':
        nres = int(var[1])
        order = [0] + list(range(nres + 1, nblk)) + list(range(nres, 0, -1))
        kv_done = 0
        fill = []
        def need_kv(upto):
            nonlocal kv_done
            out = []
            while kv_done <= upto:
                out.append(kv_done)
                kv_done += 1
            return out
        ops += [('K', 0, T), ('Q', 0, T), ('V', 0, T)]
        kv_done = 1
        done = []
        for t, i in enumerate(order):
            nxt = order[t + 1] if t + 1 < len(order) else None
            newkv = need_kv(nxt) if nxt is not None else []
            ops.append(('S', 0, i))
            ops += [('K', j * T, T) for j in newkv]
            if t > 0:
                ops.append(('P', 1, order[t - 1]))
            ops.append(('S', 1, i))
            if nxt is not None:
                ops.append(('Q', nxt * T, T))
            if t >= 2:
                ops.append(('O', order[t - 2]))
            ops.append(('P', 0, i))
            ops += [('V', j * T, T) for j in newkv]
        ops += [('O', order[-2]), ('P', 1, order[-1]), ('O', order[-1])]
    elif var[0] == 'y':
        nres, od = int(var[1]), int(var[2])
        order = [0] + list(range(nres + 1, nblk)) + list(range(nres, 0, -1))
        ops += [('K', 0, T), ('Q', 0, T), ('V', 0, T)]
        kv_done = 1
        oq = []
        n = len(order)
        for t, i in enumerate(order):
            nxt = order[t + 1] if t + 1 < n else None
            newkv = list(range(kv_done, nxt + 1)) if nxt is not None else []
            kv_done = max(kv_done, (nxt + 1) if nxt is not None else 0)
            ops.append(('S', 0, i))
            ops += [('K', j * T, T) for j in newkv]
            if not newkv and len(oq) > 1:
                ops.append(('O', oq.pop(0)))
            if t > 0:
                ops.append(('P', 1, order[t - 1]))
                oq.append(order[t - 1])
            ops.append(('S', 1, i))
            if nxt is not None:
                ops.append(('Q', nxt * T, T))
            if len(oq) >= od or (not newkv and len(oq) > 1):
                ops.append(('O', oq.pop(0)))
            ops.append(('P', 0, i))
            ops += [('V', j * T, T) for j in newkv]
        ops.append(('P', 1, order[-1]))
        ops += [('O', i) for i in oq] + [('O', order[-1])]
    elif var[0] == 'v':
        ops += [('K', 0, 2 * T), ('Q', 0, 2 * T), ('V', 0, 2 * T)]
        for i in range(nblk):
            j = (i // 2 + 1) * 2
            ops.append(('S', 0, i))
            if j < nblk and i % 2 == 0:
                ops.append(('K', j * T, 2 * T))
            if j < nblk and i % 2 == 1:
                ops.append(('V', j * T, 2 * T))
            if i > 0:
                ops.append(('P', 1, i - 1))
            ops.append(('S', 1, i))
            if j < nblk and i % 2 == 0:
                ops.append(('Q', j * T, 2 * T))
            if i > 2 and i % 2 == 1:
                ops.append(('O', i - 3, i - 2))
            ops.append(('P', 0, i))
        ops += [('O', nblk - 2), ('P', 1, nblk - 1), ('O', nblk - 1)]
    return ops


def _kernel(x_hbm, ckv_hbm, wq_hbm, wk_hbm, wv_hbm, wo_hbm, w1_hbm, w2_hbm, w3_hbm, w4_hbm,
            c_hbm, wmod_hbm, o_hbm,
            x_ref, ckv_ref, w1_ref, w2_ref, w3_ref, w4_ref, c_ref, wmod_ref,
            wq_buf, wk_buf, wv_buf, wo_buf,
            mod_ref, h_ref, q_ref, k_ref, v_ref, acc_ref, base_ref, hh_ref, o_buf,
            wsem, isem, osem,
            *, S, M, Dc, H, D):
    g = pl.program_id(0)
    npairs = H // 2
    nchunks = S // TR
    nblk = S // T
    slot = g % 2

    def w_copies(pair, sl):
        cps = [
            pltpu.make_async_copy(src.bitcast(U32).at[:, pair, :], dst.at[sl], wsem.at[j, sl])
            for j, (src, dst) in enumerate(((wk_hbm, wk_buf), (wv_hbm, wv_buf), (wq_hbm, wq_buf)))
        ]
        cps.append(pltpu.make_async_copy(wo_hbm.at[pair], wo_buf.at[sl], wsem.at[3, sl]))
        return cps

    cp_c = pltpu.make_async_copy(c_hbm, c_ref, isem.at[0])
    cp_mod_a = pltpu.make_async_copy(wmod_hbm.at[:, 0:2 * M], wmod_ref.at[:, 0:2 * M], isem.at[1])
    cp_x = pltpu.make_async_copy(x_hbm, x_ref.at[0:S, :], isem.at[2])
    cp_ckv = pltpu.make_async_copy(ckv_hbm, ckv_ref, isem.at[3])
    late = [
        pltpu.make_async_copy(wmod_hbm.at[:, 2 * M:6 * M], wmod_ref.at[:, 2 * M:6 * M], isem.at[4]),
        pltpu.make_async_copy(w1_hbm, w1_ref, isem.at[5]),
        pltpu.make_async_copy(w2_hbm, w2_ref, isem.at[6]),
        pltpu.make_async_copy(w3_hbm, w3_ref, isem.at[7]),
        pltpu.make_async_copy(w4_hbm, w4_ref, isem.at[8]),
    ]

    def silu_c():
        c = c_ref[...].astype(F32)
        sc = c * (1.0 / (1.0 + jnp.exp(-c)))
        return jnp.broadcast_to(sc, (8, M)).astype(BF16)

    @pl.when(g == 0)
    def _prologue():
        cp_c.start()
        cp_mod_a.start()
        cp_x.start()
        cp_ckv.start()
        for cp in w_copies(0, 0):
            cp.start()
        acc_ref[...] = jnp.zeros(acc_ref.shape, F32)
        x_ref[S:S + HALO, :] = jnp.zeros((HALO, M), BF16)
        hh_ref[:, 0:PAD, :] = jnp.zeros((M // T, PAD, T), F32)
        cp_c.wait()
        cp_mod_a.wait()
        mod_ref[:, 0:2 * M] = _dot(silu_c(), wmod_ref[:, 0:2 * M])
        sa = mod_ref[0:1, 0:M]
        ca = mod_ref[0:1, M:2 * M]
        cp_x.wait()

        def body(i, _):
            r = pl.multiple_of(i * TR, TR)
            x = x_ref[pl.ds(r, TR), :].astype(F32)
            h_ref[pl.ds(r, TR), :] = (_ln(x) * (1.0 + ca) + sa).astype(BF16)
            return 0
        lax.fori_loop(0, nchunks, body, 0)
        cp_ckv.wait()

    for cp in w_copies(g, slot):
        cp.wait()

    @pl.when(g + 1 < npairs)
    def _():
        for cp in w_copies(g + 1, 1 - slot):
            cp.start()

    @pl.when(g == 1)
    def _():
        for cp in late:
            cp.start()

    qscale = (D ** -0.5) * math.log2(math.e)
    wk = _unpack_pair(wk_buf[slot])
    wv = _unpack_pair(wv_buf[slot])
    wq = _unpack_pair(wq_buf[slot])

    row = lax.broadcasted_iota(jnp.int32, (T, T), 0)
    col = lax.broadcasted_iota(jnp.int32, (T, T), 1)
    tri = col <= row

    def proj(dst, src, w, r0, n, scale=None):
        rows = slice(r0, r0 + n)
        y = _dot(src[rows, :], w)
        if scale is not None:
            y = y * scale
        y = y.astype(BF16)
        for hh in range(2):
            dst[hh, rows, :] = y[:, hh * D:(hh + 1) * D]

    def qk(hh, i):
        r0 = i * T
        n = r0 + T
        return _dot_nt(q_ref[hh, r0:n, :], k_ref[hh, 0:n, :])

    def pv(hh, i, s):
        n = (i + 1) * T
        p, l = _softmax_rows(s, tri)
        acc = _dot(p, v_ref[hh, 0:n, :])
        return (acc * _recip(l)).astype(BF16)

    CW = 0
    if CW:
        def tiles(x):
            return [x[:, j * T:(j + 1) * T] for j in range(x.shape[1] // T)]

        def qk(hh, i):
            r0 = i * T
            n = r0 + T
            q = q_ref[hh, r0:n, :]
            chunks = []
            mrun = None
            for c0 in range(0, n, CW):
                c1 = min(n, c0 + CW)
                s = _dot_nt(q, k_ref[hh, c0:c1, :])
                ts = tiles(s)
                if c1 == n:
                    ts[-1] = jnp.where(tri, ts[-1], NEG)
                for tt in ts:
                    mrun = tt if mrun is None else jnp.maximum(mrun, tt)
                chunks.append(ts)
            return chunks, jnp.max(mrun, axis=-1, keepdims=True)

        def pv(hh, i, sm):
            chunks, m = sm
            lrun = None
            acc = None
            c0 = 0
            for ts in chunks:
                ps = [jnp.exp2(tt - m) for tt in ts]
                for pp in ps:
                    lrun = pp if lrun is None else lrun + pp
                pb = jnp.concatenate([pp.astype(BF16) for pp in ps], axis=1)
                c1 = c0 + len(ts) * T
                d = _dot(pb, v_ref[hh, c0:c1, :])
                acc = d if acc is None else acc + d
                c0 = c1
            l = jnp.sum(lrun, axis=-1, keepdims=True)
            return (acc * _recip(l)).astype(BF16)

    def oproj(r0, ctx):
        rows = slice(r0, r0 + ctx.shape[0])
        acc_ref[rows, :] += _dot(ctx, wo_buf[slot])

    pend = {}
    ctx = {}

    def run(op):
        kind = op[0]
        if kind == 'K':
            proj(k_ref, ckv_ref, wk, op[1], op[2])
        elif kind == 'V':
            proj(v_ref, ckv_ref, wv, op[1], op[2])
        elif kind == 'Q':
            proj(q_ref, h_ref, wq, op[1], op[2], qscale)
        elif kind == 'S':
            pend[op[1:]] = qk(*op[1:])
        elif kind == 'P':
            ctx[op[1:]] = pv(*op[1:], pend.pop(op[1:]))
        elif kind == 'O':
            blks = op[1:]
            c = [jnp.concatenate([ctx.pop((0, i)), ctx.pop((1, i))], axis=1) for i in blks]
            oproj(blks[0] * T, c[0] if len(c) == 1 else jnp.concatenate(c, axis=0))

    for op in _schedule(VAR, nblk):
        run(op)
    assert not pend and not ctx

    @pl.when(g == npairs - 1)
    def _epilogue():
        for cp in late:
            cp.wait()
        mod_ref[:, 2 * M:6 * M] = _dot(silu_c(), wmod_ref[:, 2 * M:6 * M])
        ga = mod_ref[0:1, 2 * M:3 * M]
        sb = mod_ref[0:1, 3 * M:4 * M]
        cb = mod_ref[0:1, 4 * M:5 * M]
        gb = mod_ref[0:1, 5 * M:6 * M]
        nct = M // T
        cgrp = M // 4
        shifts = (-1, 1, -2, 2)
        nsub = GR // SC

        def front(q, _):
            r0 = pl.multiple_of(q * GR, GR)
            keep = {}

            def stage1(k):
                n = SC + (HALO if k == nsub - 1 else 0)
                rows = pl.ds(r0 + k * SC, n)
                x1 = x_ref[rows, :].astype(F32) + ga * acc_ref[rows, :]
                h2 = _ln(x1) * (1.0 + cb) + sb
                keep[k] = (x1[:SC], h2[:SC])
                hh = _gelu(_dot(_ln(h2).astype(BF16), w1_ref[...]))
                if k == nsub - 1:
                    rid = r0 + k * SC + lax.broadcasted_iota(jnp.int32, (n, M), 0)
                    hh = jnp.where(rid < S, hh, 0.0)
                for t in range(nct):
                    hh_ref[t, pl.ds(PAD + r0 + k * SC, n), :] = hh[:, t * T:(t + 1) * T]

            def stage2(k):
                base = PAD + r0 + k * SC
                lane = lax.broadcasted_iota(jnp.int32, (SC, T), 1)
                cols = []
                for t in range(nct):
                    lo, hi = (t * T) // cgrp, (t * T + T - 1) // cgrp
                    v = hh_ref[t, pl.ds(base + shifts[lo], SC), :]
                    if hi != lo:
                        v2 = hh_ref[t, pl.ds(base + shifts[hi], SC), :]
                        v = jnp.where(lane < hi * cgrp - t * T, v, v2)
                    cols.append(v)
                sh = jnp.concatenate(cols, axis=1).astype(BF16)
                x1, h2 = keep.pop(k)
                y1 = h2 + _dot(sh, w2_ref[...])
                rows = pl.ds(r0 + k * SC, SC)
                base_ref[rows, :] = x1 + gb * y1
                h_ref[rows, :] = _ln(y1).astype(BF16)

            lag = 2
            for k in range(nsub + lag):
                if k < nsub:
                    stage1(k)
                if k >= lag:
                    stage2(k - lag)
            return 0
        lax.fori_loop(0, S // GR, front, 0)

        def o_copy(i):
            r = pl.multiple_of(i * TR, TR)
            return pltpu.make_async_copy(o_buf.at[pl.ds(r, TR), :], o_hbm.at[pl.ds(r, TR), :], osem.at[i])

        def back(i, _):
            rows = pl.ds(pl.multiple_of(i * TR, TR), TR)
            t = _gelu(_dot_nt(h_ref[rows, :], w3_ref[...]))
            o_buf[rows, :] = (base_ref[rows, :] + gb * _dot(t.astype(BF16), w4_ref[...])).astype(o_buf.dtype)
            o_copy(i).start()
            return 0
        lax.fori_loop(0, nchunks, back, 0)
        for i in range(nchunks):
            o_copy(i).wait()


@jax.jit
def pallas_adaLN_cond__compressed_kv_cla__mixer_s_mlp__prompt_kernel(
    A_x, A_c_kv, A_w_q, A_w_uk, A_w_uv, A_w_o, B_x, B_w1, B_w2, B_w3, B_w4, c, w_mod,
):
    del B_x
    _, S, M = A_x.shape
    Dc = A_c_kv.shape[2]
    H, D = A_w_q.shape[1], A_w_q.shape[2]
    F = B_w3.shape[1]
    x = A_x.reshape(S, M)
    ckv = A_c_kv.reshape(S, Dc)
    w3t = B_w3.T
    wo = A_w_o.reshape(H // 2, 2 * D, M)
    ins = (x, ckv, A_w_q, A_w_uk, A_w_uv, wo, B_w1, B_w2, w3t, B_w4, c, w_mod)

    out = pl.pallas_call(
        functools.partial(_kernel, S=S, M=M, Dc=Dc, H=H, D=D),
        grid=(H // 2,),
        in_specs=[pl.BlockSpec(memory_space=pl.ANY) for _ in ins],
        out_specs=pl.BlockSpec(memory_space=pl.ANY),
        out_shape=jax.ShapeDtypeStruct((S, M), A_x.dtype),
        scratch_shapes=[
            pltpu.VMEM((S + HALO, M), BF16),
            pltpu.VMEM((S, Dc), BF16),
            pltpu.VMEM((M, M), BF16),
            pltpu.VMEM((M, M), BF16),
            pltpu.VMEM((F, M), BF16),
            pltpu.VMEM((F, M), BF16),
            pltpu.VMEM((1, M), BF16),
            pltpu.VMEM((M, 6 * M), BF16),
            pltpu.VMEM((2, M, D), U32),
            pltpu.VMEM((2, Dc, D), U32),
            pltpu.VMEM((2, Dc, D), U32),
            pltpu.VMEM((2, 2 * D, M), BF16),
            pltpu.VMEM((8, 6 * M), F32),
            pltpu.VMEM((S, M), BF16),
            pltpu.VMEM((2, S, D), BF16),
            pltpu.VMEM((2, S, D), BF16),
            pltpu.VMEM((2, S, D), BF16),
            pltpu.VMEM((S + HALO, M), F32),
            pltpu.VMEM((S, M), F32),
            pltpu.VMEM((M // T, PAD + S + HALO, T), F32),
            pltpu.VMEM((S, M), A_x.dtype),
            pltpu.SemaphoreType.DMA((4, 2)),
            pltpu.SemaphoreType.DMA((9,)),
            pltpu.SemaphoreType.DMA((S // TR,)),
        ],
        compiler_params=pltpu.CompilerParams(
            dimension_semantics=("arbitrary",),
            vmem_limit_bytes=100 * 1024 * 1024,
        ),
    )(*ins)
    return out.reshape(1, S, M)
```

```python
import functools
import math

import jax
import jax.numpy as jnp
from jax import lax
import jax.experimental.pallas as pl
import jax.experimental.pallas.tpu as pltpu

SKIP = ''
VAR = 'y23'
GR = 512
SC = 128
HALO = 16
NEWA = 1
SUMBF = 1
KVM = 0
NEWB = 1
EPRE = 0
ELAST = 1
ELOOP = 'uivjdope'
TPL = 'aKVopbQOq'
PRE = 'KQV'
NRES = 2
ODEL = 3
B1 = 1
B2 = 1
B3 = 1
B4 = 1
PRO = 0
F32 = jnp.float32
BF16 = jnp.bfloat16
U32 = jnp.uint32
EPS = 1e-5
NEG = -1e30
T = 128
TR = 256
PAD = 8


def _ln(x):
    m = jnp.mean(x, axis=-1, keepdims=True)
    xc = x - m
    v = jnp.mean(xc * xc, axis=-1, keepdims=True)
    return xc * lax.rsqrt(v + EPS)


def _gelu(x):
    c = math.sqrt(2.0 / math.pi)
    hx = 0.5 * x
    return hx + hx * jnp.tanh(x * (c + (c * 0.044715) * (x * x)))


def _dot(a, b):
    return jnp.dot(a, b, preferred_element_type=F32)


def _dot_nt(a, b):
    return lax.dot_general(a, b, (((1,), (1,)), ((), ())), preferred_element_type=F32)


def _recip(l):
    r = pl.reciprocal(l, approx=True)
    return r * (2.0 - l * r)


def _unpack_pair(u):
    if NEWA:
        lo = pltpu.bitcast(u << 16, F32)
        hi = pltpu.bitcast(u & jnp.uint32(0xFFFF0000), F32)
        return jnp.concatenate([lo, hi], axis=1).astype(BF16)
    lo = pltpu.bitcast(u << 16, F32).astype(BF16)
    hi = pltpu.bitcast(u & jnp.uint32(0xFFFF0000), F32).astype(BF16)
    return jnp.concatenate([lo, hi], axis=1)


def _softmax_rows(s, tri):
    n = s.shape[1]
    sd = jnp.where(tri, s[:, n - T:], NEG)
    s = sd if n == T else jnp.concatenate([s[:, :n - T], sd], axis=1)
    m = jnp.max(s, axis=-1, keepdims=True)
    p = jnp.exp2(s - m)
    if SUMBF:
        pb = p.astype(BF16)
        return pb, jnp.sum(pb.astype(F32), axis=-1, keepdims=True)
    l = jnp.sum(p, axis=-1, keepdims=True)
    return p.astype(BF16), l


def _schedule(var, nblk):
    order = [0] + list(range(NRES + 1, nblk)) + list(range(NRES, 0, -1))
    ops = [(k, 0, T) for k in PRE]
    kv_done = 1
    oq = []
    n = len(order)
    for t, i in enumerate(order):
        nxt = order[t + 1] if t + 1 < n else None
        newkv = list(range(kv_done, nxt + 1)) if nxt is not None else []
        kv_done = max(kv_done, (nxt + 1) if nxt is not None else 0)
        for ch in TPL:
            if ch == 'a':
                ops.append(('S', 0, i))
            elif ch == 'b':
                ops.append(('S', 1, i))
            elif ch == 'p':
                if t > 0:
                    ops.append(('P', 1, order[t - 1]))
                    oq.append(order[t - 1])
            elif ch == 'q':
                ops.append(('P', 0, i))
            elif ch in 'KV':
                ops += [(ch, j * T, T) for j in newkv]
            elif ch == 'Q':
                if nxt is not None:
                    ops.append(('Q', nxt * T, T))
            elif ch == 'o':
                if not newkv and len(oq) > 1:
                    ops.append(('O', oq.pop(0)))
            elif ch == 'O':
                if len(oq) >= ODEL or (not newkv and len(oq) > 1):
                    ops.append(('O', oq.pop(0)))
    ops.append(('P', 1, order[-1]))
    ops += [('O', i) for i in oq] + [('O', order[-1])]
    return ops


def _kernel(x_hbm, ckv_hbm, wq_hbm, wk_hbm, wv_hbm, wo_hbm, w1_hbm, w2_hbm, w3_hbm, w4_hbm,
            c_hbm, wmod_hbm, o_hbm,
            x_ref, ckv_ref, w1_ref, w2_ref, w3_ref, w4_ref, c_ref, wmod_ref,
            wq_buf, wk_buf, wv_buf, wo_buf,
            mod_ref, h_ref, q_ref, k_ref, v_ref, acc_ref, base_ref, hh_ref, o_buf,
            wsem, isem, osem,
            *, S, M, Dc, H, D):
    g = pl.program_id(0)
    npairs = H // 2
    nchunks = S // TR
    nblk = S // T
    slot = g % 2

    def w_copies(pair, sl):
        cps = [
            pltpu.make_async_copy(src.bitcast(U32).at[:, pair, :], dst.at[sl], wsem.at[j, sl])
            for j, (src, dst) in enumerate(((wk_hbm, wk_buf), (wv_hbm, wv_buf), (wq_hbm, wq_buf)))
        ]
        cps.append(pltpu.make_async_copy(wo_hbm.at[pair], wo_buf.at[sl], wsem.at[3, sl]))
        return cps

    cp_c = pltpu.make_async_copy(c_hbm, c_ref, isem.at[0])
    cp_mod_a = pltpu.make_async_copy(wmod_hbm.at[:, 0:2 * M], wmod_ref.at[:, 0:2 * M], isem.at[1])

    def cp_x(i):
        rows = pl.ds(pl.multiple_of(i * TR, TR), TR)
        return pltpu.make_async_copy(x_hbm.at[rows, :], x_ref.at[rows, :], osem.at[i])
    cp_ckv = pltpu.make_async_copy(ckv_hbm, ckv_ref, isem.at[3])
    late = [
        pltpu.make_async_copy(wmod_hbm.at[:, 2 * M:6 * M], wmod_ref.at[:, 2 * M:6 * M], isem.at[4]),
        pltpu.make_async_copy(w1_hbm, w1_ref, isem.at[5]),
        pltpu.make_async_copy(w2_hbm, w2_ref, isem.at[6]),
        pltpu.make_async_copy(w3_hbm, w3_ref, isem.at[7]),
        pltpu.make_async_copy(w4_hbm, w4_ref, isem.at[8]),
    ]

    def silu_c():
        c = c_ref[...].astype(F32)
        sc = c * (1.0 / (1.0 + jnp.exp(-c)))
        return jnp.broadcast_to(sc, (8, M)).astype(BF16)

    @pl.when(g == 0)
    @jax.named_scope('prologue')
    def _prologue():
        cp_c.start()
        cp_mod_a.start()
        for i in range(nchunks):
            cp_x(i).start()
        if PRO == 0:
            cp_ckv.start()
            for cp in w_copies(0, 0):
                cp.start()
        if B1:
            def zero(i, _):
                acc_ref[pl.ds(pl.multiple_of(i * T, T), T), :] = jnp.zeros((T, M), F32)
                return 0
            lax.fori_loop(0, nblk, zero, 0)
            acc_ref[S:S + HALO, :] = jnp.zeros((HALO, M), F32)
        else:
            acc_ref[...] = jnp.zeros(acc_ref.shape, F32)
        x_ref[S:S + HALO, :] = jnp.zeros((HALO, M), BF16)
        hh_ref[:, 0:PAD, :] = jnp.zeros((M // T, PAD, T), F32)
        cp_c.wait()
        cp_mod_a.wait()
        if PRO == 1:
            cp_ckv.start()
            for cp in w_copies(0, 0):
                cp.start()
        mod_ref[:, 0:2 * M] = _dot(silu_c(), wmod_ref[:, 0:2 * M])
        sa = mod_ref[0:1, 0:M]
        ca = mod_ref[0:1, M:2 * M]

        def body(i, _):
            cp_x(i).wait()
            if B2:
                sa2 = mod_ref[0:1, 0:M]
                ca1 = 1.0 + mod_ref[0:1, M:2 * M]
                for j in range(TR // T):
                    rows = pl.ds(pl.multiple_of(i * TR + j * T, T), T)
                    h_ref[rows, :] = (_ln(x_ref[rows, :].astype(F32)) * ca1 + sa2).astype(BF16)
                return 0
            r = pl.multiple_of(i * TR, TR)
            x = x_ref[pl.ds(r, TR), :].astype(F32)
            h_ref[pl.ds(r, TR), :] = (_ln(x) * (1.0 + ca) + sa).astype(BF16)
            return 0
        lax.fori_loop(0, nchunks, body, 0)
        cp_ckv.wait()
        if B4:
            for cp in late:
                cp.start()

    with jax.named_scope('body'):
        with jax.named_scope('step_wait'):
            for cp in w_copies(g, slot):
                cp.wait()

        @pl.when(g + 1 < npairs)
        def _():
            for cp in w_copies(g + 1, 1 - slot):
                cp.start()

        if not B4:
            @pl.when(g == 1)
            def _():
                for cp in late:
                    cp.start()

        qscale = (D ** -0.5) * math.log2(math.e)
        wk = _unpack_pair(wk_buf[slot])
        wv = _unpack_pair(wv_buf[slot])
        wq = _unpack_pair(wq_buf[slot])

        row = lax.broadcasted_iota(jnp.int32, (T, T), 0)
        col = lax.broadcasted_iota(jnp.int32, (T, T), 1)
        tri = col <= row

        def proj(dst, src, w, r0, n, scale=None):
            rows = slice(r0, r0 + n)
            y = _dot(src[rows, :], w)
            if scale is not None:
                y = y * scale
            if not NEWB:
                y = y.astype(BF16)
            for hh in range(2):
                dst[hh, rows, :] = y[:, hh * D:(hh + 1) * D].astype(BF16)

        def qk(hh, i):
            r0 = i * T
            n = r0 + T
            return _dot_nt(q_ref[hh, r0:n, :], k_ref[hh, 0:n, :])

        def pv(hh, i, s):
            n = (i + 1) * T
            p, l = _softmax_rows(s, tri)
            acc = _dot(p, v_ref[hh, 0:n, :])
            return (acc * _recip(l)).astype(BF16)

        def oproj(r0, ctx):
            rows = slice(r0, r0 + ctx.shape[0])
            acc_ref[rows, :] += _dot(ctx, wo_buf[slot])

        pend = {}
        ctx = {}

        def run(op):
            kind = op[0]
            if kind == 'K':
                proj(k_ref, ckv_ref, wk, op[1], op[2])
            elif kind == 'V':
                proj(v_ref, ckv_ref, wv, op[1], op[2])
            elif kind == 'Q':
                proj(q_ref, h_ref, wq, op[1], op[2], qscale)
            elif kind == 'S':
                pend[op[1:]] = qk(*op[1:])
            elif kind == 'P':
                ctx[op[1:]] = pv(*op[1:], pend.pop(op[1:]))
            elif kind == 'O':
                blks = op[1:]
                c = [jnp.concatenate([ctx.pop((0, i)), ctx.pop((1, i))], axis=1) for i in blks]
                oproj(blks[0] * T, c[0] if len(c) == 1 else jnp.concatenate(c, axis=0))

        for op in _schedule(VAR, nblk):
            run(op)
        assert not pend and not ctx

    @pl.when(g == npairs - 1)
    @jax.named_scope('epilogue')
    def _epilogue():
        for cp in late:
            cp.wait()
        mod_ref[:, 2 * M:6 * M] = _dot(silu_c(), wmod_ref[:, 2 * M:6 * M])
        ga = mod_ref[0:1, 2 * M:3 * M]
        sb = mod_ref[0:1, 3 * M:4 * M]
        cb = mod_ref[0:1, 4 * M:5 * M]
        gb = mod_ref[0:1, 5 * M:6 * M]
        cb1 = 1.0 + cb
        nct = M // T
        cgrp = M // 4
        shifts = (-1, 1, -2, 2)

        def x1_of(rows):
            return x_ref[rows, :].astype(F32) + ga * acc_ref[rows, :]

        def mix_in(r, n, last):
            rows = pl.ds(r, n)
            h2 = _ln(x1_of(rows)) * (cb1 if B3 else (1.0 + cb)) + sb
            base_ref[rows, :] = h2
            hh = _gelu(_dot(_ln(h2).astype(BF16), w1_ref[...]))
            if last:
                rid = r + lax.broadcasted_iota(jnp.int32, (n, M), 0)
                hh = jnp.where(rid < S, hh, 0.0)
            for t in range(nct):
                hh_ref[t, pl.ds(PAD + r, n), :] = hh[:, t * T:(t + 1) * T]

        def mix_out(r, n):
            lane = lax.broadcasted_iota(jnp.int32, (n, T), 1)
            cols = []
            for t in range(nct):
                lo, hi = (t * T) // cgrp, (t * T + T - 1) // cgrp
                v = hh_ref[t, pl.ds(PAD + r + shifts[lo], n), :]
                if hi != lo:
                    v2 = hh_ref[t, pl.ds(PAD + r + shifts[hi], n), :]
                    v = jnp.where(lane < hi * cgrp - t * T, v, v2)
                cols.append(v)
            sh = jnp.concatenate(cols, axis=1).astype(BF16)
            rows = pl.ds(r, n)
            y1 = base_ref[rows, :] + _dot(sh, w2_ref[...])
            base_ref[rows, :] = x1_of(rows) + gb * y1
            h_ref[rows, :] = _ln(y1).astype(BF16)

        def ffn_up(r, n=TR):
            return _gelu(_dot_nt(h_ref[pl.ds(r, n), :], w3_ref[...])).astype(BF16)

        def ffn_down(r, t):
            rows = pl.ds(r, t.shape[0])
            o_buf[rows, :] = (base_ref[rows, :] + gb * _dot(t, w4_ref[...])).astype(o_buf.dtype)

        def o_copy(i):
            r = pl.multiple_of(i * TR, TR)
            return pltpu.make_async_copy(o_buf.at[pl.ds(r, TR), :], o_hbm.at[pl.ds(r, TR), :], osem.at[i])

        HR = TR // 2
        QR = TR // 4
        if EPRE == 0:
            mix_in(0, HR, False)
            mix_in(HR, HR + HALO, False)
            mix_out(0, HR)
            mix_out(HR, HR)
        elif EPRE == 1:
            mix_in(0, QR, False)
            mix_in(QR, QR, False)
            mix_in(HR, HR + HALO, False)
            mix_out(0, HR)
            mix_out(HR, QR)
            mix_out(HR + QR, QR)
        elif EPRE == 2:
            mix_in(0, QR, False)
            mix_in(QR, QR, False)
            mix_in(2 * QR, QR, False)
            mix_out(0, QR)
            mix_in(3 * QR, QR + HALO, False)
            mix_out(QR, QR)
            mix_out(2 * QR, QR)
            mix_out(3 * QR, QR)

        def body(i, _):
            r = pl.multiple_of(i * TR, TR)
            rn = r + TR
            t = {}
            for ch in ELOOP:
                if ch == 'U':
                    tt = ffn_up(r)
                    t[0], t[1] = tt[:HR], tt[HR:]
                elif ch == 'u':
                    t[0] = ffn_up(r, HR)
                elif ch == 'v':
                    t[1] = ffn_up(r + HR, HR)
                elif ch == 'I':
                    mix_in(rn, TR + HALO, True)
                elif ch == 'i':
                    mix_in(rn, HR, False)
                elif ch == 'j':
                    mix_in(rn + HR, HR + HALO, True)
                elif ch == 'O':
                    mix_out(rn, TR)
                elif ch == 'o':
                    mix_out(rn, HR)
                elif ch == 'p':
                    mix_out(rn + HR, HR)
                elif ch == 'd':
                    ffn_down(r, t[0])
                elif ch == 'e':
                    ffn_down(r + HR, t[1])
            o_copy(i).start()
            return 0
        with jax.named_scope('eloop'):
            lax.fori_loop(0, nchunks - 1, body, 0)
        with jax.named_scope('elast'):
            r = (nchunks - 1) * TR
            if ELAST == 0:
                ffn_down(r, ffn_up(r))
                o_copy(nchunks - 1).start()
                for i in range(nchunks):
                    o_copy(i).wait()
            else:
                tt = ffn_up(r)
                ca = pltpu.make_async_copy(o_buf.at[r:r + HR, :], o_hbm.at[r:r + HR, :], osem.at[nchunks - 1])
                cb_ = pltpu.make_async_copy(o_buf.at[r + HR:r + TR, :], o_hbm.at[r + HR:r + TR, :], isem.at[0])
                ffn_down(r, tt[:HR])
                ca.start()
                ffn_down(r + HR, tt[HR:])
                cb_.start()
                for i in range(nchunks - 1):
                    o_copy(i).wait()
                ca.wait()
                cb_.wait()


@jax.jit
def pallas_adaLN_cond__compressed_kv_cla__mixer_s_mlp__prompt_kernel(
    A_x, A_c_kv, A_w_q, A_w_uk, A_w_uv, A_w_o, B_x, B_w1, B_w2, B_w3, B_w4, c, w_mod,
):
    del B_x
    _, S, M = A_x.shape
    Dc = A_c_kv.shape[2]
    H, D = A_w_q.shape[1], A_w_q.shape[2]
    F = B_w3.shape[1]
    x = A_x.reshape(S, M)
    ckv = A_c_kv.reshape(S, Dc)
    w3t = B_w3.T
    wo = A_w_o.reshape(H // 2, 2 * D, M)
    ins = (x, ckv, A_w_q, A_w_uk, A_w_uv, wo, B_w1, B_w2, w3t, B_w4, c, w_mod)

    out = pl.pallas_call(
        functools.partial(_kernel, S=S, M=M, Dc=Dc, H=H, D=D),
        grid=(H // 2,),
        in_specs=[pl.BlockSpec(memory_space=pl.ANY) for _ in ins],
        out_specs=pl.BlockSpec(memory_space=pl.ANY),
        out_shape=jax.ShapeDtypeStruct((S, M), A_x.dtype),
        scratch_shapes=[
            pltpu.VMEM((S + HALO, M), BF16),
            pltpu.VMEM((S, Dc), BF16),
            pltpu.VMEM((M, M), BF16),
            pltpu.VMEM((M, M), BF16),
            pltpu.VMEM((F, M), BF16),
            pltpu.VMEM((F, M), BF16),
            pltpu.VMEM((1, M), BF16),
            pltpu.VMEM((M, 6 * M), BF16),
            pltpu.VMEM((2, M, D), U32),
            pltpu.VMEM((2, Dc, D), U32),
            pltpu.VMEM((2, Dc, D), U32),
            pltpu.VMEM((2, 2 * D, M), BF16),
            pltpu.VMEM((8, 6 * M), F32),
            pltpu.VMEM((S, M), BF16),
            pltpu.VMEM((2, S, D), BF16),
            pltpu.VMEM((2, S, D), BF16),
            pltpu.VMEM((2, S, D), BF16),
            pltpu.VMEM((S + HALO, M), F32),
            pltpu.VMEM((S + HALO, M), F32),
            pltpu.VMEM((M // T, PAD + S + HALO, T), F32),
            pltpu.VMEM((S, M), A_x.dtype),
            pltpu.SemaphoreType.DMA((4, 2)),
            pltpu.SemaphoreType.DMA((9,)),
            pltpu.SemaphoreType.DMA((S // TR,)),
        ],
        compiler_params=pltpu.CompilerParams(
            dimension_semantics=("arbitrary",),
            vmem_limit_bytes=100 * 1024 * 1024,
        ),
    )(*ins)
    return out.reshape(1, S, M)
```

```python
import functools
import math

import jax
import jax.numpy as jnp
from jax import lax
import jax.experimental.pallas as pl
import jax.experimental.pallas.tpu as pltpu

SKIP = ''
VAR = 'y23'
GR = 512
SC = 128
HALO = 16
NOBC = 1
W3T = 1
ENDW = 1
NEWA = 1
SUMBF = 1
KVM = 0
NEWB = 1
EPRE = 0
ELAST = 1
ELOOP = 'uivjdOe'
TPL = 'aKVopbQOq'
PRE = 'KQV'
NRES = 2
ODEL = 3
B1 = 1
B2 = 1
B3 = 1
B4 = 1
PRO = 0
F32 = jnp.float32
BF16 = jnp.bfloat16
U32 = jnp.uint32
EPS = 1e-5
NEG = -1e30
T = 128
TR = 256
PAD = 8


def _ln(x):
    m = jnp.mean(x, axis=-1, keepdims=True)
    xc = x - m
    v = jnp.mean(xc * xc, axis=-1, keepdims=True)
    return xc * lax.rsqrt(v + EPS)


def _gelu(x):
    c = math.sqrt(2.0 / math.pi)
    hx = 0.5 * x
    return hx + hx * jnp.tanh(x * (c + (c * 0.044715) * (x * x)))


def _dot(a, b):
    return jnp.dot(a, b, preferred_element_type=F32)


def _dot_nt(a, b):
    return lax.dot_general(a, b, (((1,), (1,)), ((), ())), preferred_element_type=F32)


def _recip(l):
    r = pl.reciprocal(l, approx=True)
    return r * (2.0 - l * r)


def _unpack_pair(u):
    if NEWA:
        lo = pltpu.bitcast(u << 16, F32)
        hi = pltpu.bitcast(u & jnp.uint32(0xFFFF0000), F32)
        return jnp.concatenate([lo, hi], axis=1).astype(BF16)
    lo = pltpu.bitcast(u << 16, F32).astype(BF16)
    hi = pltpu.bitcast(u & jnp.uint32(0xFFFF0000), F32).astype(BF16)
    return jnp.concatenate([lo, hi], axis=1)


def _softmax_rows(s, tri):
    n = s.shape[1]
    sd = jnp.where(tri, s[:, n - T:], NEG)
    s = sd if n == T else jnp.concatenate([s[:, :n - T], sd], axis=1)
    m = jnp.max(s, axis=-1, keepdims=True)
    p = jnp.exp2(s - m)
    if SUMBF:
        pb = p.astype(BF16)
        return pb, jnp.sum(pb.astype(F32), axis=-1, keepdims=True)
    l = jnp.sum(p, axis=-1, keepdims=True)
    return p.astype(BF16), l


def _schedule(var, nblk):
    order = [0] + list(range(NRES + 1, nblk)) + list(range(NRES, 0, -1))
    ops = [(k, 0, T) for k in PRE]
    kv_done = 1
    oq = []
    n = len(order)
    for t, i in enumerate(order):
        nxt = order[t + 1] if t + 1 < n else None
        newkv = list(range(kv_done, nxt + 1)) if nxt is not None else []
        kv_done = max(kv_done, (nxt + 1) if nxt is not None else 0)
        for ch in TPL:
            if ch == 'a':
                ops.append(('S', 0, i))
            elif ch == 'b':
                ops.append(('S', 1, i))
            elif ch == 'p':
                if t > 0:
                    ops.append(('P', 1, order[t - 1]))
                    oq.append(order[t - 1])
            elif ch == 'q':
                ops.append(('P', 0, i))
            elif ch in 'KV':
                ops += [(ch, j * T, T) for j in newkv]
            elif ch == 'Q':
                if nxt is not None:
                    ops.append(('Q', nxt * T, T))
            elif ch == 'o':
                if not newkv and len(oq) > 1:
                    ops.append(('O', oq.pop(0)))
            elif ch == 'O':
                if len(oq) >= ODEL or (not newkv and len(oq) > 1):
                    ops.append(('O', oq.pop(0)))
    ops.append(('P', 1, order[-1]))
    ops += [('O', i) for i in oq] + [('O', order[-1])]
    return ops


def _kernel(x_hbm, ckv_hbm, wq_hbm, wk_hbm, wv_hbm, wo_hbm, w1_hbm, w2_hbm, w3_hbm, w4_hbm,
            c_hbm, wmod_hbm, o_hbm,
            x_ref, ckv_ref, w1_ref, w2_ref, w3_ref, w4_ref, c_ref, wmod_ref,
            wq_buf, wk_buf, wv_buf, wo_buf,
            mod_ref, h_ref, q_ref, k_ref, v_ref, acc_ref, base_ref, hh_ref, o_buf,
            wsem, isem, osem,
            *, S, M, Dc, H, D):
    g = pl.program_id(0)
    npairs = H // 2
    nchunks = S // TR
    nblk = S // T
    slot = g % 2

    def w_copies(pair, sl):
        cps = [
            pltpu.make_async_copy(src.bitcast(U32).at[:, pair, :], dst.at[sl], wsem.at[j, sl])
            for j, (src, dst) in enumerate(((wk_hbm, wk_buf), (wv_hbm, wv_buf), (wq_hbm, wq_buf)))
        ]
        cps.append(pltpu.make_async_copy(wo_hbm.at[pair], wo_buf.at[sl], wsem.at[3, sl]))
        return cps

    cp_c = pltpu.make_async_copy(c_hbm, c_ref, isem.at[0])
    cp_mod_a = pltpu.make_async_copy(wmod_hbm.at[:, 0:2 * M], wmod_ref.at[:, 0:2 * M], isem.at[1])

    def cp_x(i):
        rows = pl.ds(pl.multiple_of(i * TR, TR), TR)
        return pltpu.make_async_copy(x_hbm.at[rows, :], x_ref.at[rows, :], osem.at[i])
    cp_ckv = pltpu.make_async_copy(ckv_hbm, ckv_ref, isem.at[3])
    late = [
        pltpu.make_async_copy(wmod_hbm.at[:, 2 * M:6 * M], wmod_ref.at[:, 2 * M:6 * M], isem.at[4]),
        pltpu.make_async_copy(w1_hbm, w1_ref, isem.at[5]),
        pltpu.make_async_copy(w2_hbm, w2_ref, isem.at[6]),
        pltpu.make_async_copy(w3_hbm, w3_ref, isem.at[7]),
        pltpu.make_async_copy(w4_hbm, w4_ref, isem.at[8]),
    ]

    def silu_c():
        c = c_ref[...].astype(F32)
        sc = c * (1.0 / (1.0 + jnp.exp(-c)))
        return jnp.broadcast_to(sc, (8, M)).astype(BF16)

    @pl.when(g == 0)
    @jax.named_scope('prologue')
    def _prologue():
        cp_c.start()
        cp_mod_a.start()
        for i in range(nchunks):
            cp_x(i).start()
        if PRO == 0:
            cp_ckv.start()
            for cp in w_copies(0, 0):
                cp.start()
        if B1:
            def zero(i, _):
                acc_ref[pl.ds(pl.multiple_of(i * T, T), T), :] = jnp.zeros((T, M), F32)
                return 0
            lax.fori_loop(0, nblk, zero, 0)
            acc_ref[S:S + HALO, :] = jnp.zeros((HALO, M), F32)
        else:
            acc_ref[...] = jnp.zeros(acc_ref.shape, F32)
        x_ref[S:S + HALO, :] = jnp.zeros((HALO, M), BF16)
        hh_ref[:, 0:PAD, :] = jnp.zeros((M // T, PAD, T), F32)
        cp_c.wait()
        cp_mod_a.wait()
        if PRO == 1:
            cp_ckv.start()
            for cp in w_copies(0, 0):
                cp.start()
        mod_ref[:, 0:2 * M] = _dot(silu_c(), wmod_ref[:, 0:2 * M])
        sa = mod_ref[0:1, 0:M]
        ca = mod_ref[0:1, M:2 * M]

        def body(i, _):
            cp_x(i).wait()
            if B2:
                sa2 = mod_ref[0:1, 0:M]
                ca1 = 1.0 + mod_ref[0:1, M:2 * M]
                for j in range(TR // T):
                    rows = pl.ds(pl.multiple_of(i * TR + j * T, T), T)
                    h_ref[rows, :] = (_ln(x_ref[rows, :].astype(F32)) * ca1 + sa2).astype(BF16)
                return 0
            r = pl.multiple_of(i * TR, TR)
            x = x_ref[pl.ds(r, TR), :].astype(F32)
            h_ref[pl.ds(r, TR), :] = (_ln(x) * (1.0 + ca) + sa).astype(BF16)
            return 0
        lax.fori_loop(0, nchunks, body, 0)
        cp_ckv.wait()
        if ENDW:
            for cp in w_copies(1, 1):
                cp.start()
        if B4:
            for cp in late:
                cp.start()

    with jax.named_scope('body'):
        with jax.named_scope('step_wait'):
            for cp in w_copies(g, slot):
                cp.wait()

        if not ENDW:
            @pl.when(g + 1 < npairs)
            def _():
                for cp in w_copies(g + 1, 1 - slot):
                    cp.start()

        if not B4:
            @pl.when(g == 1)
            def _():
                for cp in late:
                    cp.start()

        qscale = (D ** -0.5) * math.log2(math.e)
        wk = _unpack_pair(wk_buf[slot])
        wv = _unpack_pair(wv_buf[slot])
        wq = _unpack_pair(wq_buf[slot])

        row = lax.broadcasted_iota(jnp.int32, (T, T), 0)
        col = lax.broadcasted_iota(jnp.int32, (T, T), 1)
        tri = col <= row

        def proj(dst, src, w, r0, n, scale=None):
            rows = slice(r0, r0 + n)
            y = _dot(src[rows, :], w)
            if scale is not None:
                y = y * scale
            if not NEWB:
                y = y.astype(BF16)
            for hh in range(2):
                dst[hh, rows, :] = y[:, hh * D:(hh + 1) * D].astype(BF16)

        def qk(hh, i):
            r0 = i * T
            n = r0 + T
            return _dot_nt(q_ref[hh, r0:n, :], k_ref[hh, 0:n, :])

        def pv(hh, i, s):
            n = (i + 1) * T
            p, l = _softmax_rows(s, tri)
            acc = _dot(p, v_ref[hh, 0:n, :])
            return (acc * _recip(l)).astype(BF16)

        def oproj(r0, ctx):
            rows = slice(r0, r0 + ctx.shape[0])
            acc_ref[rows, :] += _dot(ctx, wo_buf[slot])

        pend = {}
        ctx = {}

        def run(op):
            kind = op[0]
            if kind == 'K':
                proj(k_ref, ckv_ref, wk, op[1], op[2])
            elif kind == 'V':
                proj(v_ref, ckv_ref, wv, op[1], op[2])
            elif kind == 'Q':
                proj(q_ref, h_ref, wq, op[1], op[2], qscale)
            elif kind == 'S':
                pend[op[1:]] = qk(*op[1:])
            elif kind == 'P':
                ctx[op[1:]] = pv(*op[1:], pend.pop(op[1:]))
            elif kind == 'O':
                blks = op[1:]
                c = [jnp.concatenate([ctx.pop((0, i)), ctx.pop((1, i))], axis=1) for i in blks]
                oproj(blks[0] * T, c[0] if len(c) == 1 else jnp.concatenate(c, axis=0))

        for op in _schedule(VAR, nblk):
            run(op)
        assert not pend and not ctx
        if ENDW:
            @pl.when(g + 2 < npairs)
            def _():
                for cp in w_copies(g + 2, slot):
                    cp.start()

    @pl.when(g == npairs - 1)
    @jax.named_scope('epilogue')
    def _epilogue():
        for cp in late:
            cp.wait()
        mod_ref[:, 2 * M:6 * M] = _dot(silu_c(), wmod_ref[:, 2 * M:6 * M])
        ga = mod_ref[0:1, 2 * M:3 * M]
        sb = mod_ref[0:1, 3 * M:4 * M]
        cb = mod_ref[0:1, 4 * M:5 * M]
        gb = mod_ref[0:1, 5 * M:6 * M]
        cb1 = 1.0 + cb
        nct = M // T
        cgrp = M // 4
        shifts = (-1, 1, -2, 2)

        def x1_of(rows):
            return x_ref[rows, :].astype(F32) + ga * acc_ref[rows, :]

        def mix_in(r, n, last):
            rows = pl.ds(r, n)
            h2 = _ln(x1_of(rows)) * (cb1 if B3 else (1.0 + cb)) + sb
            base_ref[rows, :] = h2
            hh = _gelu(_dot(_ln(h2).astype(BF16), w1_ref[...]))
            if last:
                rid = r + lax.broadcasted_iota(jnp.int32, (n, M), 0)
                hh = jnp.where(rid < S, hh, 0.0)
            for t in range(nct):
                hh_ref[t, pl.ds(PAD + r, n), :] = hh[:, t * T:(t + 1) * T]

        def mix_out(r, n):
            lane = lax.broadcasted_iota(jnp.int32, (n, T), 1)
            cols = []
            for t in range(nct):
                lo, hi = (t * T) // cgrp, (t * T + T - 1) // cgrp
                v = hh_ref[t, pl.ds(PAD + r + shifts[lo], n), :]
                if hi != lo:
                    v2 = hh_ref[t, pl.ds(PAD + r + shifts[hi], n), :]
                    v = jnp.where(lane < hi * cgrp - t * T, v, v2)
                cols.append(v)
            sh = jnp.concatenate(cols, axis=1).astype(BF16)
            rows = pl.ds(r, n)
            y1 = base_ref[rows, :] + _dot(sh, w2_ref[...])
            base_ref[rows, :] = x1_of(rows) + gb * y1
            h_ref[rows, :] = _ln(y1).astype(BF16)

        def ffn_up(r, n=TR):
            z = h_ref[pl.ds(r, n), :]
            F = w3_ref.shape[0]
            fm = (F // T) * T
            if W3T == 0 or fm == F:
                return _gelu(_dot_nt(z, w3_ref[...])).astype(BF16)
            if W3T == 1:
                tail = _gelu(_dot_nt(w3_ref[fm:F, :], z)).T
                main = _gelu(_dot_nt(z, w3_ref[0:fm, :]))
            else:
                main = _gelu(_dot_nt(z, w3_ref[0:fm, :]))
                tail = _gelu(_dot_nt(w3_ref[fm:F, :], z)).T
            return jnp.concatenate([main, tail], axis=1).astype(BF16)

        def ffn_down(r, t):
            rows = pl.ds(r, t.shape[0])
            o_buf[rows, :] = (base_ref[rows, :] + gb * _dot(t, w4_ref[...])).astype(o_buf.dtype)

        def o_copy(i):
            r = pl.multiple_of(i * TR, TR)
            return pltpu.make_async_copy(o_buf.at[pl.ds(r, TR), :], o_hbm.at[pl.ds(r, TR), :], osem.at[i])

        HR = TR // 2
        QR = TR // 4
        if EPRE == 0:
            mix_in(0, HR, False)
            mix_in(HR, HR + HALO, False)
            mix_out(0, HR)
            mix_out(HR, HR)
        elif EPRE == 1:
            mix_in(0, QR, False)
            mix_in(QR, QR, False)
            mix_in(HR, HR + HALO, False)
            mix_out(0, HR)
            mix_out(HR, QR)
            mix_out(HR + QR, QR)
        elif EPRE == 2:
            mix_in(0, QR, False)
            mix_in(QR, QR, False)
            mix_in(2 * QR, QR, False)
            mix_out(0, QR)
            mix_in(3 * QR, QR + HALO, False)
            mix_out(QR, QR)
            mix_out(2 * QR, QR)
            mix_out(3 * QR, QR)

        def body(i, _):
            r = pl.multiple_of(i * TR, TR)
            rn = r + TR
            t = {}
            for ch in ELOOP:
                if ch == 'U':
                    tt = ffn_up(r)
                    t[0], t[1] = tt[:HR], tt[HR:]
                elif ch == 'u':
                    t[0] = ffn_up(r, HR)
                elif ch == 'v':
                    t[1] = ffn_up(r + HR, HR)
                elif ch == 'I':
                    mix_in(rn, TR + HALO, True)
                elif ch == 'i':
                    mix_in(rn, HR, False)
                elif ch == 'j':
                    mix_in(rn + HR, HR + HALO, True)
                elif ch == 'O':
                    mix_out(rn, TR)
                elif ch == 'o':
                    mix_out(rn, HR)
                elif ch == 'p':
                    mix_out(rn + HR, HR)
                elif ch == 'd':
                    ffn_down(r, t[0])
                elif ch == 'e':
                    ffn_down(r + HR, t[1])
            o_copy(i).start()
            return 0
        with jax.named_scope('eloop'):
            lax.fori_loop(0, nchunks - 1, body, 0)
        with jax.named_scope('elast'):
            r = (nchunks - 1) * TR
            if ELAST == 0:
                ffn_down(r, ffn_up(r))
                o_copy(nchunks - 1).start()
                for i in range(nchunks):
                    o_copy(i).wait()
            else:
                tt = ffn_up(r)
                ca = pltpu.make_async_copy(o_buf.at[r:r + HR, :], o_hbm.at[r:r + HR, :], osem.at[nchunks - 1])
                cb_ = pltpu.make_async_copy(o_buf.at[r + HR:r + TR, :], o_hbm.at[r + HR:r + TR, :], isem.at[0])
                ffn_down(r, tt[:HR])
                ca.start()
                ffn_down(r + HR, tt[HR:])
                cb_.start()
                for i in range(nchunks - 1):
                    o_copy(i).wait()
                ca.wait()
                cb_.wait()


@jax.jit
def pallas_adaLN_cond__compressed_kv_cla__mixer_s_mlp__prompt_kernel(
    A_x, A_c_kv, A_w_q, A_w_uk, A_w_uv, A_w_o, B_x, B_w1, B_w2, B_w3, B_w4, c, w_mod,
):
    del B_x
    _, S, M = A_x.shape
    Dc = A_c_kv.shape[2]
    H, D = A_w_q.shape[1], A_w_q.shape[2]
    F = B_w3.shape[1]
    x = A_x.reshape(S, M)
    ckv = A_c_kv.reshape(S, Dc)
    w3t = B_w3.T
    wo = A_w_o.reshape(H // 2, 2 * D, M)
    ins = (x, ckv, A_w_q, A_w_uk, A_w_uv, wo, B_w1, B_w2, w3t, B_w4, c, w_mod)

    out = pl.pallas_call(
        functools.partial(_kernel, S=S, M=M, Dc=Dc, H=H, D=D),
        grid=(H // 2,),
        in_specs=[pl.BlockSpec(memory_space=pl.ANY) for _ in ins],
        out_specs=pl.BlockSpec(memory_space=pl.ANY),
        out_shape=jax.ShapeDtypeStruct((S, M), A_x.dtype),
        scratch_shapes=[
            pltpu.VMEM((S + HALO, M), BF16),
            pltpu.VMEM((S, Dc), BF16),
            pltpu.VMEM((M, M), BF16),
            pltpu.VMEM((M, M), BF16),
            pltpu.VMEM((F, M), BF16),
            pltpu.VMEM((F, M), BF16),
            pltpu.VMEM((1, M), BF16),
            pltpu.VMEM((M, 6 * M), BF16),
            pltpu.VMEM((2, M, D), U32),
            pltpu.VMEM((2, Dc, D), U32),
            pltpu.VMEM((2, Dc, D), U32),
            pltpu.VMEM((2, 2 * D, M), BF16),
            pltpu.VMEM((8, 6 * M), F32),
            pltpu.VMEM((S, M), BF16),
            pltpu.VMEM((2, S, D), BF16),
            pltpu.VMEM((2, S, D), BF16),
            pltpu.VMEM((2, S, D), BF16),
            pltpu.VMEM((S + HALO, M), F32),
            pltpu.VMEM((S + HALO, M), F32),
            pltpu.VMEM((M // T, PAD + S + HALO, T), F32),
            pltpu.VMEM((S, M), A_x.dtype),
            pltpu.SemaphoreType.DMA((4, 2)),
            pltpu.SemaphoreType.DMA((9,)),
            pltpu.SemaphoreType.DMA((S // TR,)),
        ],
        compiler_params=pltpu.CompilerParams(
            dimension_semantics=("arbitrary",),
            vmem_limit_bytes=100 * 1024 * 1024,
            disable_bounds_checks=bool(NOBC),
        ),
    )(*ins)
    return out.reshape(1, S, M)
```

```python
import functools
import math

import jax
import jax.numpy as jnp
from jax import lax
import jax.experimental.pallas as pl
import jax.experimental.pallas.tpu as pltpu

F32 = jnp.float32
BF16 = jnp.bfloat16
U32 = jnp.uint32
EPS = 1e-5
NEG = -1e30
T = 128
TR = 256
PAD = 8
HALO = 16
NRES = 2
ODEL = 3
LAST = 64


def _ln(x):
    m = jnp.mean(x, axis=-1, keepdims=True)
    xc = x - m
    v = jnp.mean(xc * xc, axis=-1, keepdims=True)
    return xc * lax.rsqrt(v + EPS)


def _gelu(x):
    c = math.sqrt(2.0 / math.pi)
    hx = 0.5 * x
    return hx + hx * jnp.tanh(x * (c + (c * 0.044715) * (x * x)))


def _dot(a, b):
    return jnp.dot(a, b, preferred_element_type=F32)


def _dot_nt(a, b):
    return lax.dot_general(a, b, (((1,), (1,)), ((), ())), preferred_element_type=F32)


def _recip(l):
    r = pl.reciprocal(l, approx=True)
    return r * (2.0 - l * r)


def _unpack_pair(u):
    lo = pltpu.bitcast(u << 16, F32)
    hi = pltpu.bitcast(u & jnp.uint32(0xFFFF0000), F32)
    return jnp.concatenate([lo, hi], axis=1).astype(BF16)


def _rows_bf16(ref, a=None, b=None):
    return pltpu.bitcast(ref[...] if a is None else ref[a // 2:b // 2, :], BF16)


def _softmax_rows(s, tri):
    n = s.shape[1]
    sd = jnp.where(tri, s[:, n - T:], NEG)
    s = sd if n == T else jnp.concatenate([s[:, :n - T], sd], axis=1)
    m = jnp.max(s, axis=-1, keepdims=True)
    p = jnp.exp2(s - m).astype(BF16)
    return p, jnp.sum(p.astype(F32), axis=-1, keepdims=True)


def _schedule(nblk):
    order = [0] + list(range(NRES + 1, nblk)) + list(range(NRES, 0, -1))
    ops = [('K', 0), ('Q', 0), ('V', 0)]
    kv_done = 1
    oq = []
    for t, i in enumerate(order):
        nxt = order[t + 1] if t + 1 < nblk else None
        newkv = list(range(kv_done, nxt + 1)) if nxt is not None else []
        kv_done += len(newkv)
        ops.append(('S', 0, i))
        ops += [('V', j) for j in newkv] + [('K', j) for j in newkv]
        if not newkv and len(oq) > 1:
            ops.append(('O', oq.pop(0)))
        if t > 0:
            ops.append(('P', 1, order[t - 1]))
            oq.append(order[t - 1])
        ops.append(('S', 1, i))
        if nxt is not None:
            ops.append(('Q', nxt))
        if len(oq) >= ODEL or (not newkv and len(oq) > 1):
            ops.append(('O', oq.pop(0)))
        ops.append(('P', 0, i))
    ops.append(('P', 1, order[-1]))
    ops += [('O', i) for i in oq] + [('O', order[-1])]
    return ops


def _kernel(x_hbm, ckv_hbm, wq_hbm, wk_hbm, wv_hbm, wo_hbm, w1_hbm, w2_hbm, w3_hbm, w4_hbm,
            c_hbm, wmod_hbm, o_hbm,
            x_ref, ckv_ref, w1_ref, w2_ref, w3_ref, w4_ref, c_ref, wmod_ref,
            wq_buf, wk_buf, wv_buf, wo_buf,
            mod_ref, h_ref, q_ref, k_ref, v_ref, acc_ref, base_ref, hh_ref, o_buf,
            wsem, isem, xsem,
            *, S, M, Dc, H, D, F):
    g = pl.program_id(0)
    npairs = H // 2
    nchunks = S // TR
    nblk = S // T
    slot = g % 2

    def w_copies(pair, sl):
        cps = [
            pltpu.make_async_copy(src.bitcast(U32).at[:, pair, :], dst.at[sl], wsem.at[j, sl])
            for j, (src, dst) in enumerate(((wk_hbm, wk_buf), (wv_hbm, wv_buf), (wq_hbm, wq_buf)))
        ]
        cps.append(pltpu.make_async_copy(wo_hbm.at[pair], wo_buf.at[sl], wsem.at[3, sl]))
        return cps

    def x_copy(i):
        rows = pl.ds(pl.multiple_of(i * TR, TR), TR)
        return pltpu.make_async_copy(x_hbm.at[rows, :], x_ref.at[rows, :], xsem.at[i])

    def late_copies():
        return [
            pltpu.make_async_copy(wmod_hbm.at[:, 2 * M:6 * M], wmod_ref.at[:, 2 * M:6 * M], isem.at[3]),
            pltpu.make_async_copy(w1_hbm.bitcast(U32), w1_ref, isem.at[4]),
            pltpu.make_async_copy(w2_hbm.bitcast(U32), w2_ref, isem.at[5]),
            pltpu.make_async_copy(w3_hbm.bitcast(U32), w3_ref, isem.at[6]),
            pltpu.make_async_copy(w4_hbm.bitcast(U32), w4_ref, isem.at[7]),
        ]

    def silu_c():
        c = c_ref[...].astype(F32)
        sc = c * (1.0 / (1.0 + jnp.exp(-c)))
        return jnp.broadcast_to(sc, (8, M)).astype(BF16)

    @pl.when(g == 0)
    def _prologue():
        cp_c = pltpu.make_async_copy(c_hbm, c_ref, isem.at[0])
        cp_mod = pltpu.make_async_copy(wmod_hbm.at[:, 0:2 * M], wmod_ref.at[:, 0:2 * M], isem.at[1])
        cp_ckv = pltpu.make_async_copy(ckv_hbm, ckv_ref, isem.at[2])
        cp_c.start()
        cp_mod.start()
        for i in range(nchunks):
            x_copy(i).start()
        cp_ckv.start()
        for cp in w_copies(0, 0):
            cp.start()

        def zero(i, _):
            acc_ref[pl.ds(pl.multiple_of(i * T, T), T), :] = jnp.zeros((T, M), F32)
            return 0
        lax.fori_loop(0, nblk, zero, 0)
        acc_ref[S:S + HALO, :] = jnp.zeros((HALO, M), F32)
        x_ref[S:S + HALO, :] = jnp.zeros((HALO, M), BF16)
        hh_ref[:, 0:PAD, :] = jnp.zeros((M // T, PAD, T), F32)

        cp_c.wait()
        cp_mod.wait()
        mod_ref[:, 0:2 * M] = _dot(silu_c(), wmod_ref[:, 0:2 * M])

        def adaln(i, _):
            x_copy(i).wait()
            sa = mod_ref[0:1, 0:M]
            ca1 = 1.0 + mod_ref[0:1, M:2 * M]
            for j in range(TR // T):
                rows = pl.ds(pl.multiple_of(i * TR + j * T, T), T)
                h_ref[rows, :] = (_ln(x_ref[rows, :].astype(F32)) * ca1 + sa).astype(BF16)
            return 0
        lax.fori_loop(0, nchunks, adaln, 0)
        cp_ckv.wait()
        for cp in w_copies(1, 1) + late_copies():
            cp.start()

    for cp in w_copies(g, slot):
        cp.wait()

    qscale = (D ** -0.5) * math.log2(math.e)
    wk = _unpack_pair(wk_buf[slot])
    wv = _unpack_pair(wv_buf[slot])
    wq = _unpack_pair(wq_buf[slot])

    row = lax.broadcasted_iota(jnp.int32, (T, T), 0)
    col = lax.broadcasted_iota(jnp.int32, (T, T), 1)
    tri = col <= row

    def proj(dst, src, w, i, scale=None):
        rows = slice(i * T, (i + 1) * T)
        y = _dot(src[rows, :], w)
        if scale is not None:
            y = y * scale
        for hh in range(2):
            dst[hh, rows, :] = y[:, hh * D:(hh + 1) * D].astype(BF16)

    scores, ctx = {}, {}
    for op in _schedule(nblk):
        kind, i = op[0], op[-1]
        if kind == 'K':
            proj(k_ref, ckv_ref, wk, i)
        elif kind == 'V':
            proj(v_ref, ckv_ref, wv, i)
        elif kind == 'Q':
            proj(q_ref, h_ref, wq, i, qscale)
        elif kind == 'S':
            hh = op[1]
            scores[hh, i] = _dot_nt(q_ref[hh, i * T:(i + 1) * T, :], k_ref[hh, 0:(i + 1) * T, :])
        elif kind == 'P':
            hh = op[1]
            p, l = _softmax_rows(scores.pop((hh, i)), tri)
            ctx[hh, i] = (_dot(p, v_ref[hh, 0:(i + 1) * T, :]) * _recip(l)).astype(BF16)
        else:
            c = jnp.concatenate([ctx.pop((0, i)), ctx.pop((1, i))], axis=1)
            acc_ref[i * T:(i + 1) * T, :] += _dot(c, wo_buf[slot])
    assert not scores and not ctx

    @pl.when(g + 2 < npairs)
    def _():
        for cp in w_copies(g + 2, slot):
            cp.start()

    @pl.when(g == npairs - 1)
    def _epilogue():
        for cp in late_copies():
            cp.wait()
        mod_ref[:, 2 * M:6 * M] = _dot(silu_c(), wmod_ref[:, 2 * M:6 * M])
        ga = mod_ref[0:1, 2 * M:3 * M]
        sb = mod_ref[0:1, 3 * M:4 * M]
        cb1 = 1.0 + mod_ref[0:1, 4 * M:5 * M]
        gb = mod_ref[0:1, 5 * M:6 * M]
        nct = M // T
        cgrp = M // 4
        shifts = (-1, 1, -2, 2)

        def x1_of(rows):
            return x_ref[rows, :].astype(F32) + ga * acc_ref[rows, :]

        def mix_in(r, n, may_overrun):
            rows = pl.ds(r, n)
            h2 = _ln(x1_of(rows)) * cb1 + sb
            base_ref[rows, :] = h2
            hh = _gelu(_dot(_ln(h2).astype(BF16), _rows_bf16(w1_ref)))
            if may_overrun:
                rid = r + lax.broadcasted_iota(jnp.int32, (n, M), 0)
                hh = jnp.where(rid < S, hh, 0.0)
            for t in range(nct):
                hh_ref[t, pl.ds(PAD + r, n), :] = hh[:, t * T:(t + 1) * T]

        def mix_out(r, n):
            lane = lax.broadcasted_iota(jnp.int32, (n, T), 1)
            cols = []
            for t in range(nct):
                lo, hi = (t * T) // cgrp, (t * T + T - 1) // cgrp
                v = hh_ref[t, pl.ds(PAD + r + shifts[lo], n), :]
                if hi != lo:
                    v2 = hh_ref[t, pl.ds(PAD + r + shifts[hi], n), :]
                    v = jnp.where(lane < hi * cgrp - t * T, v, v2)
                cols.append(v)
            sh = jnp.concatenate(cols, axis=1).astype(BF16)
            rows = pl.ds(r, n)
            y1 = base_ref[rows, :] + _dot(sh, _rows_bf16(w2_ref))
            base_ref[rows, :] = x1_of(rows) + gb * y1
            h_ref[rows, :] = _ln(y1).astype(BF16)

        def ffn_up(r, n):
            z = h_ref[pl.ds(r, n), :]
            fm = (F // T) * T
            if fm == F:
                return _gelu(_dot_nt(z, _rows_bf16(w3_ref))).astype(BF16)
            tail = _gelu(_dot_nt(_rows_bf16(w3_ref, fm, F), z)).T
            main = _gelu(_dot_nt(z, _rows_bf16(w3_ref, 0, fm)))
            return jnp.concatenate([main, tail], axis=1).astype(BF16)

        def ffn_down(r, t):
            rows = pl.ds(r, t.shape[0])
            o_buf[rows, :] = (base_ref[rows, :] + gb * _dot(t, _rows_bf16(w4_ref))).astype(o_buf.dtype)

        def o_copy(r, n, sem):
            return pltpu.make_async_copy(o_buf.at[pl.ds(r, n), :], o_hbm.at[pl.ds(r, n), :], sem)

        HR = TR // 2
        mix_in(0, HR, False)
        mix_in(HR, HR + HALO, False)
        mix_out(0, HR)
        mix_out(HR, HR)

        def body(i, _):
            r = pl.multiple_of(i * TR, TR)
            rn = r + TR
            t0 = ffn_up(r, HR)
            mix_in(rn, HR, False)
            t1 = ffn_up(r + HR, HR)
            mix_in(rn + HR, HR + HALO, True)
            ffn_down(r, t0)
            mix_out(rn, TR)
            ffn_down(r + HR, t1)
            o_copy(r, TR, xsem.at[i]).start()
            return 0
        lax.fori_loop(0, nchunks - 1, body, 0)

        r = (nchunks - 1) * TR
        n1 = TR - LAST
        cp_a = o_copy(r, n1, xsem.at[nchunks - 1])
        cp_b = o_copy(r + n1, LAST, isem.at[0])
        t = ffn_up(r, TR)
        ffn_down(r, t[:n1])
        cp_a.start()
        ffn_down(r + n1, t[n1:])
        cp_b.start()
        for i in range(nchunks - 1):
            o_copy(i * TR, TR, xsem.at[i]).wait()
        cp_a.wait()
        cp_b.wait()


@jax.jit
def pallas_adaLN_cond__compressed_kv_cla__mixer_s_mlp__prompt_kernel(
    A_x, A_c_kv, A_w_q, A_w_uk, A_w_uv, A_w_o, B_x, B_w1, B_w2, B_w3, B_w4, c, w_mod,
):
    del B_x
    _, S, M = A_x.shape
    Dc = A_c_kv.shape[2]
    H, D = A_w_q.shape[1], A_w_q.shape[2]
    F = B_w3.shape[1]
    ins = (A_x.reshape(S, M), A_c_kv.reshape(S, Dc), A_w_q, A_w_uk, A_w_uv,
           A_w_o.reshape(H // 2, 2 * D, M), B_w1, B_w2, B_w3.T, B_w4, c, w_mod)

    out = pl.pallas_call(
        functools.partial(_kernel, S=S, M=M, Dc=Dc, H=H, D=D, F=F),
        grid=(H // 2,),
        in_specs=[pl.BlockSpec(memory_space=pl.ANY) for _ in ins],
        out_specs=pl.BlockSpec(memory_space=pl.ANY),
        out_shape=jax.ShapeDtypeStruct((S, M), A_x.dtype),
        scratch_shapes=[
            pltpu.VMEM((S + HALO, M), BF16),
            pltpu.VMEM((S, Dc), BF16),
            pltpu.VMEM((M // 2, M), U32),
            pltpu.VMEM((M // 2, M), U32),
            pltpu.VMEM((F // 2, M), U32),
            pltpu.VMEM((F // 2, M), U32),
            pltpu.VMEM((1, M), BF16),
            pltpu.VMEM((M, 6 * M), BF16),
            pltpu.VMEM((2, M, D), U32),
            pltpu.VMEM((2, Dc, D), U32),
            pltpu.VMEM((2, Dc, D), U32),
            pltpu.VMEM((2, 2 * D, M), BF16),
            pltpu.VMEM((8, 6 * M), F32),
            pltpu.VMEM((S, M), BF16),
            pltpu.VMEM((2, S, D), BF16),
            pltpu.VMEM((2, S, D), BF16),
            pltpu.VMEM((2, S, D), BF16),
            pltpu.VMEM((S + HALO, M), F32),
            pltpu.VMEM((S + HALO, M), F32),
            pltpu.VMEM((M // T, PAD + S + HALO, T), F32),
            pltpu.VMEM((S, M), A_x.dtype),
            pltpu.SemaphoreType.DMA((4, 2)),
            pltpu.SemaphoreType.DMA((8,)),
            pltpu.SemaphoreType.DMA((S // TR,)),
        ],
        compiler_params=pltpu.CompilerParams(
            dimension_semantics=("arbitrary",),
            vmem_limit_bytes=100 * 1024 * 1024,
            disable_bounds_checks=True,
        ),
    )(*ins)
    return out.reshape(1, S, M)
```

```python
import functools
import math

import jax
import jax.numpy as jnp
from jax import lax
import jax.experimental.pallas as pl
import jax.experimental.pallas.tpu as pltpu

F32 = jnp.float32
BF16 = jnp.bfloat16
U32 = jnp.uint32
EPS = 1e-5
NEG = -1e30
T = 128
TR = 256
PAD = 8
HALO = 16
NRES = 2
ODEL = 3
LAST = 64


def _ln(x):
    m = jnp.mean(x, axis=-1, keepdims=True)
    xc = x - m
    v = jnp.mean(xc * xc, axis=-1, keepdims=True)
    return xc * lax.rsqrt(v + EPS)


def _gelu(x):
    c = math.sqrt(2.0 / math.pi)
    hx = 0.5 * x
    return hx + hx * jnp.tanh(x * (c + (c * 0.044715) * (x * x)))


def _dot(a, b):
    return jnp.dot(a, b, preferred_element_type=F32)


def _dot_nt(a, b):
    return lax.dot_general(a, b, (((1,), (1,)), ((), ())), preferred_element_type=F32)


def _recip(l):
    r = pl.reciprocal(l, approx=True)
    return r * (2.0 - l * r)


def _unpack_pair(u):
    lo = pltpu.bitcast(u << 16, F32)
    hi = pltpu.bitcast(u & jnp.uint32(0xFFFF0000), F32)
    return jnp.concatenate([lo, hi], axis=1).astype(BF16)


def _rows_bf16(ref, a=None, b=None):
    return pltpu.bitcast(ref[...] if a is None else ref[a // 2:b // 2, :], BF16)


def _softmax_rows(s, tri):
    n = s.shape[1]
    sd = jnp.where(tri, s[:, n - T:], NEG)
    s = sd if n == T else jnp.concatenate([s[:, :n - T], sd], axis=1)
    m = jnp.max(s, axis=-1, keepdims=True)
    p = jnp.exp2(s - m).astype(BF16)
    return p, jnp.sum(p.astype(F32), axis=-1, keepdims=True)


def _schedule(nblk):
    order = [0] + list(range(NRES + 1, nblk)) + list(range(NRES, 0, -1))
    ops = [('K', 0), ('Q', 0), ('V', 0)]
    kv_done = 1
    oq = []
    for t, i in enumerate(order):
        nxt = order[t + 1] if t + 1 < nblk else None
        newkv = list(range(kv_done, nxt + 1)) if nxt is not None else []
        kv_done += len(newkv)
        ops.append(('S', 0, i))
        ops += [('V', j) for j in newkv] + [('K', j) for j in newkv]
        if not newkv and len(oq) > 1:
            ops.append(('O', oq.pop(0)))
        if t > 0:
            ops.append(('P', 1, order[t - 1]))
            oq.append(order[t - 1])
        ops.append(('S', 1, i))
        if nxt is not None:
            ops.append(('Q', nxt))
        if len(oq) >= ODEL or (not newkv and len(oq) > 1):
            ops.append(('O', oq.pop(0)))
        ops.append(('P', 0, i))
    ops.append(('P', 1, order[-1]))
    ops += [('O', i) for i in oq] + [('O', order[-1])]
    return ops


def _kernel(x_hbm, ckv_hbm, wq_hbm, wk_hbm, wv_hbm, wo_hbm, w1_hbm, w2_hbm, w3_hbm, w4_hbm,
            c_hbm, wmod_hbm, o_hbm,
            x_ref, ckv_ref, w1_ref, w2_ref, w3_ref, w4_ref, c_ref, wmod_ref,
            wq_buf, wk_buf, wv_buf, wo_buf,
            mod_ref, h_ref, q_ref, k_ref, v_ref, acc_ref, base_ref, hh_ref, h2_ref, z_ref, o_buf,
            wsem, isem, xsem,
            *, S, M, Dc, H, D, F):
    g = pl.program_id(0)
    npairs = H // 2
    nchunks = S // TR
    nblk = S // T
    slot = g % 2

    def w_copies(pair, sl):
        cps = [
            pltpu.make_async_copy(src.bitcast(U32).at[:, pair, :], dst.at[sl], wsem.at[j, sl])
            for j, (src, dst) in enumerate(((wk_hbm, wk_buf), (wv_hbm, wv_buf), (wq_hbm, wq_buf)))
        ]
        cps.append(pltpu.make_async_copy(wo_hbm.at[pair], wo_buf.at[sl], wsem.at[3, sl]))
        return cps

    def x_copy(i):
        rows = pl.ds(pl.multiple_of(i * TR, TR), TR)
        return pltpu.make_async_copy(x_hbm.at[rows, :], x_ref.at[rows, :], xsem.at[i])

    def late_copies():
        return [
            pltpu.make_async_copy(wmod_hbm.at[:, 2 * M:6 * M], wmod_ref.at[:, 2 * M:6 * M], isem.at[3]),
            pltpu.make_async_copy(w1_hbm.bitcast(U32), w1_ref, isem.at[4]),
            pltpu.make_async_copy(w2_hbm.bitcast(U32), w2_ref, isem.at[5]),
            pltpu.make_async_copy(w3_hbm.bitcast(U32), w3_ref, isem.at[6]),
            pltpu.make_async_copy(w4_hbm.bitcast(U32), w4_ref, isem.at[7]),
        ]

    def silu_c():
        c = c_ref[...].astype(F32)
        sc = c * (1.0 / (1.0 + jnp.exp(-c)))
        return jnp.broadcast_to(sc, (8, M)).astype(BF16)

    @pl.when(g == 0)
    def _prologue():
        cp_c = pltpu.make_async_copy(c_hbm, c_ref, isem.at[0])
        cp_mod = pltpu.make_async_copy(wmod_hbm.at[:, 0:2 * M], wmod_ref.at[:, 0:2 * M], isem.at[1])
        cp_ckv = pltpu.make_async_copy(ckv_hbm, ckv_ref, isem.at[2])
        cp_c.start()
        cp_mod.start()
        for i in range(nchunks):
            x_copy(i).start()
        cp_ckv.start()
        for cp in w_copies(0, 0):
            cp.start()

        def zero(i, _):
            acc_ref[pl.ds(pl.multiple_of(i * T, T), T), :] = jnp.zeros((T, M), F32)
            return 0
        lax.fori_loop(0, nblk, zero, 0)
        acc_ref[S:S + HALO, :] = jnp.zeros((HALO, M), F32)
        x_ref[S:S + HALO, :] = jnp.zeros((HALO, M), BF16)
        hh_ref[:, 0:PAD, :] = jnp.zeros((M // T, PAD, T), F32)

        cp_c.wait()
        cp_mod.wait()
        mod_ref[:, 0:2 * M] = _dot(silu_c(), wmod_ref[:, 0:2 * M])

        def adaln(i, _):
            x_copy(i).wait()
            sa = mod_ref[0:1, 0:M]
            ca1 = 1.0 + mod_ref[0:1, M:2 * M]
            for j in range(TR // T):
                rows = pl.ds(pl.multiple_of(i * TR + j * T, T), T)
                h_ref[rows, :] = (_ln(x_ref[rows, :].astype(F32)) * ca1 + sa).astype(BF16)
            return 0
        lax.fori_loop(0, nchunks, adaln, 0)
        cp_ckv.wait()
        for cp in w_copies(1, 1) + late_copies():
            cp.start()

    for cp in w_copies(g, slot):
        cp.wait()

    qscale = (D ** -0.5) * math.log2(math.e)
    wk = _unpack_pair(wk_buf[slot])
    wv = _unpack_pair(wv_buf[slot])
    wq = _unpack_pair(wq_buf[slot])

    row = lax.broadcasted_iota(jnp.int32, (T, T), 0)
    col = lax.broadcasted_iota(jnp.int32, (T, T), 1)
    tri = col <= row

    def proj(dst, src, w, i, scale=None):
        rows = slice(i * T, (i + 1) * T)
        y = _dot(src[rows, :], w)
        if scale is not None:
            y = y * scale
        for hh in range(2):
            dst[hh, rows, :] = y[:, hh * D:(hh + 1) * D].astype(BF16)

    scores, ctx = {}, {}
    for op in _schedule(nblk):
        kind, i = op[0], op[-1]
        if kind == 'K':
            proj(k_ref, ckv_ref, wk, i)
        elif kind == 'V':
            proj(v_ref, ckv_ref, wv, i)
        elif kind == 'Q':
            proj(q_ref, h_ref, wq, i, qscale)
        elif kind == 'S':
            hh = op[1]
            scores[hh, i] = _dot_nt(q_ref[hh, i * T:(i + 1) * T, :], k_ref[hh, 0:(i + 1) * T, :])
        elif kind == 'P':
            hh = op[1]
            p, l = _softmax_rows(scores.pop((hh, i)), tri)
            ctx[hh, i] = (_dot(p, v_ref[hh, 0:(i + 1) * T, :]) * _recip(l)).astype(BF16)
        else:
            c = jnp.concatenate([ctx.pop((0, i)), ctx.pop((1, i))], axis=1)
            acc_ref[i * T:(i + 1) * T, :] += _dot(c, wo_buf[slot])
    assert not scores and not ctx

    @pl.when(g + 2 < npairs)
    def _():
        for cp in w_copies(g + 2, slot):
            cp.start()

    @pl.when(g == npairs - 1)
    def _epilogue():
        for cp in late_copies():
            cp.wait()
        mod_ref[:, 2 * M:6 * M] = _dot(silu_c(), wmod_ref[:, 2 * M:6 * M])
        ga = mod_ref[0:1, 2 * M:3 * M]
        sb = mod_ref[0:1, 3 * M:4 * M]
        cb1 = 1.0 + mod_ref[0:1, 4 * M:5 * M]
        gb = mod_ref[0:1, 5 * M:6 * M]
        nct = M // T
        cgrp = M // 4
        shifts = (-1, 1, -2, 2)

        def x1_of(rows):
            return x_ref[rows, :].astype(F32) + ga * acc_ref[rows, :]

        def mix_in(r0, k, n, may_overrun):
            rows = pl.ds(r0 + k, n)
            h2 = _ln(x1_of(rows)) * cb1 + sb
            h2_ref[k:k + n, :] = h2
            hh = _gelu(_dot(_ln(h2).astype(BF16), _rows_bf16(w1_ref)))
            if may_overrun:
                rid = r0 + k + lax.broadcasted_iota(jnp.int32, (n, M), 0)
                hh = jnp.where(rid < S, hh, 0.0)
            for t in range(nct):
                hh_ref[t, PAD + k:PAD + k + n, :] = hh[:, t * T:(t + 1) * T]

        def mix_out(r0, k, n):
            lane = lax.broadcasted_iota(jnp.int32, (n, T), 1)
            cols = []
            for t in range(nct):
                lo, hi = (t * T) // cgrp, (t * T + T - 1) // cgrp
                v = hh_ref[t, pl.ds(PAD + k + shifts[lo], n), :]
                if hi != lo:
                    v2 = hh_ref[t, pl.ds(PAD + k + shifts[hi], n), :]
                    v = jnp.where(lane < hi * cgrp - t * T, v, v2)
                cols.append(v)
            sh = jnp.concatenate(cols, axis=1).astype(BF16)
            rows = pl.ds(r0 + k, n)
            y1 = h2_ref[k:k + n, :] + _dot(sh, _rows_bf16(w2_ref))
            base_ref[rows, :] = x1_of(rows) + gb * y1
            z_ref[k:k + n, :] = _ln(y1).astype(BF16)

        def ffn_up(k, n):
            z = z_ref[k:k + n, :]
            fm = (F // T) * T
            if fm == F:
                return _gelu(_dot_nt(z, _rows_bf16(w3_ref))).astype(BF16)
            tail = _gelu(_dot_nt(_rows_bf16(w3_ref, fm, F), z)).T
            main = _gelu(_dot_nt(z, _rows_bf16(w3_ref, 0, fm)))
            return jnp.concatenate([main, tail], axis=1).astype(BF16)

        def ffn_down(r, t):
            rows = pl.ds(r, t.shape[0])
            o_buf[rows, :] = (base_ref[rows, :] + gb * _dot(t, _rows_bf16(w4_ref))).astype(o_buf.dtype)

        def o_copy(r, n, sem):
            return pltpu.make_async_copy(o_buf.at[pl.ds(r, n), :], o_hbm.at[pl.ds(r, n), :], sem)

        HR = TR // 2
        mix_in(0, 0, HR, False)
        mix_in(0, HR, HR + HALO, False)
        mix_out(0, 0, HR)
        mix_out(0, HR, HR)

        def body(i, _):
            r = pl.multiple_of(i * TR, TR)
            rn = pl.multiple_of(r + TR, TR)
            hh_ref[:, 0:PAD + HALO, :] = hh_ref[:, TR:TR + PAD + HALO, :]
            h2_ref[0:HALO, :] = h2_ref[TR:TR + HALO, :]
            t0 = ffn_up(0, HR)
            mix_in(rn, HALO, HR, False)
            t1 = ffn_up(HR, HR)
            mix_out(rn, 0, HR)
            mix_in(rn, HALO + HR, HR, True)
            ffn_down(r, t0)
            mix_out(rn, HR, HR)
            ffn_down(r + HR, t1)
            o_copy(r, TR, xsem.at[i]).start()
            return 0
        lax.fori_loop(0, nchunks - 1, body, 0)

        r = (nchunks - 1) * TR
        n1 = TR - LAST
        cp_a = o_copy(r, n1, xsem.at[nchunks - 1])
        cp_b = o_copy(r + n1, LAST, isem.at[0])
        t = ffn_up(0, TR)
        ffn_down(r, t[:n1])
        cp_a.start()
        ffn_down(r + n1, t[n1:])
        cp_b.start()
        for i in range(nchunks - 1):
            o_copy(i * TR, TR, xsem.at[i]).wait()
        cp_a.wait()
        cp_b.wait()


@jax.jit
def pallas_adaLN_cond__compressed_kv_cla__mixer_s_mlp__prompt_kernel(
    A_x, A_c_kv, A_w_q, A_w_uk, A_w_uv, A_w_o, B_x, B_w1, B_w2, B_w3, B_w4, c, w_mod,
):
    del B_x
    _, S, M = A_x.shape
    Dc = A_c_kv.shape[2]
    H, D = A_w_q.shape[1], A_w_q.shape[2]
    F = B_w3.shape[1]
    ins = (A_x.reshape(S, M), A_c_kv.reshape(S, Dc), A_w_q, A_w_uk, A_w_uv,
           A_w_o.reshape(H // 2, 2 * D, M), B_w1, B_w2, B_w3.T, B_w4, c, w_mod)

    out = pl.pallas_call(
        functools.partial(_kernel, S=S, M=M, Dc=Dc, H=H, D=D, F=F),
        grid=(H // 2,),
        in_specs=[pl.BlockSpec(memory_space=pl.ANY) for _ in ins],
        out_specs=pl.BlockSpec(memory_space=pl.ANY),
        out_shape=jax.ShapeDtypeStruct((S, M), A_x.dtype),
        scratch_shapes=[
            pltpu.VMEM((S + HALO, M), BF16),
            pltpu.VMEM((S, Dc), BF16),
            pltpu.VMEM((M // 2, M), U32),
            pltpu.VMEM((M // 2, M), U32),
            pltpu.VMEM((F // 2, M), U32),
            pltpu.VMEM((F // 2, M), U32),
            pltpu.VMEM((1, M), BF16),
            pltpu.VMEM((M, 6 * M), BF16),
            pltpu.VMEM((2, M, D), U32),
            pltpu.VMEM((2, Dc, D), U32),
            pltpu.VMEM((2, Dc, D), U32),
            pltpu.VMEM((2, 2 * D, M), BF16),
            pltpu.VMEM((8, 6 * M), F32),
            pltpu.VMEM((S, M), BF16),
            pltpu.VMEM((2, S, D), BF16),
            pltpu.VMEM((2, S, D), BF16),
            pltpu.VMEM((2, S, D), BF16),
            pltpu.VMEM((S + HALO, M), F32),
            pltpu.VMEM((S, M), F32),
            pltpu.VMEM((M // T, PAD + TR + HALO, T), F32),
            pltpu.VMEM((TR + HALO, M), F32),
            pltpu.VMEM((TR, M), BF16),
            pltpu.VMEM((S, M), A_x.dtype),
            pltpu.SemaphoreType.DMA((4, 2)),
            pltpu.SemaphoreType.DMA((8,)),
            pltpu.SemaphoreType.DMA((S // TR,)),
        ],
        compiler_params=pltpu.CompilerParams(
            dimension_semantics=("arbitrary",),
            vmem_limit_bytes=100 * 1024 * 1024,
            disable_bounds_checks=True,
        ),
    )(*ins)
    return out.reshape(1, S, M)
```

```python
import functools
import math

import jax
import jax.numpy as jnp
from jax import lax
import jax.experimental.pallas as pl
import jax.experimental.pallas.tpu as pltpu

F32 = jnp.float32
BF16 = jnp.bfloat16
U32 = jnp.uint32
EPS = 1e-5
NEG = -1e30
T = 128
TR = 256
PAD = 8
HALO = 16
TPL = 'aKVopbQOq'
ODEL = 3
TPL2 = 'aepbeOq'
OD2 = 2
ORDL = ''
PEEL = 0
T0 = 11
MODP = 10
EU = 1
NA = 6
NB = 4
SORD = 'lbsm'
TAILO = 'KQV'
NOST = 0
PB = 'kvqqqq'
LAST = 64


def _ln(x):
    m = jnp.mean(x, axis=-1, keepdims=True)
    xc = x - m
    v = jnp.mean(xc * xc, axis=-1, keepdims=True)
    return xc * lax.rsqrt(v + EPS)


def _gelu(x):
    c = math.sqrt(2.0 / math.pi)
    hx = 0.5 * x
    return hx + hx * jnp.tanh(x * (c + (c * 0.044715) * (x * x)))


def _dot(a, b):
    return jnp.dot(a, b, preferred_element_type=F32)


def _dot_nt(a, b):
    return lax.dot_general(a, b, (((1,), (1,)), ((), ())), preferred_element_type=F32)


def _recip(l):
    r = pl.reciprocal(l, approx=True)
    return r * (2.0 - l * r)


def _unpack_pair(u):
    lo = pltpu.bitcast(u << 16, F32)
    hi = pltpu.bitcast(u & jnp.uint32(0xFFFF0000), F32)
    return jnp.concatenate([lo, hi], axis=1).astype(BF16)


def _rows_bf16(ref, a=None, b=None):
    return pltpu.bitcast(ref[...] if a is None else ref[a // 2:b // 2, :], BF16)


def _softmax_rows(s):
    m = jnp.max(s, axis=-1, keepdims=True)
    p = jnp.exp2(s - m).astype(BF16)
    return p, jnp.sum(p.astype(F32), axis=-1, keepdims=True)


def _schedule(nblk):
    order = list(range(nblk - 1, -1, -1))
    ops = []
    oq = []
    dead = {'K': [], 'V': [], 'Q': []}
    for t, i in enumerate(order):
        mate = order[t + 1] if t % 2 == 0 else None
        for ch in TPL:
            if ch == 'a':
                ops.append(('S', 0, mate, i))
            elif ch == 'b':
                ops.append(('S', 1, mate, i))
                dead['K'].append(i)
                dead['Q'].append(i)
            elif ch == 'p':
                if t > 0:
                    ops.append(('P', 1, order[t - 1]))
                    oq.append(order[t - 1])
                    dead['V'].append(order[t - 1])
            elif ch == 'q':
                ops.append(('P', 0, i))
            elif ch in 'KVQ':
                if dead[ch]:
                    ops.append((ch, dead[ch].pop(0)))
            elif ch == 'O':
                if len(oq) >= ODEL:
                    ops.append(('O', oq.pop(0)))
    rest = [(k, j) for k in TAILO for j in dead[k]]
    ops += rest[:1] + [('P', 1, order[-1])] + rest[1:]
    ops += [('O', i) for i in oq] + [('V', order[-1]), ('O', order[-1])]
    return ops


def _schedule_last(nblk, extras):
    need = max(n for _, n in extras)
    if ORDL:
        order = [int(v) for v in ORDL.split(',')]
    else:
        small, big = list(range(need)), list(range(nblk - 1, need - 1, -1))
        order = []
        while small or big:
            if big:
                order.append(big.pop(0))
            if small:
                order.append(small.pop(0))
    ops, oq, odone = [], [], set()
    extras = list(extras)

    def ready():
        return extras and set(range(extras[0][1])) <= odone
    for t, i in enumerate(order):
        mate = order[t + 1] if t % 2 == 0 else None
        for ch in TPL2:
            if ch == 'a':
                ops.append(('S', 0, mate, i))
            elif ch == 'b':
                ops.append(('S', 1, mate, i))
            elif ch == 'p':
                if t > 0:
                    ops.append(('P', 1, order[t - 1]))
                    oq.append(order[t - 1])
            elif ch == 'q':
                ops.append(('P', 0, i))
            elif ch == 'e':
                if ready() and (t >= T0 or extras[0][1] == 0):
                    ops.append(('E', extras.pop(0)[0]))
            elif ch == 'O':
                if len(oq) >= OD2:
                    odone.add(oq[0])
                    ops.append(('O', oq.pop(0)))
    tail = [('P', 1, order[-1])] + [('O', i) for i in oq + [order[-1]]]
    for op in tail:
        if ready():
            ops.append(('E', extras.pop(0)[0]))
        ops.append(op)
        if op[0] == 'O':
            odone.add(op[1])
    ops += [('E', n) for n, _ in extras]
    return ops


def _kernel(x_hbm, ckv_hbm, wq_hbm, wk_hbm, wv_hbm, wo_hbm, w1_hbm, w2_hbm, w3_hbm, w4_hbm,
            c_hbm, wmod_hbm, o_hbm,
            x_ref, ckv_ref, w1_ref, w2_ref, w3_ref, w4_ref, c_ref, wmod_ref,
            wq_buf, wk_buf, wv_buf, wo_buf,
            mod_ref, h_ref, q_ref, k_ref, v_ref, acc_ref, base_ref, hh_ref, h2_ref, z_ref, o_buf,
            wkv_ref, wqs_ref,
            wsem, isem, xsem, csem,
            *, S, M, Dc, H, D, F):
    npairs = H // 2
    nchunks = S // TR
    nblk = S // T
    qscale = (D ** -0.5) * math.log2(math.e)

    def w_copies(pair, sl):
        return [
            pltpu.make_async_copy(src.bitcast(U32).at[:, pair, :], dst.at[sl], wsem.at[j, sl])
            for j, (src, dst) in enumerate(((wk_hbm, wk_buf), (wv_hbm, wv_buf), (wq_hbm, wq_buf)))
        ]

    def wo_copy(pair, sl):
        return pltpu.make_async_copy(wo_hbm.at[pair], wo_buf.at[sl], wsem.at[3, sl])

    def late_copies():
        return [
            pltpu.make_async_copy(wmod_hbm.at[:, 2 * M:6 * M], wmod_ref.at[:, 2 * M:6 * M], isem.at[3]),
            pltpu.make_async_copy(w1_hbm.bitcast(U32), w1_ref, isem.at[4]),
            pltpu.make_async_copy(w2_hbm.bitcast(U32), w2_ref, isem.at[5]),
            pltpu.make_async_copy(w3_hbm.bitcast(U32), w3_ref, isem.at[6]),
            pltpu.make_async_copy(w4_hbm.bitcast(U32), w4_ref, isem.at[7]),
        ]

    def silu_c():
        c = c_ref[...].astype(F32)
        sc = c * (1.0 / (1.0 + jnp.exp(-c)))
        return jnp.broadcast_to(sc, (8, M)).astype(BF16)

    def store_heads(dst, rows, y):
        for hh in range(2):
            dst[hh, rows, :] = y[:, hh * D:(hh + 1) * D].astype(BF16)

    @jax.named_scope('prologue')
    def prologue():
        na = min(NA, nchunks - 1)
        kr = (nchunks - na) * TR // NB
        xr = S // NB
        cp_c = pltpu.make_async_copy(c_hbm, c_ref, isem.at[0])
        cp_mod = pltpu.make_async_copy(wmod_hbm.at[:, 0:2 * M], wmod_ref.at[:, 0:2 * M], isem.at[1])

        def ca_copy(i):
            rows = pl.ds(pl.multiple_of(i * TR, TR), TR)
            return pltpu.make_async_copy(ckv_hbm.at[rows, :], ckv_ref.at[rows, :], csem.at[i])

        def b_copies(i):
            rc = pl.ds(pl.multiple_of(na * TR + i * kr, kr), kr)
            rx = pl.ds(pl.multiple_of(i * xr, xr), xr)
            return [pltpu.make_async_copy(ckv_hbm.at[rc, :], ckv_ref.at[rc, :], csem.at[na + i]),
                    pltpu.make_async_copy(x_hbm.at[rx, :], x_ref.at[rx, :], xsem.at[i])]

        w0 = w_copies(0, 1)
        w0[0].start()
        w0[1].start()
        ca_copy(0).start()

        def zero(i, _):
            acc_ref[pl.ds(pl.multiple_of(i * T, T), T), :] = jnp.zeros((T, M), F32)
            return 0
        lax.fori_loop(0, nblk, zero, 0)
        acc_ref[S:S + HALO, :] = jnp.zeros((HALO, M), F32)
        x_ref[S:S + HALO, :] = jnp.zeros((HALO, M), BF16)
        hh_ref[:, 0:PAD, :] = jnp.zeros((M // T, PAD, T), F32)
        half = na // 2
        for cp in ([ca_copy(i) for i in range(1, half)] + [cp_c, cp_mod]
                   + [ca_copy(i) for i in range(half, na)] + [w0[2]] + b_copies(0)):
            cp.start()
        w0[0].wait()
        w0[1].wait()
        wkv_ref[:, 0:2 * D] = pltpu.bitcast(_unpack_pair(wk_buf[1]), U32)
        wkv_ref[:, 2 * D:4 * D] = pltpu.bitcast(_unpack_pair(wv_buf[1]), U32)

        def kv_proj(rows, which):
            w = pltpu.bitcast(wkv_ref[:, which * 2 * D:(which + 1) * 2 * D], BF16)
            store_heads(v_ref if which else k_ref, rows, _dot(ckv_ref[rows, :], w))

        def phase_a(i, _):
            ca_copy(i).wait()
            rows = pl.ds(pl.multiple_of(i * TR, TR), TR)
            kv_proj(rows, 0)
            kv_proj(rows, 1)
            return 0
        lax.fori_loop(0, na, phase_a, 0)
        for cp in b_copies(1):
            cp.start()
        cp_c.wait()
        cp_mod.wait()
        w0[2].wait()
        mod_ref[:, 0:2 * M] = _dot(silu_c(), wmod_ref[:, 0:2 * M])
        wqs_ref[...] = pltpu.bitcast(_unpack_pair(wq_buf[1]), U32)

        def phase_b(i, _):
            for cp in b_copies(i):
                cp.wait()

            @pl.when(i + 2 < NB)
            def _():
                for cp in b_copies(i + 2):
                    cp.start()

            @pl.when(i == 1)
            def _():
                for cp in w_copies(1, 0) + [wo_copy(0, 0)]:
                    cp.start()
            rows = pl.ds(pl.multiple_of(na * TR + i * kr, kr), kr)
            sa = mod_ref[0:1, 0:M]
            ca1 = 1.0 + mod_ref[0:1, M:2 * M]
            n = xr // PB.count('q')
            j = 0
            for ch in PB:
                if ch in 'kv':
                    kv_proj(rows, 'kv'.index(ch))
                else:
                    rx = pl.ds(pl.multiple_of(i * xr + j * n, n), n)
                    j += 1
                    h = (_ln(x_ref[rx, :].astype(F32)) * ca1 + sa).astype(BF16)
                    h_ref[rx, :] = h
                    store_heads(q_ref, rx, _dot(h, pltpu.bitcast(wqs_ref[...], BF16)) * qscale)
            return 0
        lax.fori_loop(0, NB, phase_b, 0)
        for cp in w_copies(2, 1) + [wo_copy(1, 1)] + late_copies():
            cp.start()

    def run_ops(ops, slot, w=None, extras=None):
        row = lax.broadcasted_iota(jnp.int32, (T, T), 0)
        col = lax.broadcasted_iota(jnp.int32, (T, T), 1)
        tri = col <= row
        HT = T // 2
        low_lanes = lax.broadcasted_iota(jnp.int32, (HT, T), 1) < HT
        left = {}

        def scores_of(hh, mate, i):
            r = i * T
            for ch in SORD:
                if ch == 's' and i >= 1:
                    ks = jnp.concatenate([k_ref[hh, r:r + HT, :], k_ref[hh, HT:T, :]], axis=0)
                    top = _dot_nt(q_ref[hh, r:r + HT, :], ks)
                elif ch == 'm' and i >= 2:
                    mid = _dot_nt(q_ref[hh, r:r + T, :], k_ref[hh, T:r, :])
                elif ch == 'b':
                    kb = k_ref[hh, 0:T, :]
                    if i >= 1:
                        kb = jnp.concatenate([kb, k_ref[hh, r:r + T, :]], axis=0)
                    bot = _dot_nt(q_ref[hh, r + HT:r + T, :], kb)
                elif ch == 'l' and mate is not None:
                    qt = jnp.concatenate([q_ref[hh, j * T:j * T + HT, :] for j in (i, mate)], axis=0)
                    lt = _dot_nt(k_ref[hh, 0:HT, :], qt)
                    lt = jnp.concatenate([lt, lt], axis=0).T
                    left[hh, i], left[hh, mate] = lt[:HT], lt[HT:]
            lf = left.pop((hh, i))
            if i == 0:
                return jnp.where(tri, jnp.concatenate([lf, bot], axis=0), NEG)
            first = jnp.concatenate([jnp.where(low_lanes, lf, top), bot[:, :T]], axis=0)
            diag = jnp.where(tri, jnp.concatenate([top, bot[:, T:]], axis=0), NEG)
            return jnp.concatenate([first] + ([mid] if i >= 2 else []) + [diag], axis=1)

        scores, ctx = {}, {}
        for op in ops:
            kind, i = op[0], op[-1]
            if kind == 'E':
                extras[i]()
                continue
            rows = slice(i * T, (i + 1) * T)
            if kind == 'K':
                store_heads(k_ref, rows, _dot(ckv_ref[rows, :], w['K']))
            elif kind == 'V':
                store_heads(v_ref, rows, _dot(ckv_ref[rows, :], w['V']))
            elif kind == 'Q':
                store_heads(q_ref, rows, _dot(h_ref[rows, :], w['Q']) * qscale)
            elif kind == 'S':
                scores[op[1], i] = scores_of(op[1], op[2], i)
            elif kind == 'P':
                hh = op[1]
                p, l = _softmax_rows(scores.pop((hh, i)))
                ctx[hh, i] = (_dot(p, v_ref[hh, 0:(i + 1) * T, :]) * _recip(l)).astype(BF16)
            else:
                c = jnp.concatenate([ctx.pop((0, i)), ctx.pop((1, i))], axis=1)
                acc_ref[rows, :] += _dot(c, wo_buf[slot])
        assert not scores and not ctx and not left

    @jax.named_scope('body')
    def step(g, _):
        slot = g & 1
        wo_copy(g, slot).wait()
        for cp in w_copies(g + 1, slot):
            cp.wait()
        w = {'K': _unpack_pair(wk_buf[slot]), 'V': _unpack_pair(wv_buf[slot]), 'Q': _unpack_pair(wq_buf[slot])}
        run_ops(_schedule(nblk), slot, w)

        @pl.when(g + 3 < npairs)
        def _():
            for cp in w_copies(g + 3, slot):
                cp.start()

        @pl.when(g + 2 < npairs)
        def _():
            wo_copy(g + 2, slot).start()
        return 0

    @jax.named_scope('epilogue')
    def epilogue():
        slot = (npairs - 1) % 2
        wo_copy(npairs - 1, slot).wait()
        for cp in late_copies():
            cp.wait()
        nct = M // T
        cgrp = M // 4
        shifts = (-1, 1, -2, 2)
        HR = TR // 2
        sc = silu_c()

        def mod_piece(j):
            wd = 4 * M // MODP
            cols = slice(2 * M + j * wd, 2 * M + (j + 1) * wd)
            mod_ref[:, cols] = _dot(sc, wmod_ref[:, cols])

        def mvec(j):
            return mod_ref[0:1, j * M:(j + 1) * M]

        def x1_of(rows):
            return x_ref[rows, :].astype(F32) + mvec(2) * acc_ref[rows, :]

        def mix_in(r0, k, n, may_overrun):
            rows = pl.ds(r0 + k, n)
            h2 = _ln(x1_of(rows)) * (1.0 + mvec(4)) + mvec(3)
            h2_ref[k:k + n, :] = h2
            hh = _gelu(_dot(_ln(h2).astype(BF16), _rows_bf16(w1_ref)))
            if may_overrun:
                rid = r0 + k + lax.broadcasted_iota(jnp.int32, (n, M), 0)
                hh = jnp.where(rid < S, hh, 0.0)
            for t in range(nct):
                hh_ref[t, PAD + k:PAD + k + n, :] = hh[:, t * T:(t + 1) * T]

        def mix_out(r0, k, n):
            lane = lax.broadcasted_iota(jnp.int32, (n, T), 1)
            cols = []
            for t in range(nct):
                lo, hi = (t * T) // cgrp, (t * T + T - 1) // cgrp
                v = hh_ref[t, pl.ds(PAD + k + shifts[lo], n), :]
                if hi != lo:
                    v2 = hh_ref[t, pl.ds(PAD + k + shifts[hi], n), :]
                    v = jnp.where(lane < hi * cgrp - t * T, v, v2)
                cols.append(v)
            sh = jnp.concatenate(cols, axis=1).astype(BF16)
            rows = pl.ds(r0 + k, n)
            y1 = h2_ref[k:k + n, :] + _dot(sh, _rows_bf16(w2_ref))
            base_ref[rows, :] = x1_of(rows) + mvec(5) * y1
            z_ref[k:k + n, :] = _ln(y1).astype(BF16)

        def ffn_up(k, n):
            z = z_ref[k:k + n, :]
            fm = (F // T) * T
            if fm == F:
                return _gelu(_dot_nt(z, _rows_bf16(w3_ref))).astype(BF16)
            tail = _gelu(_dot_nt(_rows_bf16(w3_ref, fm, F), z)).T
            main = _gelu(_dot_nt(z, _rows_bf16(w3_ref, 0, fm)))
            return jnp.concatenate([main, tail], axis=1).astype(BF16)

        def ffn_down(r, t):
            rows = pl.ds(r, t.shape[0])
            o_buf[rows, :] = (base_ref[rows, :] + mvec(5) * _dot(t, _rows_bf16(w4_ref))).astype(o_buf.dtype)

        def o_copy(r, n, sem):
            return pltpu.make_async_copy(o_buf.at[pl.ds(r, n), :], o_hbm.at[pl.ds(r, n), :], sem)

        def chunk_pieces(i, r, rn, overrun):
            t = {}

            def up0():
                hh_ref[:, 0:PAD + HALO, :] = hh_ref[:, TR:TR + PAD + HALO, :]
                h2_ref[0:HALO, :] = h2_ref[TR:TR + HALO, :]
                t[0] = ffn_up(0, HR)

            def up1():
                t[1] = ffn_up(HR, HR)

            def down1():
                ffn_down(r + HR, t[1])
                if not NOST:
                    o_copy(r, TR, xsem.at[i]).start()
            return [(up0, 0), (lambda: mix_in(rn, HALO, HR, False), HALO + HR), (up1, 0),
                    (lambda: mix_out(rn, 0, HR), 0), (lambda: mix_in(rn, HALO + HR, HR, overrun), HALO + TR),
                    (lambda: ffn_down(r, t[0]), 0), (lambda: mix_out(rn, HR, HR), 0), (down1, 0)]

        blocks = lambda rows: min(nblk, -(-rows // T))
        pieces = [(functools.partial(mod_piece, j), 0) for j in range(MODP)]
        pieces += [(lambda: mix_in(0, 0, HR, False), blocks(HR)), (lambda: mix_in(0, HR, HR + HALO, False), blocks(TR + HALO)),
                   (lambda: mix_out(0, 0, HR), 1), (lambda: mix_out(0, HR, HR), 1)]
        peel = min(PEEL, nchunks - 1)
        for i in range(peel):
            rn = (i + 1) * TR
            pieces += [(f, blocks(rn + n) if n else 1) for f, n in chunk_pieces(i, i * TR, rn, rn + TR + HALO > S)]
        with jax.named_scope('laststep'):
            run_ops(_schedule_last(nblk, [(j, n) for j, (_, n) in enumerate(pieces)]), slot,
                    extras=[f for f, _ in pieces])

        def body(i, _):
            r = pl.multiple_of(i * TR, TR)
            for f, _n in chunk_pieces(i, r, pl.multiple_of(r + TR, TR), True):
                f()
            return 0
        if peel < nchunks - 1:
            with jax.named_scope('eloop'):
                lax.fori_loop(peel, nchunks - 1, body, 0, unroll=EU)

        if NOST:
            for i in range(nchunks - 1):
                o_copy(i * TR, TR, xsem.at[i]).start()
        r = (nchunks - 1) * TR
        n1 = TR - LAST
        cp_a = o_copy(r, n1, xsem.at[nchunks - 1])
        cp_b = o_copy(r + n1, LAST, isem.at[0])
        t = ffn_up(0, TR)
        ffn_down(r, t[:n1])
        cp_a.start()
        ffn_down(r + n1, t[n1:])
        cp_b.start()
        for i in range(nchunks - 1):
            o_copy(i * TR, TR, xsem.at[i]).wait()
        cp_a.wait()
        cp_b.wait()

    prologue()
    with jax.named_scope('loop'):
        lax.fori_loop(0, npairs - 1, step, 0)
    epilogue()


@jax.jit
def pallas_adaLN_cond__compressed_kv_cla__mixer_s_mlp__prompt_kernel(
    A_x, A_c_kv, A_w_q, A_w_uk, A_w_uv, A_w_o, B_x, B_w1, B_w2, B_w3, B_w4, c, w_mod,
):
    del B_x
    _, S, M = A_x.shape
    Dc = A_c_kv.shape[2]
    H, D = A_w_q.shape[1], A_w_q.shape[2]
    F = B_w3.shape[1]
    ins = (A_x.reshape(S, M), A_c_kv.reshape(S, Dc), A_w_q, A_w_uk, A_w_uv,
           A_w_o.reshape(H // 2, 2 * D, M), B_w1, B_w2, B_w3.T, B_w4, c, w_mod)

    out = pl.pallas_call(
        functools.partial(_kernel, S=S, M=M, Dc=Dc, H=H, D=D, F=F),
        in_specs=[pl.BlockSpec(memory_space=pl.ANY) for _ in ins],
        out_specs=pl.BlockSpec(memory_space=pl.ANY),
        out_shape=jax.ShapeDtypeStruct((S, M), A_x.dtype),
        scratch_shapes=[
            pltpu.VMEM((S + HALO, M), BF16),
            pltpu.VMEM((S, Dc), BF16),
            pltpu.VMEM((M // 2, M), U32),
            pltpu.VMEM((M // 2, M), U32),
            pltpu.VMEM((F // 2, M), U32),
            pltpu.VMEM((F // 2, M), U32),
            pltpu.VMEM((1, M), BF16),
            pltpu.VMEM((M, 6 * M), BF16),
            pltpu.VMEM((2, M, D), U32),
            pltpu.VMEM((2, Dc, D), U32),
            pltpu.VMEM((2, Dc, D), U32),
            pltpu.VMEM((2, 2 * D, M), BF16),
            pltpu.VMEM((8, 6 * M), F32),
            pltpu.VMEM((S, M), BF16),
            pltpu.VMEM((2, S, D), BF16),
            pltpu.VMEM((2, S, D), BF16),
            pltpu.VMEM((2, S, D), BF16),
            pltpu.VMEM((S + HALO, M), F32),
            pltpu.VMEM((S, M), F32),
            pltpu.VMEM((M // T, PAD + TR + HALO, T), F32),
            pltpu.VMEM((TR + HALO, M), F32),
            pltpu.VMEM((TR, M), BF16),
            pltpu.VMEM((S, M), A_x.dtype),
            pltpu.VMEM((Dc // 2, 4 * D), U32),
            pltpu.VMEM((M // 2, 2 * D), U32),
            pltpu.SemaphoreType.DMA((4, 2)),
            pltpu.SemaphoreType.DMA((8,)),
            pltpu.SemaphoreType.DMA((max(S // TR, NB),)),
            pltpu.SemaphoreType.DMA((S // TR + NB,)),
        ],
        compiler_params=pltpu.CompilerParams(
            vmem_limit_bytes=100 * 1024 * 1024,
            disable_bounds_checks=True,
        ),
    )(*ins)
    return out.reshape(1, S, M)
```

```python
import functools
import math

import jax
import jax.numpy as jnp
from jax import lax
import jax.experimental.pallas as pl
import jax.experimental.pallas.tpu as pltpu

F32 = jnp.float32
BF16 = jnp.bfloat16
U32 = jnp.uint32
EPS = 1e-5
NEG = -1e30
T = 128
G = 32
NG = T // G
TR = 256
PAD = 8
HALO = 16
NA = 6
NB = 4
MODP = 10
LAST = 64


def _ln(x):
    m = jnp.mean(x, axis=-1, keepdims=True)
    xc = x - m
    v = jnp.mean(xc * xc, axis=-1, keepdims=True)
    return xc * lax.rsqrt(v + EPS)


def _gelu(x):
    c = math.sqrt(2.0 / math.pi)
    hx = 0.5 * x
    return hx + hx * jnp.tanh(x * (c + (c * 0.044715) * (x * x)))


def _dot(a, b):
    return jnp.dot(a, b, preferred_element_type=F32)


def _dot_nt(a, b):
    return lax.dot_general(a, b, (((1,), (1,)), ((), ())), preferred_element_type=F32)


def _recip(l):
    r = pl.reciprocal(l, approx=True)
    return r * (2.0 - l * r)


def _unpack_pair(u, axis=1):
    lo = pltpu.bitcast(u << 16, F32)
    hi = pltpu.bitcast(u & jnp.uint32(0xFFFF0000), F32)
    return jnp.concatenate([lo, hi], axis=axis).astype(BF16)


def _bf(u):
    return pltpu.bitcast(u, BF16)


def _pk(x):
    return pltpu.bitcast(x.astype(BF16), U32)


def _softmax_rows(s):
    m = jnp.max(s, axis=-1, keepdims=True)
    p = jnp.exp2(s - m).astype(BF16)
    return p, jnp.sum(p.astype(F32), axis=-1, keepdims=True)


def _schedule(nblk):
    order = list(range(nblk - 1, -1, -1))
    ops, oq, kq, vq = [], [], [], []
    for t, i in enumerate(order):
        mates = tuple(order[t:t + NG]) if t % NG == 0 else None
        ops.append(('S', 0, mates, i))
        ops += [('K', kq.pop())] if kq else []
        ops += [('V', vq.pop())] if vq else []
        if t > 0:
            ops.append(('P', 1, order[t - 1]))
            oq.append(order[t - 1])
            vq.append(order[t - 1])
        ops += [('S', 1, mates, i), ('Q', i)]
        kq.append(i)
        if len(oq) >= 3:
            ops.append(('O', oq.pop(0)))
        ops.append(('P', 0, i))
    ops += [('K', kq.pop()), ('P', 1, 0), ('V', vq.pop())]
    ops += [('O', i) for i in oq] + [('V', 0), ('O', 0)]
    return ops


def _schedule_last(nblk, extras):
    small, big = list(range(max(extras))), list(range(nblk - 1, max(extras) - 1, -1))
    order = []
    while small or big:
        order += [big.pop(0)] if big else []
        order += [small.pop(0)] if small else []
    ops, oq, final = [], [], set()
    todo = list(enumerate(extras))

    def extra(allow_rows):
        if todo and (todo[0][1] == 0 or (allow_rows and set(range(todo[0][1])) <= final)):
            ops.append(('E', todo.pop(0)[0]))
    for t, i in enumerate(order):
        mates = tuple(order[t:t + NG]) if t % NG == 0 else None
        ops.append(('S', 0, mates, i))
        extra(False)
        if t > 0:
            ops.append(('P', 1, order[t - 1]))
            oq.append(order[t - 1])
        ops.append(('S', 1, mates, i))
        extra(t >= nblk - 4)
        if len(oq) >= 2:
            final.add(oq[0])
            ops.append(('O', oq.pop(0)))
        ops.append(('P', 0, i))
    for op in [('P', 1, order[-1])] + [('O', i) for i in oq + [order[-1]]]:
        extra(True)
        ops.append(op)
        if op[0] == 'O':
            final.add(op[1])
    ops += [('E', j) for j, _ in todo]
    return ops


def _kernel(x_hbm, ckv_hbm, wq_hbm, wk_hbm, wv_hbm, wo_hbm, w1_hbm, w2_hbm, w3_hbm, w4_hbm,
            c_hbm, wmod_hbm, o_hbm,
            x_ref, ckv_ref, w1_ref, w2_ref, w3_ref, w4_ref, c_ref, wmod_ref,
            wq_buf, wk_buf, wv_buf, wo_buf,
            mod_ref, h_ref, q_ref, kt_ref, v_ref, acc_ref, base_ref, hh_ref, h2_ref, z_ref, o_buf,
            wks_ref, wvs_ref, wqs_ref, k0_ref,
            wsem, isem, xsem, csem,
            *, S, M, Dc, H, D, F):
    npairs = H // 2
    nchunks = S // TR
    nblk = S // T
    qscale = (D ** -0.5) * math.log2(math.e)

    def w_copies(pair, sl):
        return [
            pltpu.make_async_copy(src.bitcast(U32).at[:, pair, :], dst.at[sl], wsem.at[j, sl])
            for j, (src, dst) in enumerate(((wk_hbm, wk_buf), (wv_hbm, wv_buf), (wq_hbm, wq_buf)))
        ]

    def wo_copy(pair, sl):
        return pltpu.make_async_copy(wo_hbm.at[pair], wo_buf.at[sl], wsem.at[3, sl])

    def late_copies():
        return [
            pltpu.make_async_copy(wmod_hbm.at[:, 2 * M:6 * M], wmod_ref.at[:, 2 * M:6 * M], isem.at[2]),
            pltpu.make_async_copy(w1_hbm.bitcast(U32), w1_ref, isem.at[3]),
            pltpu.make_async_copy(w2_hbm.bitcast(U32), w2_ref, isem.at[4]),
            pltpu.make_async_copy(w3_hbm.bitcast(U32), w3_ref, isem.at[5]),
            pltpu.make_async_copy(w4_hbm.bitcast(U32), w4_ref, isem.at[6]),
        ]

    def silu_c():
        c = c_ref[...].astype(F32)
        sc = c * (1.0 / (1.0 + jnp.exp(-c)))
        return jnp.broadcast_to(sc, (8, M)).astype(BF16)

    def store_heads(dst, rows, y):
        for hh in range(2):
            dst[hh, rows, :] = y[:, hh * D:(hh + 1) * D].astype(BF16)

    def store_kt(blk, yt):
        for hh in range(2):
            for j in range(yt.shape[1] // T):
                tile = yt[hh * D:(hh + 1) * D, j * T:(j + 1) * T]
                kt_ref[hh, blk + j] = _pk(tile)
                if isinstance(blk, int) and blk + j == 0:
                    k0_ref[hh] = tile.T.astype(BF16)

    def prologue():
        na = min(NA, nchunks - 2)
        kr = (nchunks - na) * TR // NB
        xr = S // NB
        cp_c = pltpu.make_async_copy(c_hbm, c_ref, isem.at[0])
        cp_mod = pltpu.make_async_copy(wmod_hbm.at[:, 0:2 * M], wmod_ref.at[:, 0:2 * M], isem.at[1])

        def a_copy(i):
            rows = pl.ds(pl.multiple_of(i * TR, TR), TR)
            return pltpu.make_async_copy(ckv_hbm.at[rows, :], ckv_ref.at[rows, :], csem.at[i])

        def b_copies(i):
            rc = pl.ds(pl.multiple_of(na * TR + i * kr, kr), kr)
            rx = pl.ds(pl.multiple_of(i * xr, xr), xr)
            return [pltpu.make_async_copy(ckv_hbm.at[rc, :], ckv_ref.at[rc, :], csem.at[na + i]),
                    pltpu.make_async_copy(x_hbm.at[rx, :], x_ref.at[rx, :], xsem.at[i])]

        w0 = w_copies(0, 1)
        w0[0].start()
        w0[1].start()
        a_copy(0).start()

        def zero(i, _):
            acc_ref[pl.ds(pl.multiple_of(i * T, T), T), :] = jnp.zeros((T, M), F32)
            return 0
        lax.fori_loop(0, nblk, zero, 0)
        acc_ref[S:S + HALO, :] = jnp.zeros((HALO, M), F32)
        x_ref[S:S + HALO, :] = jnp.zeros((HALO, M), BF16)
        hh_ref[:, 0:PAD, :] = jnp.zeros((M // T, PAD, T), F32)
        for cp in ([a_copy(i) for i in range(1, na // 2)] + [cp_c, cp_mod]
                   + [a_copy(i) for i in range(na // 2, na)] + [w0[2]] + b_copies(0)):
            cp.start()
        w0[0].wait()
        w0[1].wait()
        wks_ref[...] = _pk(_unpack_pair(wk_buf[1].T, axis=0))
        wvs_ref[...] = _pk(_unpack_pair(wv_buf[1]))

        def k_proj(r, n):
            store_kt(r // T, _dot_nt(_bf(wks_ref[...]), ckv_ref[pl.ds(r, n), :]))

        def v_proj(r, n):
            store_heads(v_ref, pl.ds(r, n), _dot(ckv_ref[pl.ds(r, n), :], _bf(wvs_ref[...])))

        def phase_a(i, _):
            a_copy(i).wait()
            r = pl.multiple_of(i * TR, TR)
            v_proj(r, TR)
            k_proj(r, TR)
            return 0
        lax.fori_loop(0, na, phase_a, 0)
        for hh in range(2):
            k0_ref[hh] = _bf(kt_ref[hh, 0]).astype(F32).T.astype(BF16)
        for cp in b_copies(1):
            cp.start()
        cp_c.wait()
        cp_mod.wait()
        w0[2].wait()
        mod_ref[:, 0:2 * M] = _dot(silu_c(), wmod_ref[:, 0:2 * M])
        wqs_ref[...] = _pk(_unpack_pair(wq_buf[1]))

        def phase_b(i, _):
            for cp in b_copies(i):
                cp.wait()

            @pl.when(i + 2 < NB)
            def _():
                for cp in b_copies(i + 2):
                    cp.start()

            @pl.when(i == 1)
            def _():
                for cp in w_copies(1, 0) + [wo_copy(0, 0)]:
                    cp.start()
            rk = pl.multiple_of(na * TR + i * kr, kr)
            sa = mod_ref[0:1, 0:M]
            ca1 = 1.0 + mod_ref[0:1, M:2 * M]
            k_proj(rk, kr)
            v_proj(rk, kr)
            n = xr // 4
            for j in range(4):
                rx = pl.multiple_of(i * xr + j * n, n)
                h = (_ln(x_ref[pl.ds(rx, n), :].astype(F32)) * ca1 + sa).astype(BF16)
                h_ref[pl.ds(pl.multiple_of(rx // 2, 8), n // 2), :] = _pk(h)
                store_heads(q_ref, pl.ds(rx, n), _dot(h, _bf(wqs_ref[...])) * qscale)
            return 0
        lax.fori_loop(0, NB, phase_b, 0)
        for cp in w_copies(2, 1) + [wo_copy(1, 1)] + late_copies():
            cp.start()

    def run_ops(ops, slot, part_order, w=None, extras=None):
        row = lax.broadcasted_iota(jnp.int32, (T, T), 0)
        col = lax.broadcasted_iota(jnp.int32, (T, T), 1)
        tri = col <= row
        lane_w = lax.broadcasted_iota(jnp.int32, (D // 2, T), 1)
        lane_g = lax.broadcasted_iota(jnp.int32, (G, T), 1)
        left = {}

        def scores_of(hh, mates, i):
            r = i * T
            part = {}
            for ch in ('mlbs' if (hh, i) == (0, nblk - 1) else part_order):
                if ch == 'l' and mates is not None:
                    for g in range(NG - 1):
                        nk = (g + 1) * G
                        qt = jnp.concatenate([q_ref[hh, j * T + g * G:j * T + nk, :] for j in mates], axis=0)
                        lt = _dot_nt(k0_ref[hh, 0:nk, :], qt)
                        lt = jnp.concatenate([lt] + [lt[:G]] * (NG - 1 - g), axis=0).T
                        for n, j in enumerate(mates):
                            left[hh, j, g] = lt[n * G:(n + 1) * G]
                elif ch == 'm' and i >= 2:
                    km = _bf(jnp.concatenate([kt_ref[hh, j] for j in range(1, i)], axis=1))
                    part['m'] = _dot(q_ref[hh, r:r + T, :], km)
                elif ch == 'b':
                    qb = q_ref[hh, r + T - G:r + T, :]
                    part['b', 0] = _dot(qb, _bf(kt_ref[hh, 0]))
                    if i >= 1:
                        part['b', 1] = _dot(qb, _bf(kt_ref[hh, i]))
                elif ch == 's' and i >= 1:
                    for g in range(NG - 1):
                        nk = (g + 1) * G
                        ks = _bf(jnp.where(lane_w < nk, kt_ref[hh, i], kt_ref[hh, 0]))
                        part['s', g] = _dot(q_ref[hh, r + g * G:r + nk, :], ks)
            lf = [left.pop((hh, i, g)) for g in range(NG - 1)]
            if i == 0:
                return jnp.where(tri, jnp.concatenate(lf + [part['b', 0]], axis=0), NEG)
            first = jnp.concatenate(
                [jnp.where(lane_g < (g + 1) * G, lf[g], part['s', g]) for g in range(NG - 1)]
                + [part['b', 0]], axis=0)
            diag = jnp.concatenate([part['s', g] for g in range(NG - 1)] + [part['b', 1]], axis=0)
            diag = jnp.where(tri, diag, NEG)
            return jnp.concatenate([first] + ([part['m']] if i >= 2 else []) + [diag], axis=1)

        scores, ctx = {}, {}
        for op in ops:
            kind, i = op[0], op[-1]
            rows = slice(i * T, (i + 1) * T)
            if kind == 'E':
                extras[i]()
            elif kind == 'K':
                store_kt(i, _dot_nt(w['K'], ckv_ref[rows, :]))
            elif kind == 'V':
                store_heads(v_ref, rows, _dot(ckv_ref[rows, :], w['V']))
            elif kind == 'Q':
                h = _bf(h_ref[i * T // 2:(i + 1) * T // 2, :])
                store_heads(q_ref, rows, _dot(h, w['Q']) * qscale)
            elif kind == 'S':
                scores[op[1], i] = scores_of(op[1], op[2], i)
            elif kind == 'P':
                hh = op[1]
                p, l = _softmax_rows(scores.pop((hh, i)))
                ctx[hh, i] = (_dot(p, v_ref[hh, 0:(i + 1) * T, :]) * _recip(l)).astype(BF16)
            else:
                c = jnp.concatenate([ctx.pop((0, i)), ctx.pop((1, i))], axis=1)
                acc_ref[rows, :] += _dot(c, wo_buf[slot])
        assert not scores and not ctx and not left

    def step(g, _):
        slot = g & 1
        wo_copy(g, slot).wait()
        for cp in w_copies(g + 1, slot):
            cp.wait()
        w = {'K': _unpack_pair(wk_buf[slot].T, axis=0), 'V': _unpack_pair(wv_buf[slot]),
             'Q': _unpack_pair(wq_buf[slot])}
        run_ops(_schedule(nblk), slot, 'lbsm', w=w)

        @pl.when(g + 3 < npairs)
        def _():
            for cp in w_copies(g + 3, slot):
                cp.start()

        @pl.when(g + 2 < npairs)
        def _():
            wo_copy(g + 2, slot).start()
        return 0

    def epilogue():
        slot = (npairs - 1) % 2
        wo_copy(npairs - 1, slot).wait()
        for cp in late_copies():
            cp.wait()
        nct = M // T
        cgrp = M // 4
        shifts = (-1, 1, -2, 2)
        HR = TR // 2
        sc = silu_c()
        hoisted = {}

        def mod_piece(j):
            wd = 4 * M // MODP
            cols = slice(2 * M + j * wd, 2 * M + (j + 1) * wd)
            mod_ref[:, cols] = _dot(sc, wmod_ref[:, cols])

        def mvec(j):
            if j in hoisted:
                return hoisted[j]
            v = mod_ref[0:1, j * M:(j + 1) * M]
            return 1.0 + v if j == 4 else v

        def x1_of(rows):
            return x_ref[rows, :].astype(F32) + mvec(2) * acc_ref[rows, :]

        def mix_in(r0, k, n, may_overrun):
            rows = pl.ds(r0 + k, n)
            h2 = _ln(x1_of(rows)) * mvec(4) + mvec(3)
            h2_ref[k:k + n, :] = h2
            hh = _gelu(_dot(_ln(h2).astype(BF16), _bf(w1_ref[...])))
            if may_overrun:
                rid = r0 + k + lax.broadcasted_iota(jnp.int32, (n, M), 0)
                hh = jnp.where(rid < S, hh, 0.0)
            for t in range(nct):
                hh_ref[t, PAD + k:PAD + k + n, :] = hh[:, t * T:(t + 1) * T]

        def mix_out(r0, k, n):
            lane = lax.broadcasted_iota(jnp.int32, (n, T), 1)
            cols = []
            for t in range(nct):
                lo, hi = (t * T) // cgrp, (t * T + T - 1) // cgrp
                v = hh_ref[t, pl.ds(PAD + k + shifts[lo], n), :]
                if hi != lo:
                    v2 = hh_ref[t, pl.ds(PAD + k + shifts[hi], n), :]
                    v = jnp.where(lane < hi * cgrp - t * T, v, v2)
                cols.append(v)
            sh = jnp.concatenate(cols, axis=1).astype(BF16)
            rows = pl.ds(r0 + k, n)
            y1 = h2_ref[k:k + n, :] + _dot(sh, _bf(w2_ref[...]))
            base_ref[rows, :] = x1_of(rows) + mvec(5) * y1
            z_ref[k:k + n, :] = _ln(y1).astype(BF16)

        def ffn_up(k, n):
            z = z_ref[k:k + n, :]
            fm = (F // T) * T
            if fm == F:
                return _gelu(_dot_nt(z, _bf(w3_ref[...]))).astype(BF16)
            tail = _gelu(_dot_nt(_bf(w3_ref[fm // 2:F // 2, :]), z)).T
            main = _gelu(_dot_nt(z, _bf(w3_ref[0:fm // 2, :])))
            return jnp.concatenate([main, tail], axis=1).astype(BF16)

        def ffn_down(r, t):
            rows = pl.ds(r, t.shape[0])
            o_buf[rows, :] = (base_ref[rows, :] + mvec(5) * _dot(t, _bf(w4_ref[...]))).astype(o_buf.dtype)

        def o_copy(r, n, sem):
            return pltpu.make_async_copy(o_buf.at[pl.ds(r, n), :], o_hbm.at[pl.ds(r, n), :], sem)

        pieces = [(functools.partial(mod_piece, j), 0) for j in range(MODP)]
        pieces += [(functools.partial(mix_in, 0, 0, HR, False), pl.cdiv(HR, T)),
                   (functools.partial(mix_in, 0, HR, HR + HALO, False), pl.cdiv(TR + HALO, T)),
                   (functools.partial(mix_out, 0, 0, HR), 1),
                   (functools.partial(mix_out, 0, HR, HR), 1)]
        run_ops(_schedule_last(nblk, [n for _, n in pieces]), slot, 'smbl', extras=[f for f, _ in pieces])
        hoisted.update({j: mvec(j) for j in range(2, 6)})

        def body(i, _):
            r = pl.multiple_of(i * TR, TR)
            rn = pl.multiple_of(r + TR, TR)
            hh_ref[:, 0:PAD + HALO, :] = hh_ref[:, TR:TR + PAD + HALO, :]
            h2_ref[0:HALO, :] = h2_ref[TR:TR + HALO, :]
            t0 = ffn_up(0, HR)
            mix_in(rn, HALO, HR, False)
            t1 = ffn_up(HR, HR)
            mix_out(rn, 0, HR)
            mix_in(rn, HALO + HR, HR, True)
            ffn_down(r, t0)
            mix_out(rn, HR, HR)
            ffn_down(r + HR, t1)
            o_copy(r, TR, xsem.at[i]).start()
            return 0
        lax.fori_loop(0, nchunks - 1, body, 0)

        r = (nchunks - 1) * TR
        n1 = TR - LAST
        cp_a = o_copy(r, n1, xsem.at[nchunks - 1])
        cp_b = o_copy(r + n1, LAST, isem.at[0])
        t = ffn_up(0, TR)
        ffn_down(r, t[:n1])
        cp_a.start()
        ffn_down(r + n1, t[n1:])
        cp_b.start()
        for i in range(nchunks - 1):
            o_copy(i * TR, TR, xsem.at[i]).wait()
        cp_a.wait()
        cp_b.wait()

    prologue()
    lax.fori_loop(0, npairs - 1, step, 0)
    epilogue()


@jax.jit
def pallas_adaLN_cond__compressed_kv_cla__mixer_s_mlp__prompt_kernel(
    A_x, A_c_kv, A_w_q, A_w_uk, A_w_uv, A_w_o, B_x, B_w1, B_w2, B_w3, B_w4, c, w_mod,
):
    del B_x
    _, S, M = A_x.shape
    Dc = A_c_kv.shape[2]
    H, D = A_w_q.shape[1], A_w_q.shape[2]
    F = B_w3.shape[1]
    ins = (A_x.reshape(S, M), A_c_kv.reshape(S, Dc), A_w_q, A_w_uk, A_w_uv,
           A_w_o.reshape(H // 2, 2 * D, M), B_w1, B_w2, B_w3.T, B_w4, c, w_mod)

    out = pl.pallas_call(
        functools.partial(_kernel, S=S, M=M, Dc=Dc, H=H, D=D, F=F),
        in_specs=[pl.BlockSpec(memory_space=pl.ANY) for _ in ins],
        out_specs=pl.BlockSpec(memory_space=pl.ANY),
        out_shape=jax.ShapeDtypeStruct((S, M), A_x.dtype),
        scratch_shapes=[
            pltpu.VMEM((S + HALO, M), BF16),
            pltpu.VMEM((S, Dc), BF16),
            pltpu.VMEM((M // 2, M), U32),
            pltpu.VMEM((M // 2, M), U32),
            pltpu.VMEM((F // 2, M), U32),
            pltpu.VMEM((F // 2, M), U32),
            pltpu.VMEM((1, M), BF16),
            pltpu.VMEM((M, 6 * M), BF16),
            pltpu.VMEM((2, M, D), U32),
            pltpu.VMEM((2, Dc, D), U32),
            pltpu.VMEM((2, Dc, D), U32),
            pltpu.VMEM((2, 2 * D, M), BF16),
            pltpu.VMEM((8, 6 * M), F32),
            pltpu.VMEM((S // 2, M), U32),
            pltpu.VMEM((2, S, D), BF16),
            pltpu.VMEM((2, S // T, D // 2, T), U32),
            pltpu.VMEM((2, S, D), BF16),
            pltpu.VMEM((S + HALO, M), F32),
            pltpu.VMEM((S, M), F32),
            pltpu.VMEM((M // T, PAD + TR + HALO, T), F32),
            pltpu.VMEM((TR + HALO, M), F32),
            pltpu.VMEM((TR, M), BF16),
            pltpu.VMEM((S, M), A_x.dtype),
            pltpu.VMEM((D, Dc), U32),
            pltpu.VMEM((Dc // 2, 2 * D), U32),
            pltpu.VMEM((M // 2, 2 * D), U32),
            pltpu.VMEM((2, T, D), BF16),
            pltpu.SemaphoreType.DMA((4, 2)),
            pltpu.SemaphoreType.DMA((7,)),
            pltpu.SemaphoreType.DMA((max(S // TR, NB),)),
            pltpu.SemaphoreType.DMA((S // TR + NB,)),
        ],
        compiler_params=pltpu.CompilerParams(
            vmem_limit_bytes=100 * 1024 * 1024,
            disable_bounds_checks=True,
        ),
    )(*ins)
    return out.reshape(1, S, M)
```

```python
import functools
import math

import jax
import jax.numpy as jnp
from jax import lax
import jax.experimental.pallas as pl
import jax.experimental.pallas.tpu as pltpu

F32 = jnp.float32
BF16 = jnp.bfloat16
U32 = jnp.uint32
EPS = 1e-5
NEG = -1e30
T = 128
G = 32
NG = T // G
TR = 256
PAD = 8
HALO = 16
NA = 6
NB = 4
MODP = 10
LAST = 64


def _ln(x):
    m = jnp.mean(x, axis=-1, keepdims=True)
    xc = x - m
    v = jnp.mean(xc * xc, axis=-1, keepdims=True)
    return xc * lax.rsqrt(v + EPS)


def _gelu(x):
    c = math.sqrt(2.0 / math.pi)
    hx = 0.5 * x
    return hx + hx * jnp.tanh(x * (c + (c * 0.044715) * (x * x)))


def _dot(a, b):
    return jnp.dot(a, b, preferred_element_type=F32)


def _dot_nt(a, b):
    return lax.dot_general(a, b, (((1,), (1,)), ((), ())), preferred_element_type=F32)


def _recip(l):
    r = pl.reciprocal(l, approx=True)
    return r * (2.0 - l * r)


def _unpack_pair(u, axis=1):
    lo = pltpu.bitcast(u << 16, F32)
    hi = pltpu.bitcast(u & jnp.uint32(0xFFFF0000), F32)
    return jnp.concatenate([lo, hi], axis=axis).astype(BF16)


def _bf(u):
    return pltpu.bitcast(u, BF16)


def _pk(x):
    return pltpu.bitcast(x.astype(BF16), U32)


def _softmax_rows(s):
    m = jnp.max(s, axis=-1, keepdims=True)
    p = jnp.exp2(s - m).astype(BF16)
    return p, jnp.sum(p.astype(F32), axis=-1, keepdims=True)


def _schedule(nblk):
    order = list(range(nblk - 1, -1, -1))
    ops, oq, kq, vq = [], [], [], []
    for t, i in enumerate(order):
        mates = tuple(order[t:t + NG]) if t % NG == 0 else None
        ops.append(('S', 0, mates, i))
        ops += [('K', kq.pop())] if kq else []
        ops += [('V', vq.pop())] if vq else []
        if t > 0:
            ops.append(('P', 1, order[t - 1]))
            oq.append(order[t - 1])
            vq.append(order[t - 1])
        ops += [('S', 1, mates, i), ('Q', i)]
        kq.append(i)
        if len(oq) >= 3:
            ops.append(('O', oq.pop(0)))
        ops.append(('P', 0, i))
    ops += [('K', kq.pop()), ('P', 1, 0), ('V', vq.pop())]
    ops += [('O', i) for i in oq] + [('V', 0), ('O', T - G, 0)]
    return ops


def _schedule_last(nblk, extras):
    small, big = list(range(max(extras))), list(range(nblk - 1, max(extras) - 1, -1))
    order = []
    while small or big:
        order += [big.pop(0)] if big else []
        order += [small.pop(0)] if small else []
    ops, oq, final = [], [], set()
    todo = list(enumerate(extras))

    def extra(allow_rows):
        if todo and (todo[0][1] == 0 or (allow_rows and set(range(todo[0][1])) <= final)):
            ops.append(('E', todo.pop(0)[0]))
    for t, i in enumerate(order):
        mates = tuple(order[t:t + NG]) if t % NG == 0 else None
        ops.append(('S', 0, mates, i))
        extra(False)
        if t > 0:
            ops.append(('P', 1, order[t - 1]))
            oq.append(order[t - 1])
        ops.append(('S', 1, mates, i))
        extra(t >= nblk - 4)
        if len(oq) >= 2:
            final.add(oq[0])
            ops.append(('O', oq.pop(0)))
        ops.append(('P', 0, i))
    for op in [('P', 1, order[-1])] + [('O', i) for i in oq + [order[-1]]]:
        extra(True)
        ops.append(op)
        if op[0] == 'O':
            final.add(op[1])
    ops += [('E', j) for j, _ in todo]
    return ops


def _kernel(x_hbm, ckv_hbm, wq_hbm, wk_hbm, wv_hbm, wo_hbm, w1_hbm, w2_hbm, w3_hbm, w4_hbm,
            c_hbm, wmod_hbm, o_hbm,
            x_ref, ckv_ref, w1_ref, w2_ref, w3_ref, w4_ref, c_ref, wmod_ref,
            wq_buf, wk_buf, wv_buf, wo_buf,
            mod_ref, h_ref, q_ref, kt_ref, v_ref, acc_ref, base_ref, hh_ref, h2_ref, z_ref, o_buf,
            wks_ref, wvs_ref, wqs_ref, k0_ref,
            wsem, isem, xsem, csem,
            *, S, M, Dc, H, D, F):
    npairs = H // 2
    nchunks = S // TR
    nblk = S // T
    qscale = (D ** -0.5) * math.log2(math.e)

    def w_copies(pair, sl):
        return [
            pltpu.make_async_copy(src.bitcast(U32).at[:, pair, :], dst.at[sl], wsem.at[j, sl])
            for j, (src, dst) in enumerate(((wk_hbm, wk_buf), (wv_hbm, wv_buf), (wq_hbm, wq_buf)))
        ]

    def wo_copy(pair, sl):
        return pltpu.make_async_copy(wo_hbm.at[pair], wo_buf.at[sl], wsem.at[3, sl])

    def late_copies():
        return [
            pltpu.make_async_copy(wmod_hbm.at[:, 2 * M:6 * M], wmod_ref.at[:, 2 * M:6 * M], isem.at[2]),
            pltpu.make_async_copy(w1_hbm.bitcast(U32), w1_ref, isem.at[3]),
            pltpu.make_async_copy(w2_hbm.bitcast(U32), w2_ref, isem.at[4]),
            pltpu.make_async_copy(w3_hbm.bitcast(U32), w3_ref, isem.at[5]),
            pltpu.make_async_copy(w4_hbm.bitcast(U32), w4_ref, isem.at[6]),
        ]

    def silu_c():
        c = c_ref[...].astype(F32)
        sc = c * (1.0 / (1.0 + jnp.exp(-c)))
        return jnp.broadcast_to(sc, (8, M)).astype(BF16)

    def store_heads(dst, rows, y):
        for hh in range(2):
            dst[hh, rows, :] = y[:, hh * D:(hh + 1) * D].astype(BF16)

    def store_kt(blk, yt):
        for hh in range(2):
            for j in range(yt.shape[1] // T):
                tile = yt[hh * D:(hh + 1) * D, j * T:(j + 1) * T]
                kt_ref[hh, blk + j] = _pk(tile)
                if isinstance(blk, int) and blk + j == 0:
                    k0_ref[hh] = tile.T.astype(BF16)

    def prologue():
        na = min(NA, nchunks - 2)
        kr = (nchunks - na) * TR // NB
        xr = S // NB
        cp_c = pltpu.make_async_copy(c_hbm, c_ref, isem.at[0])
        cp_mod = pltpu.make_async_copy(wmod_hbm.at[:, 0:2 * M], wmod_ref.at[:, 0:2 * M], isem.at[1])

        def a_copy(i):
            rows = pl.ds(pl.multiple_of(i * TR, TR), TR)
            return pltpu.make_async_copy(ckv_hbm.at[rows, :], ckv_ref.at[rows, :], csem.at[i])

        def b_copies(i):
            rc = pl.ds(pl.multiple_of(na * TR + i * kr, kr), kr)
            rx = pl.ds(pl.multiple_of(i * xr, xr), xr)
            return [pltpu.make_async_copy(ckv_hbm.at[rc, :], ckv_ref.at[rc, :], csem.at[na + i]),
                    pltpu.make_async_copy(x_hbm.at[rx, :], x_ref.at[rx, :], xsem.at[i])]

        w0 = w_copies(0, 1)
        w0[0].start()
        w0[1].start()
        a_copy(0).start()

        def zero(i, _):
            acc_ref[pl.ds(pl.multiple_of(i * T, T), T), :] = jnp.zeros((T, M), F32)
            return 0
        lax.fori_loop(0, nblk, zero, 0)
        acc_ref[S:S + HALO, :] = jnp.zeros((HALO, M), F32)
        x_ref[S:S + HALO, :] = jnp.zeros((HALO, M), BF16)
        hh_ref[:, 0:PAD, :] = jnp.zeros((M // T, PAD, T), F32)
        for cp in ([a_copy(i) for i in range(1, na // 2)] + [cp_c, cp_mod]
                   + [a_copy(i) for i in range(na // 2, na)] + [w0[2]] + b_copies(0)):
            cp.start()
        w0[0].wait()
        w0[1].wait()
        wks_ref[...] = _pk(_unpack_pair(wk_buf[1].T, axis=0))
        wvs_ref[...] = _pk(_unpack_pair(wv_buf[1]))

        def k_proj(r, n):
            store_kt(r // T, _dot_nt(_bf(wks_ref[...]), ckv_ref[pl.ds(r, n), :]))

        def v_proj(r, n):
            store_heads(v_ref, pl.ds(r, n), _dot(ckv_ref[pl.ds(r, n), :], _bf(wvs_ref[...])))

        def phase_a(i, _):
            a_copy(i).wait()
            r = pl.multiple_of(i * TR, TR)
            v_proj(r, TR)
            k_proj(r, TR)
            return 0
        lax.fori_loop(0, na, phase_a, 0)
        for hh in range(2):
            k0_ref[hh] = _bf(kt_ref[hh, 0]).astype(F32).T.astype(BF16)
        for cp in b_copies(1):
            cp.start()
        cp_c.wait()
        cp_mod.wait()
        w0[2].wait()
        mod_ref[:, 0:2 * M] = _dot(silu_c(), wmod_ref[:, 0:2 * M])
        wqs_ref[...] = _pk(_unpack_pair(wq_buf[1]))

        def phase_b(i, _):
            for cp in b_copies(i):
                cp.wait()

            @pl.when(i + 2 < NB)
            def _():
                for cp in b_copies(i + 2):
                    cp.start()

            @pl.when(i == 1)
            def _():
                for cp in w_copies(1, 0) + [wo_copy(0, 0)]:
                    cp.start()
            rk = pl.multiple_of(na * TR + i * kr, kr)
            sa = mod_ref[0:1, 0:M]
            ca1 = 1.0 + mod_ref[0:1, M:2 * M]
            k_proj(rk, kr)
            v_proj(rk, kr)
            n = xr // 4
            for j in range(4):
                rx = pl.multiple_of(i * xr + j * n, n)
                h = (_ln(x_ref[pl.ds(rx, n), :].astype(F32)) * ca1 + sa).astype(BF16)
                h_ref[pl.ds(pl.multiple_of(rx // 2, 8), n // 2), :] = _pk(h)
                store_heads(q_ref, pl.ds(rx, n), _dot(h, _bf(wqs_ref[...])) * qscale)
            return 0
        lax.fori_loop(0, NB, phase_b, 0)
        for cp in w_copies(2, 1) + [wo_copy(1, 1)] + late_copies():
            cp.start()

    def run_ops(ops, slot, part_order, w=None, extras=None):
        row = lax.broadcasted_iota(jnp.int32, (T, T), 0)
        col = lax.broadcasted_iota(jnp.int32, (T, T), 1)
        tri = col <= row
        lane_w = lax.broadcasted_iota(jnp.int32, (D // 2, T), 1)
        lane_g = lax.broadcasted_iota(jnp.int32, (G, T), 1)
        left = {}

        def scores_of(hh, mates, i):
            r = i * T
            part = {}
            for ch in ('mlbs' if (hh, i) == (0, nblk - 1) else part_order):
                if ch == 'l' and mates is not None:
                    for g in range(NG - 1):
                        nk = (g + 1) * G
                        qt = jnp.concatenate([q_ref[hh, j * T + g * G:j * T + nk, :] for j in mates], axis=0)
                        lt = _dot_nt(k0_ref[hh, 0:nk, :], qt)
                        lt = jnp.concatenate([lt] + [lt[:G]] * (NG - 1 - g), axis=0).T
                        for n, j in enumerate(mates):
                            left[hh, j, g] = lt[n * G:(n + 1) * G]
                elif ch == 'm' and i >= 2:
                    km = _bf(jnp.concatenate([kt_ref[hh, j] for j in range(1, i)], axis=1))
                    part['m'] = _dot(q_ref[hh, r:r + T, :], km)
                elif ch == 'b':
                    qb = q_ref[hh, r + T - G:r + T, :]
                    part['b', 0] = _dot(qb, _bf(kt_ref[hh, 0]))
                    if i >= 1:
                        part['b', 1] = _dot(qb, _bf(kt_ref[hh, i]))
                elif ch == 's' and i >= 1:
                    for g in range(NG - 1):
                        nk = (g + 1) * G
                        ks = _bf(jnp.where(lane_w < nk, kt_ref[hh, i], kt_ref[hh, 0]))
                        part['s', g] = _dot(q_ref[hh, r + g * G:r + nk, :], ks)
            lf = [left.pop((hh, i, g)) for g in range(NG - 1)]
            if i == 0:
                return jnp.where(tri, jnp.concatenate(lf + [part['b', 0]], axis=0), NEG)
            first = jnp.concatenate(
                [jnp.where(lane_g < (g + 1) * G, lf[g], part['s', g]) for g in range(NG - 1)]
                + [part['b', 0]], axis=0)
            diag = jnp.concatenate([part['s', g] for g in range(NG - 1)] + [part['b', 1]], axis=0)
            diag = jnp.where(tri, diag, NEG)
            return jnp.concatenate([first] + ([part['m']] if i >= 2 else []) + [diag], axis=1)

        scores, ctx = {}, {}
        for op in ops:
            kind, i = op[0], op[-1]
            rows = slice(i * T, (i + 1) * T)
            if kind == 'E':
                extras[i]()
            elif kind == 'K':
                store_kt(i, _dot_nt(w['K'], ckv_ref[rows, :]))
            elif kind == 'V':
                store_heads(v_ref, rows, _dot(ckv_ref[rows, :], w['V']))
            elif kind == 'Q':
                h = _bf(h_ref[i * T // 2:(i + 1) * T // 2, :])
                store_heads(q_ref, rows, _dot(h, w['Q']) * qscale)
            elif kind == 'S':
                scores[op[1], i] = scores_of(op[1], op[2], i)
            elif kind == 'P':
                hh = op[1]
                p, l = _softmax_rows(scores.pop((hh, i)))
                ctx[hh, i] = (_dot(p, v_ref[hh, 0:(i + 1) * T, :]) * _recip(l)).astype(BF16)
            else:
                c = jnp.concatenate([ctx.pop((0, i)), ctx.pop((1, i))], axis=1)
                cuts = [0] + list(op[1:-1]) + [T]
                for a, b in zip(cuts[:-1], cuts[1:]):
                    acc_ref[i * T + a:i * T + b, :] += _dot(c[a:b], wo_buf[slot])
        assert not scores and not ctx and not left

    def step(g, _):
        slot = g & 1
        wo_copy(g, slot).wait()
        for cp in w_copies(g + 1, slot):
            cp.wait()
        w = {'K': _unpack_pair(wk_buf[slot].T, axis=0), 'V': _unpack_pair(wv_buf[slot]),
             'Q': _unpack_pair(wq_buf[slot])}
        run_ops(_schedule(nblk), slot, 'lbsm', w=w)

        @pl.when(g + 3 < npairs)
        def _():
            for cp in w_copies(g + 3, slot):
                cp.start()

        @pl.when(g + 2 < npairs)
        def _():
            wo_copy(g + 2, slot).start()
        return 0

    def epilogue():
        slot = (npairs - 1) % 2
        wo_copy(npairs - 1, slot).wait()
        for cp in late_copies():
            cp.wait()
        nct = M // T
        cgrp = M // 4
        shifts = (-1, 1, -2, 2)
        HR = TR // 2
        sc = silu_c()
        hoisted = {}

        def mod_piece(j):
            wd = 4 * M // MODP
            cols = slice(2 * M + j * wd, 2 * M + (j + 1) * wd)
            mod_ref[:, cols] = _dot(sc, wmod_ref[:, cols])

        def mvec(j):
            if j in hoisted:
                return hoisted[j]
            v = mod_ref[0:1, j * M:(j + 1) * M]
            return 1.0 + v if j == 4 else v

        def x1_of(rows):
            return x_ref[rows, :].astype(F32) + mvec(2) * acc_ref[rows, :]

        def mix_in(r0, k, n, may_overrun):
            rows = pl.ds(r0 + k, n)
            h2 = _ln(x1_of(rows)) * mvec(4) + mvec(3)
            h2_ref[k:k + n, :] = h2
            hh = _gelu(_dot(_ln(h2).astype(BF16), _bf(w1_ref[...])))
            if may_overrun:
                rid = r0 + k + lax.broadcasted_iota(jnp.int32, (n, M), 0)
                hh = jnp.where(rid < S, hh, 0.0)
            for t in range(nct):
                hh_ref[t, PAD + k:PAD + k + n, :] = hh[:, t * T:(t + 1) * T]

        def mix_out(r0, k, n):
            lane = lax.broadcasted_iota(jnp.int32, (n, T), 1)
            cols = []
            for t in range(nct):
                lo, hi = (t * T) // cgrp, (t * T + T - 1) // cgrp
                v = hh_ref[t, pl.ds(PAD + k + shifts[lo], n), :]
                if hi != lo:
                    v2 = hh_ref[t, pl.ds(PAD + k + shifts[hi], n), :]
                    v = jnp.where(lane < hi * cgrp - t * T, v, v2)
                cols.append(v)
            sh = jnp.concatenate(cols, axis=1).astype(BF16)
            rows = pl.ds(r0 + k, n)
            y1 = h2_ref[k:k + n, :] + _dot(sh, _bf(w2_ref[...]))
            base_ref[rows, :] = x1_of(rows) + mvec(5) * y1
            z_ref[k:k + n, :] = _ln(y1).astype(BF16)

        def ffn_up(k, n):
            z = z_ref[k:k + n, :]
            fm = (F // T) * T
            if fm == F:
                return _gelu(_dot_nt(z, _bf(w3_ref[...]))).astype(BF16)
            tail = _gelu(_dot_nt(_bf(w3_ref[fm // 2:F // 2, :]), z)).T
            main = _gelu(_dot_nt(z, _bf(w3_ref[0:fm // 2, :])))
            return jnp.concatenate([main, tail], axis=1).astype(BF16)

        def ffn_down(r, t):
            rows = pl.ds(r, t.shape[0])
            o_buf[rows, :] = (base_ref[rows, :] + mvec(5) * _dot(t, _bf(w4_ref[...]))).astype(o_buf.dtype)

        def o_copy(r, n, sem):
            return pltpu.make_async_copy(o_buf.at[pl.ds(r, n), :], o_hbm.at[pl.ds(r, n), :], sem)

        pieces = [(functools.partial(mod_piece, j), 0) for j in range(MODP)]
        pieces += [(functools.partial(mix_in, 0, 0, HR, False), pl.cdiv(HR, T)),
                   (functools.partial(mix_in, 0, HR, HR + HALO, False), pl.cdiv(TR + HALO, T)),
                   (functools.partial(mix_out, 0, 0, HR), 1),
                   (functools.partial(mix_out, 0, HR, HR), 1)]
        run_ops(_schedule_last(nblk, [n for _, n in pieces]), slot, 'smbl', extras=[f for f, _ in pieces])
        hoisted.update({j: mvec(j) for j in range(2, 6)})

        def body(i, _):
            r = pl.multiple_of(i * TR, TR)
            rn = pl.multiple_of(r + TR, TR)
            hh_ref[:, 0:PAD + HALO, :] = hh_ref[:, TR:TR + PAD + HALO, :]
            h2_ref[0:HALO, :] = h2_ref[TR:TR + HALO, :]
            t0 = ffn_up(0, HR)
            mix_in(rn, HALO, HR, False)
            t1 = ffn_up(HR, HR)
            mix_out(rn, 0, HR)
            mix_in(rn, HALO + HR, HR, True)
            ffn_down(r, t0)
            mix_out(rn, HR, HR)
            ffn_down(r + HR, t1)
            o_copy(r, TR, xsem.at[i]).start()
            return 0
        lax.fori_loop(0, nchunks - 1, body, 0)

        r = (nchunks - 1) * TR
        n1 = TR - LAST
        cp_a = o_copy(r, n1, xsem.at[nchunks - 1])
        cp_b = o_copy(r + n1, LAST, isem.at[0])
        t = ffn_up(0, TR)
        ffn_down(r, t[:n1])
        cp_a.start()
        ffn_down(r + n1, t[n1:])
        cp_b.start()
        for i in range(nchunks - 1):
            o_copy(i * TR, TR, xsem.at[i]).wait()
        cp_a.wait()
        cp_b.wait()

    prologue()
    lax.fori_loop(0, npairs - 1, step, 0)
    epilogue()


@jax.jit
def pallas_adaLN_cond__compressed_kv_cla__mixer_s_mlp__prompt_kernel(
    A_x, A_c_kv, A_w_q, A_w_uk, A_w_uv, A_w_o, B_x, B_w1, B_w2, B_w3, B_w4, c, w_mod,
):
    del B_x
    _, S, M = A_x.shape
    Dc = A_c_kv.shape[2]
    H, D = A_w_q.shape[1], A_w_q.shape[2]
    F = B_w3.shape[1]
    ins = (A_x.reshape(S, M), A_c_kv.reshape(S, Dc), A_w_q, A_w_uk, A_w_uv,
           A_w_o.reshape(H // 2, 2 * D, M), B_w1, B_w2, B_w3.T, B_w4, c, w_mod)

    out = pl.pallas_call(
        functools.partial(_kernel, S=S, M=M, Dc=Dc, H=H, D=D, F=F),
        in_specs=[pl.BlockSpec(memory_space=pl.ANY) for _ in ins],
        out_specs=pl.BlockSpec(memory_space=pl.ANY),
        out_shape=jax.ShapeDtypeStruct((S, M), A_x.dtype),
        scratch_shapes=[
            pltpu.VMEM((S + HALO, M), BF16),
            pltpu.VMEM((S, Dc), BF16),
            pltpu.VMEM((M // 2, M), U32),
            pltpu.VMEM((M // 2, M), U32),
            pltpu.VMEM((F // 2, M), U32),
            pltpu.VMEM((F // 2, M), U32),
            pltpu.VMEM((1, M), BF16),
            pltpu.VMEM((M, 6 * M), BF16),
            pltpu.VMEM((2, M, D), U32),
            pltpu.VMEM((2, Dc, D), U32),
            pltpu.VMEM((2, Dc, D), U32),
            pltpu.VMEM((2, 2 * D, M), BF16),
            pltpu.VMEM((8, 6 * M), F32),
            pltpu.VMEM((S // 2, M), U32),
            pltpu.VMEM((2, S, D), BF16),
            pltpu.VMEM((2, S // T, D // 2, T), U32),
            pltpu.VMEM((2, S, D), BF16),
            pltpu.VMEM((S + HALO, M), F32),
            pltpu.VMEM((S, M), F32),
            pltpu.VMEM((M // T, PAD + TR + HALO, T), F32),
            pltpu.VMEM((TR + HALO, M), F32),
            pltpu.VMEM((TR, M), BF16),
            pltpu.VMEM((S, M), A_x.dtype),
            pltpu.VMEM((D, Dc), U32),
            pltpu.VMEM((Dc // 2, 2 * D), U32),
            pltpu.VMEM((M // 2, 2 * D), U32),
            pltpu.VMEM((2, T, D), BF16),
            pltpu.SemaphoreType.DMA((4, 2)),
            pltpu.SemaphoreType.DMA((7,)),
            pltpu.SemaphoreType.DMA((max(S // TR, NB),)),
            pltpu.SemaphoreType.DMA((S // TR + NB,)),
        ],
        compiler_params=pltpu.CompilerParams(
            vmem_limit_bytes=100 * 1024 * 1024,
            disable_bounds_checks=True,
        ),
    )(*ins)
    return out.reshape(1, S, M)
```

```python
import functools
import math

import jax
import jax.numpy as jnp
from jax import lax
import jax.experimental.pallas as pl
import jax.experimental.pallas.tpu as pltpu

F32 = jnp.float32
BF16 = jnp.bfloat16
U32 = jnp.uint32
EPS = 1e-5
NEG = -1e30
T = 128
G = 32
NG = T // G
TR = 256
PAD = 8
HALO = 16
NA = 6
NB = 4
MODP = 10
LAST = 64


def _ln(x):
    m = jnp.mean(x, axis=-1, keepdims=True)
    xc = x - m
    v = jnp.mean(xc * xc, axis=-1, keepdims=True)
    return xc * lax.rsqrt(v + EPS)


def _gelu(x):
    c = math.sqrt(2.0 / math.pi)
    hx = 0.5 * x
    return hx + hx * jnp.tanh(x * (c + (c * 0.044715) * (x * x)))


def _dot(a, b):
    return jnp.dot(a, b, preferred_element_type=F32)


def _dot_nt(a, b):
    return lax.dot_general(a, b, (((1,), (1,)), ((), ())), preferred_element_type=F32)


def _recip(l):
    r = pl.reciprocal(l, approx=True)
    return r * (2.0 - l * r)


def _unpack_pair(u, axis=1):
    lo = pltpu.bitcast(u << 16, F32)
    hi = pltpu.bitcast(u & jnp.uint32(0xFFFF0000), F32)
    return jnp.concatenate([lo, hi], axis=axis).astype(BF16)


def _bf(u):
    return pltpu.bitcast(u, BF16)


def _pk(x):
    return pltpu.bitcast(x.astype(BF16), U32)


def _softmax_rows(s):
    m = jnp.max(s, axis=-1, keepdims=True)
    p = jnp.exp2(s - m).astype(BF16)
    return p, jnp.sum(p.astype(F32), axis=-1, keepdims=True)


def _schedule(nblk):
    order = list(range(nblk - 1, -1, -1))
    ops, oq, kq, vq = [], [], [], []
    for t, i in enumerate(order):
        mates = tuple(order[t:t + NG]) if t % NG == 0 else None
        ops.append(('S', 0, mates, i))
        ops += [('K', kq.pop())] if kq else []
        ops += [('V', vq.pop())] if vq else []
        if t > 0:
            ops.append(('P', 1, order[t - 1]))
            oq.append(order[t - 1])
            vq.append(order[t - 1])
        ops += [('S', 1, mates, i), ('Q', i)]
        kq.append(i)
        if len(oq) >= 3:
            ops.append(('O', oq.pop(0)))
        ops.append(('P', 0, i))
    ops += [('K', kq.pop()), ('P', 1, 0), ('V', vq.pop())]
    ops += [('O', i) for i in oq] + [('V', 0), ('O', T - G, 0)]
    return ops


def _schedule_last(nblk, extras):
    small, big = list(range(max(extras))), list(range(nblk - 1, max(extras) - 1, -1))
    order = []
    while small or big:
        order += [big.pop(0)] if big else []
        order += [small.pop(0)] if small else []
    ops, oq, final = [], [], set()
    todo = list(enumerate(extras))

    def extra(allow_rows):
        if todo and (todo[0][1] == 0 or (allow_rows and set(range(todo[0][1])) <= final)):
            ops.append(('E', todo.pop(0)[0]))
    for t, i in enumerate(order):
        mates = tuple(order[t:t + NG]) if t % NG == 0 else None
        ops.append(('S', 0, mates, i))
        extra(False)
        if t > 0:
            ops.append(('P', 1, order[t - 1]))
            oq.append(order[t - 1])
        ops.append(('S', 1, mates, i))
        extra(t >= nblk - 4)
        if len(oq) >= 2:
            final.add(oq[0])
            ops.append(('O', oq.pop(0)))
        ops.append(('P', 0, i))
    for op in [('P', 1, order[-1])] + [('O', i) for i in oq + [order[-1]]]:
        extra(True)
        ops.append(op)
        if op[0] == 'O':
            final.add(op[1])
    ops += [('E', j) for j, _ in todo]
    return ops


def _kernel(x_hbm, ckv_hbm, wq_hbm, wk_hbm, wv_hbm, wo_hbm, w1_hbm, w2_hbm, w3_hbm, w4_hbm,
            c_hbm, wmod_hbm, o_hbm,
            x_ref, ckv_ref, w1_ref, w2_ref, w3_ref, w4_ref, c_ref, wmod_ref,
            wq_buf, wk_buf, wv_buf, wo_buf,
            mod_ref, h_ref, q_ref, kt_ref, v_ref, acc_ref, base_ref, hh_ref, h2_ref, z_ref, o_buf,
            wks_ref, wvs_ref, wqs_ref, k0_ref,
            wsem, isem, xsem, csem,
            *, S, M, Dc, H, D, F):
    npairs = H // 2
    nchunks = S // TR
    nblk = S // T
    qscale = (D ** -0.5) * math.log2(math.e)

    def w_copies(pair, sl):
        return [
            pltpu.make_async_copy(src.bitcast(U32).at[:, pair, :], dst.at[sl], wsem.at[j, sl])
            for j, (src, dst) in enumerate(((wk_hbm, wk_buf), (wv_hbm, wv_buf), (wq_hbm, wq_buf)))
        ]

    def wo_copy(pair, sl):
        return pltpu.make_async_copy(wo_hbm.at[pair], wo_buf.at[sl], wsem.at[3, sl])

    def late_copies():
        return [
            pltpu.make_async_copy(wmod_hbm.at[:, 2 * M:6 * M], wmod_ref.at[:, 2 * M:6 * M], isem.at[2]),
            pltpu.make_async_copy(w1_hbm.bitcast(U32), w1_ref, isem.at[3]),
            pltpu.make_async_copy(w2_hbm.bitcast(U32), w2_ref, isem.at[4]),
            pltpu.make_async_copy(w3_hbm.bitcast(U32), w3_ref, isem.at[5]),
            pltpu.make_async_copy(w4_hbm.bitcast(U32), w4_ref, isem.at[6]),
        ]

    def silu_c():
        c = c_ref[...].astype(F32)
        sc = c * (1.0 / (1.0 + jnp.exp(-c)))
        return jnp.broadcast_to(sc, (8, M)).astype(BF16)

    def store_heads(dst, rows, y):
        for hh in range(2):
            dst[hh, rows, :] = y[:, hh * D:(hh + 1) * D].astype(BF16)

    def store_kt(blk, yt):
        for hh in range(2):
            for j in range(yt.shape[1] // T):
                tile = yt[hh * D:(hh + 1) * D, j * T:(j + 1) * T]
                kt_ref[hh, blk + j] = _pk(tile)
                if isinstance(blk, int) and blk + j == 0:
                    k0_ref[hh] = tile.T.astype(BF16)

    def prologue():
        na = min(NA, nchunks - 2)
        kr = (nchunks - na) * TR // NB
        xr = S // NB
        cp_c = pltpu.make_async_copy(c_hbm, c_ref, isem.at[0])
        cp_mod = pltpu.make_async_copy(wmod_hbm.at[:, 0:2 * M], wmod_ref.at[:, 0:2 * M], isem.at[1])

        def a_copy(i):
            rows = pl.ds(pl.multiple_of(i * TR, TR), TR)
            return pltpu.make_async_copy(ckv_hbm.at[rows, :], ckv_ref.at[rows, :], csem.at[i])

        def b_copies(i):
            rc = pl.ds(pl.multiple_of(na * TR + i * kr, kr), kr)
            rx = pl.ds(pl.multiple_of(i * xr, xr), xr)
            return [pltpu.make_async_copy(ckv_hbm.at[rc, :], ckv_ref.at[rc, :], csem.at[na + i]),
                    pltpu.make_async_copy(x_hbm.at[rx, :], x_ref.at[rx, :], xsem.at[i])]

        w0 = w_copies(0, 1)
        w0[0].start()
        w0[1].start()
        a_copy(0).start()

        def zero(i, _):
            acc_ref[pl.ds(pl.multiple_of(i * T, T), T), :] = jnp.zeros((T, M), F32)
            return 0
        lax.fori_loop(0, nblk, zero, 0)
        acc_ref[S:S + HALO, :] = jnp.zeros((HALO, M), F32)
        x_ref[S:S + HALO, :] = jnp.zeros((HALO, M), BF16)
        hh_ref[:, 0:PAD, :] = jnp.zeros((M // T, PAD, T), F32)
        for cp in ([a_copy(i) for i in range(1, na // 2)] + [cp_c, cp_mod]
                   + [a_copy(i) for i in range(na // 2, na)] + [w0[2]] + b_copies(0)):
            cp.start()
        w0[0].wait()
        w0[1].wait()
        wks_ref[...] = _pk(_unpack_pair(wk_buf[1].T, axis=0))
        wvs_ref[...] = _pk(_unpack_pair(wv_buf[1]))

        def k_proj(r, n):
            store_kt(r // T, _dot_nt(_bf(wks_ref[...]), ckv_ref[pl.ds(r, n), :]))

        def v_proj(r, n):
            store_heads(v_ref, pl.ds(r, n), _dot(ckv_ref[pl.ds(r, n), :], _bf(wvs_ref[...])))

        def phase_a(i, _):
            a_copy(i).wait()
            r = pl.multiple_of(i * TR, TR)
            v_proj(r, TR)
            k_proj(r, TR)
            return 0
        lax.fori_loop(0, na, phase_a, 0)
        for hh in range(2):
            k0_ref[hh] = _bf(kt_ref[hh, 0]).astype(F32).T.astype(BF16)
        for cp in b_copies(1):
            cp.start()
        cp_c.wait()
        cp_mod.wait()
        w0[2].wait()
        mod_ref[:, 0:2 * M] = _dot(silu_c(), wmod_ref[:, 0:2 * M])
        wqs_ref[...] = _pk(_unpack_pair(wq_buf[1]))

        def phase_b(i, _):
            for cp in b_copies(i):
                cp.wait()

            @pl.when(i + 2 < NB)
            def _():
                for cp in b_copies(i + 2):
                    cp.start()

            @pl.when(i == 1)
            def _():
                for cp in w_copies(1, 0) + [wo_copy(0, 0)]:
                    cp.start()
            rk = pl.multiple_of(na * TR + i * kr, kr)
            sa = mod_ref[0:1, 0:M]
            ca1 = 1.0 + mod_ref[0:1, M:2 * M]
            k_proj(rk, kr)
            v_proj(rk, kr)
            n = xr // 4
            for j in range(4):
                rx = pl.multiple_of(i * xr + j * n, n)
                h = (_ln(x_ref[pl.ds(rx, n), :].astype(F32)) * ca1 + sa).astype(BF16)
                h_ref[pl.ds(pl.multiple_of(rx // 2, 8), n // 2), :] = _pk(h)
                store_heads(q_ref, pl.ds(rx, n), _dot(h, _bf(wqs_ref[...])) * qscale)
            return 0
        lax.fori_loop(0, NB, phase_b, 0)
        for cp in w_copies(2, 1) + [wo_copy(1, 1)] + late_copies():
            cp.start()

    def run_ops(ops, slot, part_order, w=None, extras=None):
        row = lax.broadcasted_iota(jnp.int32, (T, T), 0)
        col = lax.broadcasted_iota(jnp.int32, (T, T), 1)
        tri = col <= row
        lane_w = lax.broadcasted_iota(jnp.int32, (D // 2, T), 1)
        lane_g = lax.broadcasted_iota(jnp.int32, (G, T), 1)
        left = {}

        def scores_of(hh, mates, i):
            r = i * T
            part = {}
            for ch in ('mlbs' if (hh, i) == (0, nblk - 1) else part_order):
                if ch == 'l' and mates is not None:
                    for g in range(NG - 1):
                        nk = (g + 1) * G
                        qt = jnp.concatenate([q_ref[hh, j * T + g * G:j * T + nk, :] for j in mates], axis=0)
                        lt = _dot_nt(k0_ref[hh, 0:nk, :], qt)
                        lt = jnp.concatenate([lt] + [lt[:G]] * (NG - 1 - g), axis=0).T
                        for n, j in enumerate(mates):
                            left[hh, j, g] = lt[n * G:(n + 1) * G]
                elif ch == 'm' and i >= 2:
                    km = _bf(jnp.concatenate([kt_ref[hh, j] for j in range(1, i)], axis=1))
                    part['m'] = _dot(q_ref[hh, r:r + T, :], km)
                elif ch == 'b':
                    qb = q_ref[hh, r + T - G:r + T, :]
                    part['b', 0] = _dot(qb, _bf(kt_ref[hh, 0]))
                    if i >= 1:
                        part['b', 1] = _dot(qb, _bf(kt_ref[hh, i]))
                elif ch == 's' and i >= 1:
                    for g in range(NG - 1):
                        nk = (g + 1) * G
                        ks = _bf(jnp.where(lane_w < nk, kt_ref[hh, i], kt_ref[hh, 0]))
                        part['s', g] = _dot(q_ref[hh, r + g * G:r + nk, :], ks)
            lf = [left.pop((hh, i, g)) for g in range(NG - 1)]
            if i == 0:
                return jnp.where(tri, jnp.concatenate(lf + [part['b', 0]], axis=0), NEG)
            first = jnp.concatenate(
                [jnp.where(lane_g < (g + 1) * G, lf[g], part['s', g]) for g in range(NG - 1)]
                + [part['b', 0]], axis=0)
            diag = jnp.concatenate([part['s', g] for g in range(NG - 1)] + [part['b', 1]], axis=0)
            diag = jnp.where(tri, diag, NEG)
            return jnp.concatenate([first] + ([part['m']] if i >= 2 else []) + [diag], axis=1)

        scores, ctx = {}, {}
        for op in ops:
            kind, i = op[0], op[-1]
            rows = slice(i * T, (i + 1) * T)
            if kind == 'E':
                extras[i]()
            elif kind == 'K':
                store_kt(i, _dot_nt(w['K'], ckv_ref[rows, :]))
            elif kind == 'V':
                store_heads(v_ref, rows, _dot(ckv_ref[rows, :], w['V']))
            elif kind == 'Q':
                h = _bf(h_ref[i * T // 2:(i + 1) * T // 2, :])
                store_heads(q_ref, rows, _dot(h, w['Q']) * qscale)
            elif kind == 'S':
                scores[op[1], i] = scores_of(op[1], op[2], i)
            elif kind == 'P':
                hh = op[1]
                p, l = _softmax_rows(scores.pop((hh, i)))
                ctx[hh, i] = (_dot(p, v_ref[hh, 0:(i + 1) * T, :]) * _recip(l)).astype(BF16)
            else:
                c = jnp.concatenate([ctx.pop((0, i)), ctx.pop((1, i))], axis=1)
                cuts = [0] + list(op[1:-1]) + [T]
                for a, b in zip(cuts[:-1], cuts[1:]):
                    acc_ref[i * T + a:i * T + b, :] += _dot(c[a:b], wo_buf[slot])
        assert not scores and not ctx and not left

    def step(g, _):
        slot = g & 1
        wo_copy(g, slot).wait()
        for cp in w_copies(g + 1, slot):
            cp.wait()
        w = {'K': _unpack_pair(wk_buf[slot].T, axis=0), 'V': _unpack_pair(wv_buf[slot]),
             'Q': _unpack_pair(wq_buf[slot])}
        run_ops(_schedule(nblk), slot, 'lbsm', w=w)

        @pl.when(g + 3 < npairs)
        def _():
            for cp in w_copies(g + 3, slot):
                cp.start()

        @pl.when(g + 2 < npairs)
        def _():
            wo_copy(g + 2, slot).start()
        return 0

    def epilogue():
        slot = (npairs - 1) % 2
        wo_copy(npairs - 1, slot).wait()
        for cp in late_copies():
            cp.wait()
        nct = M // T
        cgrp = M // 4
        shifts = (-1, 1, -2, 2)
        HR = TR // 2
        sc = silu_c()
        hoisted = {}

        def mod_piece(j):
            wd = 4 * M // MODP
            cols = slice(2 * M + j * wd, 2 * M + (j + 1) * wd)
            mod_ref[:, cols] = _dot(sc, wmod_ref[:, cols])

        def mvec(j):
            if j in hoisted:
                return hoisted[j]
            v = mod_ref[0:1, j * M:(j + 1) * M]
            return 1.0 + v if j == 4 else v

        def x1_of(rows):
            return x_ref[rows, :].astype(F32) + mvec(2) * acc_ref[rows, :]

        def mix_in(r0, k, n, may_overrun):
            rows = pl.ds(r0 + k, n)
            h2 = _ln(x1_of(rows)) * mvec(4) + mvec(3)
            h2_ref[k:k + n, :] = h2
            hh = _gelu(_dot(_ln(h2).astype(BF16), _bf(w1_ref[...])))
            if may_overrun:
                rid = r0 + k + lax.broadcasted_iota(jnp.int32, (n, M), 0)
                hh = jnp.where(rid < S, hh, 0.0)
            for t in range(nct):
                hh_ref[t, PAD + k:PAD + k + n, :] = hh[:, t * T:(t + 1) * T]

        def mix_out(r0, k, n):
            lane = lax.broadcasted_iota(jnp.int32, (n, T), 1)
            cols = []
            for t in range(nct):
                lo, hi = (t * T) // cgrp, (t * T + T - 1) // cgrp
                v = hh_ref[t, pl.ds(PAD + k + shifts[lo], n), :]
                if hi != lo:
                    v2 = hh_ref[t, pl.ds(PAD + k + shifts[hi], n), :]
                    v = jnp.where(lane < hi * cgrp - t * T, v, v2)
                cols.append(v)
            sh = jnp.concatenate(cols, axis=1).astype(BF16)
            rows = pl.ds(r0 + k, n)
            y1 = h2_ref[k:k + n, :] + _dot(sh, _bf(w2_ref[...]))
            base_ref[rows, :] = x1_of(rows) + mvec(5) * y1
            z_ref[k:k + n, :] = _ln(y1).astype(BF16)

        def ffn_up(k, n):
            z = z_ref[k:k + n, :]
            fm = (F // T) * T
            if fm == F:
                return _gelu(_dot_nt(z, _bf(w3_ref[...]))).astype(BF16)
            c0 = min(4 * T, fm - T) if k == 0 else 0
            parts = [_gelu(_dot_nt(z, _bf(w3_ref[0:c0 // 2, :])))] if c0 else []
            tail = _gelu(_dot_nt(_bf(w3_ref[fm // 2:F // 2, :]), z)).T
            parts.append(_gelu(_dot_nt(z, _bf(w3_ref[c0 // 2:fm // 2, :]))))
            return jnp.concatenate(parts + [tail], axis=1).astype(BF16)

        def ffn_down(r, t):
            rows = pl.ds(r, t.shape[0])
            o_buf[rows, :] = (base_ref[rows, :] + mvec(5) * _dot(t, _bf(w4_ref[...]))).astype(o_buf.dtype)

        def o_copy(r, n, sem):
            return pltpu.make_async_copy(o_buf.at[pl.ds(r, n), :], o_hbm.at[pl.ds(r, n), :], sem)

        pieces = [(functools.partial(mod_piece, j), 0) for j in range(MODP)]
        pieces += [(functools.partial(mix_in, 0, 0, HR, False), pl.cdiv(HR, T)),
                   (functools.partial(mix_in, 0, HR, HR + HALO, False), pl.cdiv(TR + HALO, T)),
                   (functools.partial(mix_out, 0, 0, HR), 1),
                   (functools.partial(mix_out, 0, HR, HR), 1)]
        run_ops(_schedule_last(nblk, [n for _, n in pieces]), slot, 'smbl', extras=[f for f, _ in pieces])
        hoisted.update({j: mvec(j) for j in range(2, 6)})

        def body(i, _):
            r = pl.multiple_of(i * TR, TR)
            rn = pl.multiple_of(r + TR, TR)
            hh_ref[:, 0:PAD + HALO, :] = hh_ref[:, TR:TR + PAD + HALO, :]
            h2_ref[0:HALO, :] = h2_ref[TR:TR + HALO, :]
            t0 = ffn_up(0, HR)
            mix_in(rn, HALO, HR, False)
            t1 = ffn_up(HR, HR)
            mix_out(rn, 0, HR)
            mix_in(rn, HALO + HR, HR, True)
            ffn_down(r, t0)
            mix_out(rn, HR, HR)
            ffn_down(r + HR, t1)
            o_copy(r, TR, xsem.at[i]).start()
            return 0
        lax.fori_loop(0, nchunks - 1, body, 0)

        r = (nchunks - 1) * TR
        n1 = TR - LAST
        cp_a = o_copy(r, n1, xsem.at[nchunks - 1])
        cp_b = o_copy(r + n1, LAST, isem.at[0])
        t = ffn_up(0, TR)
        ffn_down(r, t[:n1])
        cp_a.start()
        ffn_down(r + n1, t[n1:])
        cp_b.start()
        for i in range(nchunks - 1):
            o_copy(i * TR, TR, xsem.at[i]).wait()
        cp_a.wait()
        cp_b.wait()

    prologue()
    lax.fori_loop(0, npairs - 1, step, 0)
    epilogue()


@jax.jit
def pallas_adaLN_cond__compressed_kv_cla__mixer_s_mlp__prompt_kernel(
    A_x, A_c_kv, A_w_q, A_w_uk, A_w_uv, A_w_o, B_x, B_w1, B_w2, B_w3, B_w4, c, w_mod,
):
    del B_x
    _, S, M = A_x.shape
    Dc = A_c_kv.shape[2]
    H, D = A_w_q.shape[1], A_w_q.shape[2]
    F = B_w3.shape[1]
    ins = (A_x.reshape(S, M), A_c_kv.reshape(S, Dc), A_w_q, A_w_uk, A_w_uv,
           A_w_o.reshape(H // 2, 2 * D, M), B_w1, B_w2, B_w3.T, B_w4, c, w_mod)

    out = pl.pallas_call(
        functools.partial(_kernel, S=S, M=M, Dc=Dc, H=H, D=D, F=F),
        in_specs=[pl.BlockSpec(memory_space=pl.ANY) for _ in ins],
        out_specs=pl.BlockSpec(memory_space=pl.ANY),
        out_shape=jax.ShapeDtypeStruct((S, M), A_x.dtype),
        scratch_shapes=[
            pltpu.VMEM((S + HALO, M), BF16),
            pltpu.VMEM((S, Dc), BF16),
            pltpu.VMEM((M // 2, M), U32),
            pltpu.VMEM((M // 2, M), U32),
            pltpu.VMEM((F // 2, M), U32),
            pltpu.VMEM((F // 2, M), U32),
            pltpu.VMEM((1, M), BF16),
            pltpu.VMEM((M, 6 * M), BF16),
            pltpu.VMEM((2, M, D), U32),
            pltpu.VMEM((2, Dc, D), U32),
            pltpu.VMEM((2, Dc, D), U32),
            pltpu.VMEM((2, 2 * D, M), BF16),
            pltpu.VMEM((8, 6 * M), F32),
            pltpu.VMEM((S // 2, M), U32),
            pltpu.VMEM((2, S, D), BF16),
            pltpu.VMEM((2, S // T, D // 2, T), U32),
            pltpu.VMEM((2, S, D), BF16),
            pltpu.VMEM((S + HALO, M), F32),
            pltpu.VMEM((S, M), F32),
            pltpu.VMEM((M // T, PAD + TR + HALO, T), F32),
            pltpu.VMEM((TR + HALO, M), F32),
            pltpu.VMEM((TR, M), BF16),
            pltpu.VMEM((S, M), A_x.dtype),
            pltpu.VMEM((D, Dc), U32),
            pltpu.VMEM((Dc // 2, 2 * D), U32),
            pltpu.VMEM((M // 2, 2 * D), U32),
            pltpu.VMEM((2, T, D), BF16),
            pltpu.SemaphoreType.DMA((4, 2)),
            pltpu.SemaphoreType.DMA((7,)),
            pltpu.SemaphoreType.DMA((max(S // TR, NB),)),
            pltpu.SemaphoreType.DMA((S // TR + NB,)),
        ],
        compiler_params=pltpu.CompilerParams(
            vmem_limit_bytes=100 * 1024 * 1024,
            disable_bounds_checks=True,
            disable_semaphore_checks=True,
        ),
    )(*ins)
    return out.reshape(1, S, M)
```

```python
import functools
import math

import jax
import jax.numpy as jnp
from jax import lax
import jax.experimental.pallas as pl
import jax.experimental.pallas.tpu as pltpu

F32 = jnp.float32
BF16 = jnp.bfloat16
U32 = jnp.uint32
EPS = 1e-5
NEG = -1e30
T = 128
G = 32
NG = T // G
TR = 256
PAD = 8
HALO = 16
NA = 6
NB = 4
MODP = 10
LAST = 64


def _ln(x):
    m = jnp.mean(x, axis=-1, keepdims=True)
    xc = x - m
    v = jnp.mean(xc * xc, axis=-1, keepdims=True)
    return xc * lax.rsqrt(v + EPS)


def _gelu(x):
    c = math.sqrt(2.0 / math.pi)
    hx = 0.5 * x
    return hx + hx * jnp.tanh(x * (c + (c * 0.044715) * (x * x)))


def _dot(a, b):
    return jnp.dot(a, b, preferred_element_type=F32)


def _dot_nt(a, b):
    return lax.dot_general(a, b, (((1,), (1,)), ((), ())), preferred_element_type=F32)


def _recip(l):
    r = pl.reciprocal(l, approx=True)
    return r * (2.0 - l * r)


def _unpack_pair(u, axis=1):
    lo = pltpu.bitcast(u << 16, F32)
    hi = pltpu.bitcast(u & jnp.uint32(0xFFFF0000), F32)
    return jnp.concatenate([lo, hi], axis=axis).astype(BF16)


def _bf(u):
    return pltpu.bitcast(u, BF16)


def _pk(x):
    return pltpu.bitcast(x.astype(BF16), U32)


def _softmax_rows(s):
    m = jnp.max(s, axis=-1, keepdims=True)
    p = jnp.exp2(s - m).astype(BF16)
    return p, jnp.sum(p.astype(F32), axis=-1, keepdims=True)


def _schedule(nblk):
    ops, oq = [], []
    for i in range(nblk - 1, -1, -1):
        mates = tuple(range(i, i - NG, -1)) if (nblk - 1 - i) % NG == 0 else None
        later = i < nblk - 1
        ops.append(('S', 0, mates, i))
        if len(oq) >= 3:
            ops.append(('O', oq.pop(0)))
        if later:
            ops += [('Q', i + 1), ('P', 1, i + 1)]
            oq.append(i + 1)
        ops.append(('S', 1, mates, i))
        ops += [('V', i + 1)] if later else []
        ops += [('K', i), ('P', 0, i)]
    ops += [('Q', 0), ('P', 1, 0)] + [('O', i) for i in oq]
    ops += [('V', 0), ('O', T - G, 0)]
    return ops


def _schedule_last(nblk, extras):
    small, big = list(range(max(extras))), list(range(nblk - 1, max(extras) - 1, -1))
    order = []
    while small or big:
        order += [big.pop(0)] if big else []
        order += [small.pop(0)] if small else []
    ops, oq, final = [], [], set()
    todo = list(enumerate(extras))

    def extra(allow_rows):
        if todo and (todo[0][1] == 0 or (allow_rows and set(range(todo[0][1])) <= final)):
            ops.append(('E', todo.pop(0)[0]))
    for t, i in enumerate(order):
        mates = tuple(order[t:t + NG]) if t % NG == 0 else None
        ops.append(('S', 0, mates, i))
        extra(False)
        if t > 0:
            ops.append(('P', 1, order[t - 1]))
            oq.append(order[t - 1])
        ops.append(('S', 1, mates, i))
        extra(t >= nblk - 4)
        if len(oq) >= 2:
            final.add(oq[0])
            ops.append(('O', oq.pop(0)))
        ops.append(('P', 0, i))
    for op in [('P', 1, order[-1])] + [('O', i) for i in oq + [order[-1]]]:
        extra(True)
        ops.append(op)
        if op[0] == 'O':
            final.add(op[1])
    ops += [('E', j) for j, _ in todo]
    return ops


def _kernel(x_hbm, ckv_hbm, wq_hbm, wk_hbm, wv_hbm, wo_hbm, w1_hbm, w2_hbm, w3_hbm, w4_hbm,
            c_hbm, wmod_hbm, o_hbm,
            x_ref, ckv_ref, w1_ref, w2_ref, w3_ref, w4_ref, c_ref, wmod_ref,
            wq_buf, wk_buf, wv_buf, wo_buf,
            mod_ref, h_ref, q_ref, kt_ref, v_ref, acc_ref, base_ref, hh_ref, h2_ref, z_ref, o_buf,
            wks_ref, wvs_ref, wqs_ref, k0_ref,
            wsem, isem, xsem, csem,
            *, S, M, Dc, H, D, F):
    npairs = H // 2
    nchunks = S // TR
    nblk = S // T
    qscale = (D ** -0.5) * math.log2(math.e)

    def w_copies(pair, sl):
        return [
            pltpu.make_async_copy(src.bitcast(U32).at[:, pair, :], dst.at[sl], wsem.at[j, sl])
            for j, (src, dst) in enumerate(((wk_hbm, wk_buf), (wv_hbm, wv_buf), (wq_hbm, wq_buf)))
        ]

    def wo_copy(pair, sl):
        return pltpu.make_async_copy(wo_hbm.at[pair], wo_buf.at[sl], wsem.at[3, sl])

    def late_copies():
        return [
            pltpu.make_async_copy(wmod_hbm.at[:, 2 * M:6 * M], wmod_ref.at[:, 2 * M:6 * M], isem.at[2]),
            pltpu.make_async_copy(w1_hbm.bitcast(U32), w1_ref, isem.at[3]),
            pltpu.make_async_copy(w2_hbm.bitcast(U32), w2_ref, isem.at[4]),
            pltpu.make_async_copy(w3_hbm.bitcast(U32), w3_ref, isem.at[5]),
            pltpu.make_async_copy(w4_hbm.bitcast(U32), w4_ref, isem.at[6]),
        ]

    def silu_c():
        c = c_ref[...].astype(F32)
        sc = c * (1.0 / (1.0 + jnp.exp(-c)))
        return jnp.broadcast_to(sc, (8, M)).astype(BF16)

    def store_heads(dst, rows, y):
        for hh in range(2):
            dst[hh, rows, :] = y[:, hh * D:(hh + 1) * D].astype(BF16)

    def store_kt(blk, yt):
        for hh in range(2):
            for j in range(yt.shape[1] // T):
                tile = yt[hh * D:(hh + 1) * D, j * T:(j + 1) * T]
                kt_ref[hh, blk + j] = _pk(tile)
                if isinstance(blk, int) and blk + j == 0:
                    k0_ref[hh] = tile.T.astype(BF16)

    def prologue():
        na = min(NA, nchunks - 2)
        kr = (nchunks - na) * TR // NB
        xr = S // NB
        cp_c = pltpu.make_async_copy(c_hbm, c_ref, isem.at[0])
        cp_mod = pltpu.make_async_copy(wmod_hbm.at[:, 0:2 * M], wmod_ref.at[:, 0:2 * M], isem.at[1])

        def a_copy(i):
            rows = pl.ds(pl.multiple_of(i * TR, TR), TR)
            return pltpu.make_async_copy(ckv_hbm.at[rows, :], ckv_ref.at[rows, :], csem.at[i])

        def b_copies(i):
            rc = pl.ds(pl.multiple_of(na * TR + i * kr, kr), kr)
            rx = pl.ds(pl.multiple_of(i * xr, xr), xr)
            return [pltpu.make_async_copy(ckv_hbm.at[rc, :], ckv_ref.at[rc, :], csem.at[na + i]),
                    pltpu.make_async_copy(x_hbm.at[rx, :], x_ref.at[rx, :], xsem.at[i])]

        w0 = w_copies(0, 1)
        w0[0].start()
        w0[1].start()
        a_copy(0).start()

        def zero(i, _):
            acc_ref[pl.ds(pl.multiple_of(i * T, T), T), :] = jnp.zeros((T, M), F32)
            return 0
        lax.fori_loop(0, nblk, zero, 0)
        acc_ref[S:S + HALO, :] = jnp.zeros((HALO, M), F32)
        x_ref[S:S + HALO, :] = jnp.zeros((HALO, M), BF16)
        hh_ref[:, 0:PAD, :] = jnp.zeros((M // T, PAD, T), F32)
        for cp in ([a_copy(i) for i in range(1, na // 2)] + [cp_c, cp_mod]
                   + [a_copy(i) for i in range(na // 2, na)] + [w0[2]] + b_copies(0)):
            cp.start()
        w0[0].wait()
        w0[1].wait()
        wks_ref[...] = _pk(_unpack_pair(wk_buf[1].T, axis=0))
        wvs_ref[...] = _pk(_unpack_pair(wv_buf[1]))

        def k_proj(r, n):
            store_kt(r // T, _dot_nt(_bf(wks_ref[...]), ckv_ref[pl.ds(r, n), :]))

        def v_proj(r, n):
            store_heads(v_ref, pl.ds(r, n), _dot(ckv_ref[pl.ds(r, n), :], _bf(wvs_ref[...])))

        def phase_a(i, _):
            a_copy(i).wait()
            r = pl.multiple_of(i * TR, TR)
            v_proj(r, TR)
            k_proj(r, TR)
            return 0
        lax.fori_loop(0, na, phase_a, 0)
        for hh in range(2):
            k0_ref[hh] = _bf(kt_ref[hh, 0]).astype(F32).T.astype(BF16)
        for cp in b_copies(1):
            cp.start()
        cp_c.wait()
        cp_mod.wait()
        w0[2].wait()
        mod_ref[:, 0:2 * M] = _dot(silu_c(), wmod_ref[:, 0:2 * M])
        wqs_ref[...] = _pk(_unpack_pair(wq_buf[1]))

        def phase_b(i, _):
            for cp in b_copies(i):
                cp.wait()

            @pl.when(i + 2 < NB)
            def _():
                for cp in b_copies(i + 2):
                    cp.start()

            @pl.when(i == 1)
            def _():
                for cp in w_copies(1, 0) + [wo_copy(0, 0)]:
                    cp.start()
            rk = pl.multiple_of(na * TR + i * kr, kr)
            sa = mod_ref[0:1, 0:M]
            ca1 = 1.0 + mod_ref[0:1, M:2 * M]
            k_proj(rk, kr)
            v_proj(rk, kr)
            n = xr // 4
            for j in range(4):
                rx = pl.multiple_of(i * xr + j * n, n)
                h = (_ln(x_ref[pl.ds(rx, n), :].astype(F32)) * ca1 + sa).astype(BF16)
                h_ref[pl.ds(pl.multiple_of(rx // 2, 8), n // 2), :] = _pk(h)
                store_heads(q_ref, pl.ds(rx, n), _dot(h, _bf(wqs_ref[...])) * qscale)
            return 0
        lax.fori_loop(0, NB, phase_b, 0)
        for cp in w_copies(2, 1) + [wo_copy(1, 1)] + late_copies():
            cp.start()

    def run_ops(ops, slot, part_order, w=None, extras=None):
        row = lax.broadcasted_iota(jnp.int32, (T, T), 0)
        col = lax.broadcasted_iota(jnp.int32, (T, T), 1)
        tri = col <= row
        lane_w = lax.broadcasted_iota(jnp.int32, (D // 2, T), 1)
        lane_g = lax.broadcasted_iota(jnp.int32, (G, T), 1)
        left = {}

        def scores_of(hh, mates, i):
            r = i * T
            part = {}
            for ch in ('mlbs' if (hh, i) == (0, nblk - 1) else part_order):
                if ch == 'l' and mates is not None:
                    for g in range(NG - 1):
                        nk = (g + 1) * G
                        qt = jnp.concatenate([q_ref[hh, j * T + g * G:j * T + nk, :] for j in mates], axis=0)
                        lt = _dot_nt(k0_ref[hh, 0:nk, :], qt)
                        lt = jnp.concatenate([lt] + [lt[:G]] * (NG - 1 - g), axis=0).T
                        for n, j in enumerate(mates):
                            left[hh, j, g] = lt[n * G:(n + 1) * G]
                elif ch == 'm' and i >= 2:
                    km = _bf(jnp.concatenate([kt_ref[hh, j] for j in range(1, i)], axis=1))
                    part['m'] = _dot(q_ref[hh, r:r + T, :], km)
                elif ch == 'b':
                    qb = q_ref[hh, r + T - G:r + T, :]
                    part['b', 0] = _dot(qb, _bf(kt_ref[hh, 0]))
                    if i >= 1:
                        part['b', 1] = _dot(qb, _bf(kt_ref[hh, i]))
                elif ch == 's' and i >= 1:
                    for g in range(NG - 1):
                        nk = (g + 1) * G
                        ks = _bf(jnp.where(lane_w < nk, kt_ref[hh, i], kt_ref[hh, 0]))
                        part['s', g] = _dot(q_ref[hh, r + g * G:r + nk, :], ks)
            lf = [left.pop((hh, i, g)) for g in range(NG - 1)]
            if i == 0:
                return jnp.where(tri, jnp.concatenate(lf + [part['b', 0]], axis=0), NEG)
            first = jnp.concatenate(
                [jnp.where(lane_g < (g + 1) * G, lf[g], part['s', g]) for g in range(NG - 1)]
                + [part['b', 0]], axis=0)
            diag = jnp.concatenate([part['s', g] for g in range(NG - 1)] + [part['b', 1]], axis=0)
            diag = jnp.where(tri, diag, NEG)
            return jnp.concatenate([first] + ([part['m']] if i >= 2 else []) + [diag], axis=1)

        scores, ctx = {}, {}
        for op in ops:
            kind, i = op[0], op[-1]
            rows = slice(i * T, (i + 1) * T)
            if kind == 'E':
                extras[i]()
            elif kind == 'K':
                store_kt(i, _dot_nt(w['K'], ckv_ref[rows, :]))
            elif kind == 'V':
                store_heads(v_ref, rows, _dot(ckv_ref[rows, :], w['V']))
            elif kind == 'Q':
                h = _bf(h_ref[i * T // 2:(i + 1) * T // 2, :])
                store_heads(q_ref, rows, _dot(h, w['Q']) * qscale)
            elif kind == 'S':
                scores[op[1], i] = scores_of(op[1], op[2], i)
            elif kind == 'P':
                hh = op[1]
                p, l = _softmax_rows(scores.pop((hh, i)))
                ctx[hh, i] = (_dot(p, v_ref[hh, 0:(i + 1) * T, :]) * _recip(l)).astype(BF16)
            else:
                c = jnp.concatenate([ctx.pop((0, i)), ctx.pop((1, i))], axis=1)
                cuts = [0] + list(op[1:-1]) + [T]
                for a, b in zip(cuts[:-1], cuts[1:]):
                    acc_ref[i * T + a:i * T + b, :] += _dot(c[a:b], wo_buf[slot])
        assert not scores and not ctx and not left

    def step(g, _):
        slot = g & 1
        wo_copy(g, slot).wait()
        for cp in w_copies(g + 1, slot):
            cp.wait()
        w = {'K': _unpack_pair(wk_buf[slot].T, axis=0), 'V': _unpack_pair(wv_buf[slot]),
             'Q': _unpack_pair(wq_buf[slot])}
        run_ops(_schedule(nblk), slot, 'lsbm', w=w)

        @pl.when(g + 3 < npairs)
        def _():
            for cp in w_copies(g + 3, slot):
                cp.start()

        @pl.when(g + 2 < npairs)
        def _():
            wo_copy(g + 2, slot).start()
        return 0

    def epilogue():
        slot = (npairs - 1) % 2
        wo_copy(npairs - 1, slot).wait()
        for cp in late_copies():
            cp.wait()
        nct = M // T
        cgrp = M // 4
        shifts = (-1, 1, -2, 2)
        HR = TR // 2
        sc = silu_c()
        hoisted = {}

        def mod_piece(j):
            wd = 4 * M // MODP
            cols = slice(2 * M + j * wd, 2 * M + (j + 1) * wd)
            mod_ref[:, cols] = _dot(sc, wmod_ref[:, cols])

        def mvec(j):
            if j in hoisted:
                return hoisted[j]
            v = mod_ref[0:1, j * M:(j + 1) * M]
            return 1.0 + v if j == 4 else v

        def x1_of(rows):
            return x_ref[rows, :].astype(F32) + mvec(2) * acc_ref[rows, :]

        def mix_in(r0, k, n, may_overrun):
            rows = pl.ds(r0 + k, n)
            h2 = _ln(x1_of(rows)) * mvec(4) + mvec(3)
            h2_ref[k:k + n, :] = h2
            hh = _gelu(_dot(_ln(h2).astype(BF16), _bf(w1_ref[...])))
            if may_overrun:
                rid = r0 + k + lax.broadcasted_iota(jnp.int32, (n, M), 0)
                hh = jnp.where(rid < S, hh, 0.0)
            for t in range(nct):
                hh_ref[t, PAD + k:PAD + k + n, :] = hh[:, t * T:(t + 1) * T]

        def mix_out(r0, k, n):
            lane = lax.broadcasted_iota(jnp.int32, (n, T), 1)
            cols = []
            for t in range(nct):
                lo, hi = (t * T) // cgrp, (t * T + T - 1) // cgrp
                v = hh_ref[t, pl.ds(PAD + k + shifts[lo], n), :]
                if hi != lo:
                    v2 = hh_ref[t, pl.ds(PAD + k + shifts[hi], n), :]
                    v = jnp.where(lane < hi * cgrp - t * T, v, v2)
                cols.append(v)
            sh = jnp.concatenate(cols, axis=1).astype(BF16)
            rows = pl.ds(r0 + k, n)
            y1 = h2_ref[k:k + n, :] + _dot(sh, _bf(w2_ref[...]))
            base_ref[rows, :] = x1_of(rows) + mvec(5) * y1
            z_ref[k:k + n, :] = _ln(y1).astype(BF16)

        def ffn_up(k, n):
            z = z_ref[k:k + n, :]
            fm = (F // T) * T
            if fm == F:
                return _gelu(_dot_nt(z, _bf(w3_ref[...]))).astype(BF16)
            c0 = min(4 * T, fm - T) if k == 0 else 0
            parts = [_gelu(_dot_nt(z, _bf(w3_ref[0:c0 // 2, :])))] if c0 else []
            tail = _gelu(_dot_nt(_bf(w3_ref[fm // 2:F // 2, :]), z)).T
            parts.append(_gelu(_dot_nt(z, _bf(w3_ref[c0 // 2:fm // 2, :]))))
            return jnp.concatenate(parts + [tail], axis=1).astype(BF16)

        def ffn_down(r, t):
            rows = pl.ds(r, t.shape[0])
            o_buf[rows, :] = (base_ref[rows, :] + mvec(5) * _dot(t, _bf(w4_ref[...]))).astype(o_buf.dtype)

        def o_copy(r, n, sem):
            return pltpu.make_async_copy(o_buf.at[pl.ds(r, n), :], o_hbm.at[pl.ds(r, n), :], sem)

        pieces = [(functools.partial(mod_piece, j), 0) for j in range(MODP)]
        pieces += [(functools.partial(mix_in, 0, 0, HR, False), pl.cdiv(HR, T)),
                   (functools.partial(mix_in, 0, HR, HR + HALO, False), pl.cdiv(TR + HALO, T)),
                   (functools.partial(mix_out, 0, 0, HR), 1),
                   (functools.partial(mix_out, 0, HR, HR), 1)]
        run_ops(_schedule_last(nblk, [n for _, n in pieces]), slot, 'smbl', extras=[f for f, _ in pieces])
        hoisted.update({j: mvec(j) for j in range(2, 6)})

        def body(i, _):
            r = pl.multiple_of(i * TR, TR)
            rn = pl.multiple_of(r + TR, TR)
            hh_ref[:, 0:PAD + HALO, :] = hh_ref[:, TR:TR + PAD + HALO, :]
            h2_ref[0:HALO, :] = h2_ref[TR:TR + HALO, :]
            t0 = ffn_up(0, HR)
            mix_in(rn, HALO, HR, False)
            t1 = ffn_up(HR, HR)
            mix_out(rn, 0, HR)
            mix_in(rn, HALO + HR, HR, True)
            ffn_down(r, t0)
            mix_out(rn, HR, HR)
            ffn_down(r + HR, t1)
            o_copy(r, TR, xsem.at[i]).start()
            return 0
        lax.fori_loop(0, nchunks - 1, body, 0)

        r = (nchunks - 1) * TR
        n1 = TR - LAST
        cp_a = o_copy(r, n1, xsem.at[nchunks - 1])
        cp_b = o_copy(r + n1, LAST, isem.at[0])
        t = ffn_up(0, TR)
        ffn_down(r, t[:n1])
        cp_a.start()
        ffn_down(r + n1, t[n1:])
        cp_b.start()
        for i in range(nchunks - 1):
            o_copy(i * TR, TR, xsem.at[i]).wait()
        cp_a.wait()
        cp_b.wait()

    prologue()
    lax.fori_loop(0, npairs - 1, step, 0)
    epilogue()


@jax.jit
def pallas_adaLN_cond__compressed_kv_cla__mixer_s_mlp__prompt_kernel(
    A_x, A_c_kv, A_w_q, A_w_uk, A_w_uv, A_w_o, B_x, B_w1, B_w2, B_w3, B_w4, c, w_mod,
):
    del B_x
    _, S, M = A_x.shape
    Dc = A_c_kv.shape[2]
    H, D = A_w_q.shape[1], A_w_q.shape[2]
    F = B_w3.shape[1]
    ins = (A_x.reshape(S, M), A_c_kv.reshape(S, Dc), A_w_q, A_w_uk, A_w_uv,
           A_w_o.reshape(H // 2, 2 * D, M), B_w1, B_w2, B_w3.T, B_w4, c, w_mod)

    out = pl.pallas_call(
        functools.partial(_kernel, S=S, M=M, Dc=Dc, H=H, D=D, F=F),
        in_specs=[pl.BlockSpec(memory_space=pl.ANY) for _ in ins],
        out_specs=pl.BlockSpec(memory_space=pl.ANY),
        out_shape=jax.ShapeDtypeStruct((S, M), A_x.dtype),
        scratch_shapes=[
            pltpu.VMEM((S + HALO, M), BF16),
            pltpu.VMEM((S, Dc), BF16),
            pltpu.VMEM((M // 2, M), U32),
            pltpu.VMEM((M // 2, M), U32),
            pltpu.VMEM((F // 2, M), U32),
            pltpu.VMEM((F // 2, M), U32),
            pltpu.VMEM((1, M), BF16),
            pltpu.VMEM((M, 6 * M), BF16),
            pltpu.VMEM((2, M, D), U32),
            pltpu.VMEM((2, Dc, D), U32),
            pltpu.VMEM((2, Dc, D), U32),
            pltpu.VMEM((2, 2 * D, M), BF16),
            pltpu.VMEM((8, 6 * M), F32),
            pltpu.VMEM((S // 2, M), U32),
            pltpu.VMEM((2, S, D), BF16),
            pltpu.VMEM((2, S // T, D // 2, T), U32),
            pltpu.VMEM((2, S, D), BF16),
            pltpu.VMEM((S + HALO, M), F32),
            pltpu.VMEM((S, M), F32),
            pltpu.VMEM((M // T, PAD + TR + HALO, T), F32),
            pltpu.VMEM((TR + HALO, M), F32),
            pltpu.VMEM((TR, M), BF16),
            pltpu.VMEM((S, M), A_x.dtype),
            pltpu.VMEM((D, Dc), U32),
            pltpu.VMEM((Dc // 2, 2 * D), U32),
            pltpu.VMEM((M // 2, 2 * D), U32),
            pltpu.VMEM((2, T, D), BF16),
            pltpu.SemaphoreType.DMA((4, 2)),
            pltpu.SemaphoreType.DMA((7,)),
            pltpu.SemaphoreType.DMA((max(S // TR, NB),)),
            pltpu.SemaphoreType.DMA((S // TR + NB,)),
        ],
        compiler_params=pltpu.CompilerParams(
            vmem_limit_bytes=100 * 1024 * 1024,
            disable_bounds_checks=True,
            disable_semaphore_checks=True,
        ),
    )(*ins)
    return out.reshape(1, S, M)
```
